```python
import jax
import jax.numpy as jnp

def _softmax(x, axis=-1):
    return jax.nn.softmax(x, axis=axis)
def _gelu(x):
    return jax.nn.gelu(x, approximate=True)
def _silu(x):
    return jax.nn.silu(x)
def _sigmoid(x):
    return jax.nn.sigmoid(x)
def _layernorm(x, axis=-1, eps=1e-5):
    m = jnp.mean(x, axis=axis, keepdims=True)
    v = jnp.var(x, axis=axis, keepdims=True)
    return (x - m) / jnp.sqrt(v + eps)
def _scatter_add(tgt, idx, src, axis=0):
    return tgt.at[idx].add(src)
def _segment_sum(src, seg, n):
    return jax.ops.segment_sum(src, seg, n)
class _Rng:
    def __init__(self, key):
        self._k = key
    def _next(self):
        self._k, sub = jax.random.split(self._k)
        return sub
    def normal(self, shape):
        return jax.random.normal(self._next(), shape, dtype=jnp.bfloat16)
    def randint(self, lo, hi, shape):
        return jax.random.randint(self._next(), shape, lo, hi, dtype=jnp.int32)
    def uniform(self, shape, lo=0.0, hi=1.0):
        return jax.random.uniform(self._next(), shape, jnp.bfloat16, lo, hi)
    def permutation(self, n):
        return jax.random.permutation(self._next(), n)


kernel_name = 'interleave_layers__compressed_kv_cla__moe_arch_mod__decode'

def setup_inputs():
    _rng = _Rng(jax.random.key(int.from_bytes(__import__("os").urandom(4), "little")))
    _w = (lambda a: (lambda t: t.astype(jnp.bfloat16) if jnp.issubdtype(t.dtype, jnp.floating) else t)(jnp.asarray(a)))
    def _A_setup():
        B, H, Sq, Sk, D, M = 1, 32, 1, 4096, 128, 640
        Dc = 4 * D
        return {
            "x": _w((lambda *s: _rng.normal(s) * 0.05)(B, Sq, M)),
            "c_kv": _w((lambda *s: _rng.normal(s) * 0.05)(B, Sk, Dc)),
            "w_q": _w((lambda *s: _rng.normal(s) * 0.05)(M, H, D) * (M ** -0.5)),
            "w_uk": _w((lambda *s: _rng.normal(s) * 0.05)(Dc, H, D) * (Dc ** -0.5)),
            "w_uv": _w((lambda *s: _rng.normal(s) * 0.05)(Dc, H, D) * (Dc ** -0.5)),
            "w_o": _w((lambda *s: _rng.normal(s) * 0.05)(H, D, M) * ((H * D) ** -0.5)),
        }
    _A_in = _A_setup()

    def _B_setup():
        B, S, D, F, C = 1, 1, 640, 1728, 1
        return {
            "x": _w((lambda *s: _rng.normal(s) * 0.05)(B, S, D)),
            "w_r": _w((lambda *s: _rng.normal(s) * 0.05)(D)),
            "w_gate": _w((lambda *s: _rng.normal(s) * 0.05)(D, F)),
            "w_up": _w((lambda *s: _rng.normal(s) * 0.05)(D, F)),
            "w_down": _w((lambda *s: _rng.normal(s) * 0.05)(F, D)),
        }
    _B_in = _B_setup()

    return {
        "A_x": _A_in["x"],
        "A_c_kv": _A_in["c_kv"],
        "A_w_q": _A_in["w_q"],
        "A_w_uk": _A_in["w_uk"],
        "A_w_uv": _A_in["w_uv"],
        "A_w_o": _A_in["w_o"],
        "B_x": _B_in["x"],
        "B_w_r": _B_in["w_r"],
        "B_w_gate": _B_in["w_gate"],
        "B_w_up": _B_in["w_up"],
        "B_w_down": _B_in["w_down"],
    }

def reference(A_x, A_c_kv, A_w_q, A_w_uk, A_w_uv, A_w_o, B_x, B_w_r, B_w_gate, B_w_up, B_w_down):
    def _A_ref(x, c_kv, w_q, w_uk, w_uv, w_o):
        B, Sq, M = x.shape[0], x.shape[1], x.shape[2]
        Sk = c_kv.shape[1]
        H, D = w_q.shape[1], w_q.shape[2]
        q = jnp.einsum("bqm,mhd->bhqd", x, w_q)
        k = jnp.einsum("bkc,chd->bhkd", c_kv, w_uk)
        v = jnp.einsum("bkc,chd->bhkd", c_kv, w_uv)
        scores = jnp.einsum("bhqd,bhkd->bhqk", q, k) * (D ** -0.5)
        off = Sk - Sq
        qi = jnp.arange(Sq)[:, None]
        kj = jnp.arange(Sk)[None, :]
        cmask = kj <= (qi + off)
        scores = jnp.where(cmask[None, None], scores, -1e9)
        p = _softmax(scores, axis=-1)
        ctx = jnp.einsum("bhqk,bhkd->bhqd", p, v)
        return jnp.einsum("bhqd,hdm->bqm", ctx, w_o)

    def _B_ref(x, w_r, w_gate, w_up, w_down):
        B, S, D = x.shape
        C = 1
        r = x @ w_r
        idx = jnp.argsort(-r, axis=-1)[:, :C]
        idx_e = jnp.repeat(idx.reshape(B, C, 1), D, axis=2)
        x_sel = jnp.take_along_axis(x, idx_e, axis=1)
        g = _silu(x_sel @ w_gate)
        u = x_sel @ w_up
        y = (g * u) @ w_down
        r_sel = _sigmoid(jnp.take_along_axis(r, idx, axis=1))
        y = y * r_sel.reshape(B, C, 1)
        b_off = (jnp.arange(B) * S).reshape(B, 1)
        flat_idx = (idx + b_off).reshape(B * C)
        zero = (x * 0.0).reshape(B * S, D)
        upd = _scatter_add(zero, flat_idx, y.reshape(B * C, D), axis=0)
        return x + upd.reshape(B, S, D)

    x = A_x
    x = x + _A_ref(_layernorm(x, axis=-1), A_c_kv, A_w_q, A_w_uk, A_w_uv, A_w_o)
    x = x + _B_ref(_layernorm(x, axis=-1), B_w_r, B_w_gate, B_w_up, B_w_down)
    x = x + _A_ref(_layernorm(x, axis=-1), A_c_kv, A_w_q, A_w_uk, A_w_uv, A_w_o)
    x = x + _B_ref(_layernorm(x, axis=-1), B_w_r, B_w_gate, B_w_up, B_w_down)
    return x
```

```python
import jax
import numpy as np
import jax.numpy as jnp
import jax.experimental.pallas as pl
import jax.experimental.pallas.tpu as pltpu

F32 = jnp.float32
BF16 = jnp.bfloat16
U32 = jnp.uint32

M, H, D, SK, DC, FF = 640, 32, 128, 4096, 512, 1728
NB = M // 128
NCB = DC // 128
NKB = SK // 128
NFB = (FF + 127) // 128
EPS = 1e-5


def _rb(x):
    return x.astype(BF16).astype(F32)


def _ld(uref, idx, r0, nrows):
    return pltpu.bitcast(uref[(*idx, pl.ds(r0 // 2, nrows // 2), slice(None))], BF16)


def _dot(a, b):
    return jax.lax.dot_general(a, b, (((1,), (0,)), ((), ())), preferred_element_type=F32)


def _layernorm(x):
    m = jnp.sum(x, axis=1, keepdims=True) * (1.0 / M)
    xc = x - m
    v = jnp.sum(xc * xc, axis=1, keepdims=True) * (1.0 / M)
    return xc * jax.lax.rsqrt(v + EPS)


def _kernel(x_hbm, wq_hbm, wuk_hbm, ckv_hbm, wuv_hbm, wo_hbm, wr_hbm, g_hbm, u_hbm, wd_hbm,
            o_ref,
            x_v, wr_v, wq_v, wuk_v, ckv_v, wuv_v, wo_v, g_v, u_v, wd_v,
            WQ, WKT, CT, WV, GT, UT, sems):
    cps = {}
    n = [0]

    def add(name, src, dst):
        cps[name] = pltpu.make_async_copy(src, dst, sems.at[n[0]])
        n[0] += 1

    add('x', x_hbm, x_v)
    add('wr', wr_hbm, wr_v)
    add('wq', wq_hbm, wq_v)
    add('wuk', wuk_hbm, wuk_v)
    for j in range(NCB):
        add(f'ckv{j}', ckv_hbm.at[:, pl.ds(128 * j, 128)], ckv_v.at[j])
    add('g', g_hbm, g_v)
    add('u', u_hbm, u_v)
    add('wuv', wuv_hbm, wuv_v)
    add('wo', wo_hbm, wo_v)
    add('wd', wd_hbm, wd_v)
    for c in cps.values():
        c.start()

    wq_u, wuk_u, wuv_u, ckv_u = (r.bitcast(U32) for r in (wq_v, wuk_v, wuv_v, ckv_v))

    def shuffle16(src_u, r0, hh, s):
        blk = src_u.at[pl.ds(pl.multiple_of(r0 * 16, 256), 256)]
        a = blk[pl.ds(8 * hh + s, 8, stride=32), :]
        b = blk[pl.ds(16 + 8 * hh + s, 8, stride=32), :]
        e = (a & np.uint32(0xFFFF)) | (b << 16)
        f = (a >> 16) | (b & np.uint32(0xFFFF0000))
        return e, f

    def relayout_q():
        def body(i, _):
            b = i // 8
            m16 = i % 8
            for hh in range(2):
                for s in range(8):
                    e, f = shuffle16(wq_u, i * 16, hh, s)
                    h = 16 * hh + 2 * s
                    WQ[b, pl.ds(pl.multiple_of(h * 64 + m16 * 8, 8), 8), :] = e
                    WQ[b, pl.ds(pl.multiple_of((h + 1) * 64 + m16 * 8, 8), 8), :] = f
            return 0
        jax.lax.fori_loop(0, M // 16, body, 0)

    def relayout_v():
        def body(i, _):
            for hh in range(2):
                for s in range(8):
                    e, f = shuffle16(wuv_u, i * 16, hh, s)
                    h = 16 * hh + 2 * s
                    WV[h, pl.ds(pl.multiple_of(i * 8, 8), 8), :] = e
                    WV[h + 1, pl.ds(pl.multiple_of(i * 8, 8), 8), :] = f
            return 0
        jax.lax.fori_loop(0, DC // 16, body, 0)

    def relayout_k():
        def body(i, _):
            for hh in range(2):
                for s in range(8):
                    e, f = shuffle16(wuk_u, i * 16, hh, s)
                    h = 16 * hh + 2 * s
                    WV[h, pl.ds(pl.multiple_of(i * 8, 8), 8), :] = e
                    WV[h + 1, pl.ds(pl.multiple_of(i * 8, 8), 8), :] = f
            return 0
        jax.lax.fori_loop(0, DC // 16, body, 0)

        def body2(h, _):
            g = h // 8
            j = h % 8
            for cb in range(NCB):
                t = pltpu.bitcast(WV[h, pl.ds(cb * 64, 64), :], BF16).T
                WKT[g * 4 + cb, pl.ds(pl.multiple_of(j * 64, 64), 64), :] = pltpu.bitcast(t, U32)
            return 0
        jax.lax.fori_loop(0, H, body2, 0)

    def relayout_c():
        def body(kb, _):
            for cb in range(NCB):
                t = pltpu.bitcast(ckv_u[cb, pl.ds(pl.multiple_of(kb * 64, 64), 64), :], BF16).T
                CT[kb, pl.ds(cb * 64, 64), :] = pltpu.bitcast(t, U32)
            return 0
        jax.lax.fori_loop(0, NKB, body, 0)

    def relayout_f(src, dst):
        def body(fb, _):
            for b in range(NB):
                t = src[pl.ds(pl.multiple_of(fb * 128, 128), 128), pl.ds(b * 128, 128)].T
                dst[fb, pl.ds(b * 64, 64), :] = pltpu.bitcast(t, U32)
            return 0
        jax.lax.fori_loop(0, NFB - 1, body, 0)
        for b in range(NB):
            t = src[pl.ds((NFB - 1) * 128, 64), pl.ds(b * 128, 128)]
            t = jnp.concatenate([t, jnp.zeros((64, 128), BF16)], axis=0).T
            dst[NFB - 1, pl.ds(b * 64, 64), :] = pltpu.bitcast(t, U32)

    row8 = jax.lax.broadcasted_iota(jnp.int32, (8, 128), 0)

    def blockdiag(vparts):
        return jnp.concatenate(
            [jnp.where(row8 == j, p, 0.0) for j in range(8) for p in vparts], axis=1)

    def attn(xn, first):
        xb = _rb(xn)
        if first:
            cps['wq'].wait()
            relayout_q()
        q = []
        for g in range(4):
            acc = None
            for b in range(NB):
                lhs = blockdiag([xb[:, b * 128:(b + 1) * 128]])
                r = _dot(lhs, _ld(WQ, (b,), g * 1024, 1024))
                acc = r if acc is None else acc + r
            q.append(_rb(acc))
        if first:
            cps['wuk'].wait()
            relayout_k()
        qa = []
        for g in range(4):
            lhs = blockdiag([q[g]])
            qa.append(jnp.concatenate(
                [_dot(lhs, _ld(WKT, (g * 4 + cb,), 0, 1024)) for cb in range(NCB)], axis=1))
        qa = jnp.concatenate(qa, axis=0).astype(BF16)
        if first:
            for j in range(NCB):
                cps[f'ckv{j}'].wait()
            relayout_c()
            cps['g'].wait()
            relayout_f(g_v, GT)
            cps['u'].wait()
            relayout_f(u_v, UT)
        s = [_dot(qa, _ld(CT, (kb,), 0, DC)) for kb in range(NKB)]
        mx = s[0]
        for kb in range(1, NKB):
            mx = jnp.maximum(mx, s[kb])
        mx = jnp.max(mx, axis=1, keepdims=True)
        sc = D ** -0.5
        p = [jnp.exp((t - mx) * sc) for t in s]
        l = p[0]
        for kb in range(1, NKB):
            l = l + p[kb]
        l = jnp.sum(l, axis=1, keepdims=True)
        pb = jnp.concatenate([t.astype(BF16) for t in p], axis=1)
        cc = [_rb(_dot(pb, _ld(ckv_u, (cb,), 0, SK))) for cb in range(NCB)]
        if first:
            cps['wuv'].wait()
            relayout_v()
        inv = 1.0 / l
        ctx = []
        for g in range(4):
            lhs = blockdiag([c[g * 8:(g + 1) * 8] for c in cc])
            rhs = jnp.concatenate([_ld(WV, (g * 8 + j,), 0, DC) for j in range(8)], axis=0)
            ctx.append(_rb(_dot(lhs, rhs) * inv[g * 8:(g + 1) * 8]))
        if first:
            cps['wo'].wait()
        outs = []
        lhs = [blockdiag([ctx[g]]) for g in range(4)]
        lhs = jnp.concatenate(lhs, axis=1)
        for b in range(NB):
            r = _dot(lhs, wo_v[:, b * 128:(b + 1) * 128])
            outs.append(jnp.sum(r, axis=0, keepdims=True))
        out = jnp.concatenate(outs, axis=1)
        return jnp.broadcast_to(out, (8, M))

    def ffn(xn, first):
        xb = _rb(xn)
        if first:
            cps['wr'].wait()
        wr = wr_v[...].reshape(1, M).astype(F32)
        r = jnp.sum(xb * wr, axis=1, keepdims=True)
        sg = jax.nn.sigmoid(r)
        hs = []
        for fb in range(NFB):
            g = _dot(xb, _ld(GT, (fb,), 0, M))
            u = _dot(xb, _ld(UT, (fb,), 0, M))
            hs.append(_rb(g * jax.nn.sigmoid(g) * u))
        if first:
            cps['wd'].wait()
        ys = []
        hfull = jnp.concatenate(hs[:-1], axis=1)
        for b in range(NB):
            y = _dot(hfull, wd_v[pl.ds(0, FF - 64), b * 128:(b + 1) * 128])
            y = y + _dot(hs[-1][:, :64], wd_v[pl.ds(FF - 64, 64), b * 128:(b + 1) * 128])
            ys.append(y)
        y = jnp.concatenate(ys, axis=1)
        return xn + (xn * 0.0 + y * sg)

    cps['x'].wait()
    x = jnp.broadcast_to(x_v[0].astype(F32), (8, M))
    x = x + attn(_layernorm(x), True)
    x = x + ffn(_layernorm(x), True)
    x = x + attn(_layernorm(x), False)
    x = x + ffn(_layernorm(x), False)
    o_ref[0] = x[0:1].astype(BF16)


@jax.jit
def pallas_interleave_layers__compressed_kv_cla__moe_arch_mod__decode_kernel(
    A_x, A_c_kv, A_w_q, A_w_uk, A_w_uv, A_w_o, B_x, B_w_r, B_w_gate, B_w_up, B_w_down,
):
    hbm = pl.BlockSpec(memory_space=pltpu.HBM)
    vm = pltpu.VMEM
    return pl.pallas_call(
        _kernel,
        out_shape=jax.ShapeDtypeStruct((1, 1, M), BF16),
        in_specs=[hbm] * 10,
        scratch_shapes=[
            vm((1, 1, M), BF16), vm((M,), BF16),
            vm((M * H, D), BF16), vm((DC * H, D), BF16), vm((NCB, SK, 128), BF16),
            vm((DC * H, D), BF16), vm((H * D, M), BF16),
            vm((FF, M), BF16), vm((FF, M), BF16), vm((FF, M), BF16),
            vm((NB, H * 64, 128), U32), vm((16, 512, 128), U32), vm((NKB, DC // 2, 128), U32),
            vm((H, DC // 2, 128), U32), vm((NFB, M // 2, 128), U32), vm((NFB, M // 2, 128), U32),
            pltpu.SemaphoreType.DMA((16,)),
        ],
        compiler_params=pltpu.CompilerParams(vmem_limit_bytes=100 * 1024 * 1024),
        name="cla_moe_decode",
    )(A_x, A_w_q.reshape(M * H, D), A_w_uk.reshape(DC * H, D), A_c_kv.reshape(SK, DC),
      A_w_uv.reshape(DC * H, D), A_w_o.reshape(H * D, M), B_w_r, B_w_gate.T, B_w_up.T, B_w_down)
```

```python
import os
import jax
import numpy as np
import jax.numpy as jnp
import jax.experimental.pallas as pl
import jax.experimental.pallas.tpu as pltpu

F32 = jnp.float32
BF16 = jnp.bfloat16
U32 = jnp.uint32
U16 = jnp.uint16

M, H, D, SK, DC, FF = 640, 32, 128, 4096, 512, 1728
NB = M // 128
NCB = DC // 128
NKB = SK // 128
NFB = (FF + 127) // 128
EPS = 1e-5

E = os.environ.get
OPT_ONLINE = int(E('ONLINE', '1'))
OPT_LINQ = int(E('LINQ', '1'))
OPT_LINF = int(E('LINF', '1'))
STOP = E('STOP', '')
SCOPES = int(E('SCOPES', '0'))
WO_SPLIT = [int(t) for t in E('WOSPLIT', '24').split(',') if t]
WD_SPLIT = [int(t) for t in E('WDSPLIT', '2,4').split(',') if t]

N_SEM = 32


def _rb(x):
    return x.astype(BF16).astype(F32)


def _dot(a, b):
    return jax.lax.dot_general(a, b, (((1,), (0,)), ((), ())), preferred_element_type=F32)


def _cat(xs, axis):
    return xs[0] if len(xs) == 1 else jnp.concatenate(xs, axis=axis)


def _stats(parts):
    s = parts[0]
    for p in parts[1:]:
        s = s + p
    m = jnp.sum(s, axis=1, keepdims=True) * (1.0 / M)
    c = [p - m for p in parts]
    v = c[0] * c[0]
    for p in c[1:]:
        v = v + p * p
    v = jnp.sum(v, axis=1, keepdims=True) * (1.0 / M)
    return m, jax.lax.rsqrt(v + EPS)


def _ln(parts):
    m, r = _stats(parts)
    return [(p - m) * r for p in parts]


class _Scope:
    def __init__(self, name):
        self.c = jax.named_scope(name) if SCOPES else None
    def __enter__(self):
        if self.c: self.c.__enter__()
    def __exit__(self, *a):
        if self.c: self.c.__exit__(*a)


def _kernel(x_hbm, wq_hbm, wuk_hbm, ckv_hbm, wuv_hbm, wo_hbm, wr_hbm, g_hbm, u_hbm, wd_hbm,
            o_ref,
            x_v, wr_v, wq_v, wuk_v, ckv_v, wuv_v, wo_v, g_v, u_v, wd_v,
            WQ, WKT, CT, WV, GT, UT, sems):
    cps = {}
    n = [0]

    def add(name, src, dst):
        cps[name] = pltpu.make_async_copy(src, dst, sems.at[n[0]])
        n[0] += 1

    add('wq', wq_hbm, wq_v)
    add('x', x_hbm, x_v)
    add('wr', wr_hbm, wr_v)
    add('wuk', wuk_hbm, wuk_v)
    for j in range(NCB):
        add(f'ckv{j}', ckv_hbm.at[:, pl.ds(128 * j, 128)], ckv_v.at[j])
    add('g', g_hbm, g_v)
    add('u', u_hbm, u_v)
    add('wuv', wuv_hbm, wuv_v)
    wo_b = [0] + WO_SPLIT + [H]
    for i in range(len(wo_b) - 1):
        sl = pl.ds(wo_b[i] * D, (wo_b[i + 1] - wo_b[i]) * D)
        add(f'wo{i}', wo_hbm.at[sl], wo_v.at[sl])
    wd_b = [0] + WD_SPLIT + [NB]
    for i in range(len(wd_b) - 1):
        sl = pl.ds(wd_b[i] * 128, (wd_b[i + 1] - wd_b[i]) * 128)
        add(f'wd{i}', wd_hbm.at[:, sl], wd_v.at[:, sl])
    assert n[0] <= N_SEM
    for c in cps.values():
        c.start()
    waited = set()

    def wait(name):
        if name not in waited:
            cps[name].wait()
            waited.add(name)

    wq_u, wuk_u, wuv_u, ckv_u = (r.bitcast(U32) for r in (wq_v, wuk_v, wuv_v, ckv_v))

    def ld(uref, idx, r0, nrows):
        return pltpu.bitcast(uref[(*idx, pl.ds(r0 // 2, nrows // 2), slice(None))], BF16)

    def shuf(src_u, r0, s):
        a = src_u[pl.ds(r0 * 16 + s, 8, stride=16), :]
        b = src_u[pl.ds((r0 + 8) * 16 + s, 8, stride=16), :]
        xx = jnp.concatenate([a, b], axis=0)
        lo = pltpu.bitcast(xx.astype(U16), U32)
        hi = pltpu.bitcast((xx >> 16).astype(U16), U32)
        return lo, hi

    def relayout_q():
        for i in range(M // 16):
            b, m16 = divmod(i, 8)
            for s in range(16):
                lo, hi = shuf(wq_u, i * 16, s)
                WQ[b, pl.ds(2 * s * 64 + m16 * 8, 8), :] = lo
                WQ[b, pl.ds((2 * s + 1) * 64 + m16 * 8, 8), :] = hi

    def relayout_v():
        for i in range(DC // 16):
            for s in range(16):
                lo, hi = shuf(wuv_u, i * 16, s)
                WV[2 * s, pl.ds(i * 8, 8), :] = lo
                WV[2 * s + 1, pl.ds(i * 8, 8), :] = hi

    def relayout_k():
        for cb in range(NCB):
            for s in range(16):
                los, his = [], []
                for i in range(8):
                    lo, hi = shuf(wuk_u, cb * 128 + i * 16, s)
                    los.append(lo)
                    his.append(hi)
                for h, parts in ((2 * s, los), (2 * s + 1, his)):
                    t = pltpu.bitcast(jnp.concatenate(parts, axis=0), BF16).T
                    WKT[(h // 8) * 4 + cb, pl.ds((h % 8) * 64, 64), :] = pltpu.bitcast(t, U32)

    def relayout_c():
        for cb in range(NCB):
            wait(f'ckv{cb}')
            for kb in range(NKB):
                t = ld(ckv_u, (cb,), kb * 128, 128).T
                CT[kb, pl.ds(cb * 64, 64), :] = pltpu.bitcast(t, U32)

    def relayout_f(src, dst):
        for fb in range(NFB):
            for b in range(NB):
                if fb < NFB - 1:
                    t = src[pl.ds(fb * 128, 128), pl.ds(b * 128, 128)]
                else:
                    t = src[pl.ds(fb * 128, 64), pl.ds(b * 128, 128)]
                    t = jnp.concatenate([t, jnp.zeros((64, 128), BF16)], axis=0)
                dst[fb, pl.ds(b * 64, 64), :] = pltpu.bitcast(t.T, U32)

    row8 = jax.lax.broadcasted_iota(jnp.int32, (8, 128), 0)

    def bd(parts):
        return jnp.concatenate(
            [jnp.where(row8 == j, p, 0.0) for j in range(8) for p in parts], axis=1)

    ones8 = jnp.ones((8, 128), F32)
    scale = D ** -0.5

    def q_block(xb, b, with_ones=False):
        lhs = bd([xb])
        if with_ones:
            lhs = jnp.concatenate([lhs, bd([ones8])], axis=0)
        return [_dot(lhs, ld(WQ, (b,), g * 1024, 1024)) for g in range(4)]

    def acc_list(a, b):
        return b if a is None else [x + y for x, y in zip(a, b)]

    def softmax_ctx(qa, first):
        nblk = 2 if OPT_ONLINE else 1
        per = NKB // nblk
        ss = []
        for blk in range(nblk):
            ss.append([_dot(qa, ld(CT, (kb,), 0, DC)) for kb in range(blk * per, (blk + 1) * per)])
        m_run = l_run = acc = None
        for blk in range(nblk):
            s = ss[blk]
            mx = s[0]
            for t in s[1:]:
                mx = jnp.maximum(mx, t)
            mx = jnp.max(mx, axis=1, keepdims=True)
            if m_run is not None:
                mx = jnp.maximum(mx, m_run)
            p = [jnp.exp((t - mx) * scale) for t in s]
            l = p[0]
            for t in p[1:]:
                l = l + t
            pb = jnp.concatenate([t.astype(BF16) for t in p], axis=1)
            cc = [_dot(pb, ld(ckv_u, (cb,), blk * per * 128, per * 128)) for cb in range(NCB)]
            if m_run is not None:
                al = jnp.exp((m_run - mx) * scale)
                cc = [c + a * al for c, a in zip(cc, acc)]
                l = l + l_run * al
            m_run, l_run, acc = mx, l, cc
        lsum = jnp.sum(l_run, axis=1, keepdims=True)
        return [_rb(c) for c in acc], 1.0 / lsum

    def attn_rest(q, first):
        if first:
            wait('wuk')
            with _Scope('relayout_k'):
                relayout_k()
        qa = []
        for g in range(4):
            lhs = bd([q[g]])
            qa.append(jnp.concatenate(
                [_dot(lhs, ld(WKT, (g * 4 + cb,), 0, 1024)) for cb in range(NCB)], axis=1))
        qa = jnp.concatenate(qa, axis=0).astype(BF16)
        if first:
            with _Scope('relayout_c'):
                relayout_c()
        cc, inv = softmax_ctx(qa, first)
        if first:
            wait('g')
            with _Scope('relayout_g'):
                relayout_f(g_v, GT)
            wait('u')
            with _Scope('relayout_u'):
                relayout_f(u_v, UT)
            wait('wuv')
            with _Scope('relayout_v'):
                relayout_v()
        ctx = []
        for g in range(4):
            lhs = bd([c[g * 8:(g + 1) * 8] for c in cc])
            rhs = jnp.concatenate([ld(WV, (g * 8 + j,), 0, DC) for j in range(8)], axis=0)
            ctx.append(_rb(_dot(lhs, rhs) * inv[g * 8:(g + 1) * 8]))
        outs = [None] * NB
        for i in range(len(wo_b) - 1):
            if first:
                wait(f'wo{i}')
            g0, g1 = wo_b[i] // 8, wo_b[i + 1] // 8
            lhs = jnp.concatenate([bd([ctx[g]]) for g in range(g0, g1)], axis=1)
            for b in range(NB):
                r = _dot(lhs, wo_v[pl.ds(g0 * 1024, (g1 - g0) * 1024), pl.ds(b * 128, 128)])
                outs[b] = r if outs[b] is None else outs[b] + r
        return [jnp.broadcast_to(jnp.sum(r, axis=0, keepdims=True), (8, 128)) for r in outs]

    def router(xn):
        wait('wr')
        wr = wr_v[...].reshape(1, M).astype(F32)
        r = None
        for b in range(NB):
            t = _rb(xn[b]) * wr[:, b * 128:(b + 1) * 128]
            r = t if r is None else r + t
        return jax.nn.sigmoid(jnp.sum(r, axis=1, keepdims=True))

    def down_block(hs, b):
        y = _dot(jnp.concatenate(hs[:-1], axis=1), wd_v[pl.ds(0, FF - 64), pl.ds(b * 128, 128)])
        return y + _dot(hs[-1][:, :64], wd_v[pl.ds(FF - 64, 64), pl.ds(b * 128, 128)])

    def finish(x):
        o_ref[0] = jnp.concatenate([p[0:1] for p in x], axis=1).astype(BF16)
        for name in cps:
            wait(name)

    with _Scope('p1_start'):
        wait('x')
        x0 = jnp.broadcast_to(x_v[0].astype(F32), (8, M))
        x0 = [x0[:, b * 128:(b + 1) * 128] for b in range(NB)]
        xn = _ln(x0)
        wait('wq')
    with _Scope('relayout_q'):
        relayout_q()
    with _Scope('A1'):
        q = None
        for b in range(NB):
            q = acc_list(q, q_block(_rb(xn[b]), b, with_ones=bool(OPT_LINQ)))
        if OPT_LINQ:
            cs = [t[8:16] for t in q]
            q = [t[0:8] for t in q]
        q = [_rb(t) for t in q]
        out = attn_rest(q, True)
        x1 = [a + b for a, b in zip(x0, out)]
    if STOP == 'A1':
        return finish(x1)
    with _Scope('B1'):
        xn1 = _ln(x1)
        sg = router(xn1)
        lhs = jnp.concatenate([_rb(t) for t in xn1], axis=1)
        if OPT_LINF:
            lhs = jnp.concatenate([lhs, jnp.ones((8, M), F32)], axis=0)
        hs, cg, cu = [], [], []
        for fb in range(NFB):
            g = _dot(lhs, ld(GT, (fb,), 0, M))
            u = _dot(lhs, ld(UT, (fb,), 0, M))
            if OPT_LINF:
                cg.append(g[8:16]); cu.append(u[8:16])
                g, u = g[0:8], u[0:8]
            hs.append(_rb(g * jax.nn.sigmoid(g) * u))
        base = [a + b for a, b in zip(x1, xn1)]
        x2 = [None] * NB
        if OPT_LINQ:
            qraw = None
            pivot = None
            xp = [None] * NB
            for i in range(len(wd_b) - 1):
                wait(f'wd{i}')
                blks = list(range(wd_b[i], wd_b[i + 1]))
                with _Scope(f'wd{i}'):
                    for b in blks:
                        x2[b] = base[b] + (xn1[b] * 0.0 + down_block(hs, b) * sg)
                    if pivot is None:
                        s = x2[blks[0]]
                        for b in blks[1:]:
                            s = s + x2[b]
                        pivot = jnp.sum(s, axis=1, keepdims=True) * (1.0 / (128 * len(blks)))
                    for b in blks:
                        xp[b] = x2[b] - pivot
                        qraw = acc_list(qraw, q_block(_rb(xp[b]), b))
        else:
            for i in range(len(wd_b) - 1):
                wait(f'wd{i}')
            for b in range(NB):
                x2[b] = base[b] + (xn1[b] * 0.0 + down_block(hs, b) * sg)
    if STOP == 'B1':
        return finish(x2)
    with _Scope('A2'):
        if OPT_LINQ:
            mu, rs = _stats(xp)
            q = [_rb((t - mu * c) * rs) for t, c in zip(qraw, cs)]
        else:
            xn = _ln(x2)
            q = None
            for b in range(NB):
                q = acc_list(q, q_block(_rb(xn[b]), b))
            q = [_rb(t) for t in q]
        out = attn_rest(q, False)
        x3 = [a + b for a, b in zip(x2, out)]
    with _Scope('B2'):
        if OPT_LINF:
            if OPT_LINQ:
                x3p = [a + b for a, b in zip(xp, out)]
            else:
                pv = jnp.sum(x2[0], axis=1, keepdims=True) * (1.0 / 128)
                x3p = [a - pv for a in x3]
            lhs = jnp.concatenate([_rb(t) for t in x3p], axis=1)
            mu, rs = _stats(x3p)
            xn3 = [(t - mu) * rs for t in x3p]
        else:
            xn3 = _ln(x3)
            lhs = jnp.concatenate([_rb(t) for t in xn3], axis=1)
        sg = router(xn3)
        hs = []
        for fb in range(NFB):
            g = _dot(lhs, ld(GT, (fb,), 0, M))
            u = _dot(lhs, ld(UT, (fb,), 0, M))
            if OPT_LINF:
                g = (g - mu * cg[fb]) * rs
                u = (u - mu * cu[fb]) * rs
            hs.append(_rb(g * jax.nn.sigmoid(g) * u))
        x4 = [x3[b] + (xn3[b] + (xn3[b] * 0.0 + down_block(hs, b) * sg)) for b in range(NB)]
    finish(x4)


@jax.jit
def pallas_interleave_layers__compressed_kv_cla__moe_arch_mod__decode_kernel(
    A_x, A_c_kv, A_w_q, A_w_uk, A_w_uv, A_w_o, B_x, B_w_r, B_w_gate, B_w_up, B_w_down,
):
    hbm = pl.BlockSpec(memory_space=pltpu.HBM)
    vm = pltpu.VMEM
    return pl.pallas_call(
        _kernel,
        out_shape=jax.ShapeDtypeStruct((1, 1, M), BF16),
        in_specs=[hbm] * 10,
        scratch_shapes=[
            vm((1, 1, M), BF16), vm((M,), BF16),
            vm((M * H, D), BF16), vm((DC * H, D), BF16), vm((NCB, SK, 128), BF16),
            vm((DC * H, D), BF16), vm((H * D, M), BF16),
            vm((FF, M), BF16), vm((FF, M), BF16), vm((FF, M), BF16),
            vm((NB, H * 64, 128), U32), vm((16, 512, 128), U32), vm((NKB, DC // 2, 128), U32),
            vm((H, DC // 2, 128), U32), vm((NFB, M // 2, 128), U32), vm((NFB, M // 2, 128), U32),
            pltpu.SemaphoreType.DMA((N_SEM,)),
        ],
        compiler_params=pltpu.CompilerParams(vmem_limit_bytes=100 * 1024 * 1024),
        name="cla_moe_decode",
    )(A_x, A_w_q.reshape(M * H, D), A_w_uk.reshape(DC * H, D), A_c_kv.reshape(SK, DC),
      A_w_uv.reshape(DC * H, D), A_w_o.reshape(H * D, M), B_w_r, B_w_gate.T, B_w_up.T, B_w_down)
```

```python
import os
import jax
import numpy as np
import jax.numpy as jnp
import jax.experimental.pallas as pl
import jax.experimental.pallas.tpu as pltpu

F32 = jnp.float32
BF16 = jnp.bfloat16
U32 = jnp.uint32
U16 = jnp.uint16

M, H, D, SK, DC, FF = 640, 32, 128, 4096, 512, 1728
NB = M // 128
NCB = DC // 128
NKB = SK // 128
NFB = (FF + 127) // 128
EPS = 1e-5

E = os.environ.get
OPT_ONLINE = int(E('ONLINE', '1'))
OPT_LINQ = int(E('LINQ', '1'))
OPT_LINF = int(E('LINF', '1'))
STOP = E('STOP', '')
SCOPES = int(E('SCOPES', '0'))
WO_SPLIT = [int(t) for t in E('WOSPLIT', '24').split(',') if t]
WD_SPLIT = [int(t) for t in E('WDSPLIT', '2,4').split(',') if t]

NF0 = int(E('NF0', '3'))
QDEF = int(E('QDEF', '1'))
NV = int(E('NV', '0'))
HV = int(E('HV', '13'))
LAG = int(E('LAG', '4'))
ANCH = int(E('ANCH', '1'))
AOFF = int(E('AOFF', '4'))
BACK = int(E('BACK', '2'))
PINS = int(E('PINS', '1'))
N_SEM = int(E('NSEM', '16'))


def _rb(x):
    return x.astype(BF16).astype(F32)


def _dot(a, b):
    return jax.lax.dot_general(a, b, (((1,), (0,)), ((), ())), preferred_element_type=F32)


def _cat(xs, axis):
    return xs[0] if len(xs) == 1 else jnp.concatenate(xs, axis=axis)


def _stats(parts):
    s = parts[0]
    for p in parts[1:]:
        s = s + p
    m = jnp.sum(s, axis=1, keepdims=True) * (1.0 / M)
    c = [p - m for p in parts]
    v = c[0] * c[0]
    for p in c[1:]:
        v = v + p * p
    v = jnp.sum(v, axis=1, keepdims=True) * (1.0 / M)
    return m, jax.lax.rsqrt(v + EPS)


def _ln(parts):
    m, r = _stats(parts)
    return [(p - m) * r for p in parts]


class _Scope:
    def __init__(self, name):
        self.c = jax.named_scope(name) if SCOPES else None
    def __enter__(self):
        if self.c: self.c.__enter__()
    def __exit__(self, *a):
        if self.c: self.c.__exit__(*a)


def _kernel(x_hbm, wq_hbm, wuk_hbm, ckv_hbm, wuv_hbm, wo_hbm, wr_hbm, g_hbm, u_hbm, wd_hbm,
            o_ref,
            x_v, wr_v, wq_v, wuk_v, ckv_v, wuv_v, wo_v, g_v, u_v, wd_v,
            WQ, WKT, CT, WV, GT, UT, WVT, WO32, WOT, PIN, sems):
    cps = {}
    n = [0]

    def add(name, src, dst):
        cps[name] = pltpu.make_async_copy(src, dst, sems.at[n[0]])
        n[0] += 1

    add('wq', wq_hbm, wq_v)
    add('x', x_hbm, x_v)
    add('wr', wr_hbm, wr_v)
    add('wuk', wuk_hbm, wuk_v)
    for j in range(NCB):
        add(f'ckv{j}', ckv_hbm.at[:, pl.ds(128 * j, 128)], ckv_v.at[j])
    add('g', g_hbm, g_v)
    add('u', u_hbm, u_v)
    add('wuv', wuv_hbm, wuv_v)
    wo_b = [0] + WO_SPLIT + [H]
    for i in range(len(wo_b) - 1):
        sl = pl.ds(wo_b[i] * D, (wo_b[i + 1] - wo_b[i]) * D)
        add(f'wo{i}', wo_hbm.at[sl], wo_v.at[sl])
    wd_b = [0] + WD_SPLIT + [NB]
    for i in range(len(wd_b) - 1):
        sl = pl.ds(wd_b[i] * 128, (wd_b[i + 1] - wd_b[i]) * 128)
        add(f'wd{i}', wd_hbm.at[:, sl], wd_v.at[:, sl])
    assert n[0] <= N_SEM
    for c in cps.values():
        c.start()
    waited = set()

    def wait(name):
        if name not in waited:
            cps[name].wait()
            waited.add(name)

    wq_u, wuk_u, wuv_u, ckv_u = (r.bitcast(U32) for r in (wq_v, wuk_v, wuv_v, ckv_v))

    pin_n = [0]

    def pin(vals, *names):
        if not PINS:
            for nm in names:
                wait(nm)
            return vals
        k0 = pin_n[0]
        for i, v in enumerate(vals):
            PIN[k0 + i] = v
        pin_n[0] += len(vals)
        for nm in names:
            wait(nm)
        return [PIN[k0 + i] for i in range(len(vals))]

    def ld(uref, idx, r0, nrows):
        return pltpu.bitcast(uref[(*idx, pl.ds(r0 // 2, nrows // 2), slice(None))], BF16)

    def shuf(src_u, r0, s):
        a = src_u[pl.ds(r0 * 16 + s, 8, stride=16), :]
        b = src_u[pl.ds((r0 + 8) * 16 + s, 8, stride=16), :]
        xx = jnp.concatenate([a, b], axis=0)
        lo = pltpu.bitcast(xx.astype(U16), U32)
        hi = pltpu.bitcast((xx >> 16).astype(U16), U32)
        return lo, hi

    def relayout_q():
        for i in range(M // 16):
            b, m16 = divmod(i, 8)
            for s in range(16):
                lo, hi = shuf(wq_u, i * 16, s)
                WQ[b, pl.ds(2 * s * 64 + m16 * 8, 8), :] = lo
                WQ[b, pl.ds((2 * s + 1) * 64 + m16 * 8, 8), :] = hi

    def relayout_v():
        for i in range(DC // 16):
            for s in range(16):
                lo, hi = shuf(wuv_u, i * 16, s)
                WV[2 * s, pl.ds(i * 8, 8), :] = lo
                WV[2 * s + 1, pl.ds(i * 8, 8), :] = hi
        for h in range(HV):
            for cb in range(NCB):
                WVT[h * NCB + cb] = ld(WV, (h,), cb * 128, 128).T.astype(F32)

    def relayout_o(h0, h1):
        for h in range(h0, h1):
            if h < HV:
                for i in range(16):
                    WO32[pl.ds(h * D + i * 8, 8), :] = wo_v[pl.ds(h * D + i * 8, 8), :].astype(F32)
            else:
                for b in range(NB):
                    WOT[b, pl.ds(h * 64, 64), :] = pltpu.bitcast(
                        wo_v[pl.ds(h * D, D), pl.ds(b * 128, 128)], U32)

    def relayout_k():
        for cb in range(NCB):
            for s in range(16):
                los, his = [], []
                for i in range(8):
                    lo, hi = shuf(wuk_u, cb * 128 + i * 16, s)
                    los.append(lo)
                    his.append(hi)
                for h, parts in ((2 * s, los), (2 * s + 1, his)):
                    t = pltpu.bitcast(jnp.concatenate(parts, axis=0), BF16).T
                    WKT[(h // 8) * 4 + cb, pl.ds((h % 8) * 64, 64), :] = pltpu.bitcast(t, U32)

    def relayout_c():
        for cb in range(NCB):
            wait(f'ckv{cb}')
            for kb in range(NKB):
                t = ld(ckv_u, (cb,), kb * 128, 128).T
                CT[kb, pl.ds(cb * 64, 64), :] = pltpu.bitcast(t, U32)

    def relayout_f(src, dst):
        for fb in range(NFB):
            for b in range(NB):
                if fb < NFB - 1:
                    t = src[pl.ds(fb * 128, 128), pl.ds(b * 128, 128)]
                else:
                    t = src[pl.ds(fb * 128, 64), pl.ds(b * 128, 128)]
                    t = jnp.concatenate([t, jnp.zeros((64, 128), BF16)], axis=0)
                dst[fb, pl.ds(b * 64, 64), :] = pltpu.bitcast(t.T, U32)

    row8 = jax.lax.broadcasted_iota(jnp.int32, (8, 128), 0)

    def bd(parts):
        return jnp.concatenate(
            [jnp.where(row8 == j, p, 0.0) for j in range(8) for p in parts], axis=1)

    ones8 = jnp.ones((8, 128), F32)
    scale = D ** -0.5

    def q_block(xb, b, with_ones=False):
        lhs = bd([xb])
        if with_ones:
            lhs = jnp.concatenate([lhs, bd([ones8])], axis=0)
        return [_dot(lhs, ld(WQ, (b,), g * 1024, 1024)) for g in range(4)]

    def q_tile(xb, b, g):
        return _dot(bd([xb]), ld(WQ, (b,), g * 1024, 1024))

    def acc_list(a, b):
        return b if a is None else [x + y for x, y in zip(a, b)]

    def softmax_ctx(qa, first):
        nblk = 2 if OPT_ONLINE else 1
        per = NKB // nblk
        ss = []
        for blk in range(nblk):
            ss.append([_dot(qa, ld(CT, (kb,), 0, DC)) for kb in range(blk * per, (blk + 1) * per)])
        m_run = l_run = acc = None
        for blk in range(nblk):
            s = ss[blk]
            mx = s[0]
            for t in s[1:]:
                mx = jnp.maximum(mx, t)
            mx = jnp.max(mx, axis=1, keepdims=True)
            if m_run is not None:
                mx = jnp.maximum(mx, m_run)
            p = [jnp.exp((t - mx) * scale) for t in s]
            l = p[0]
            for t in p[1:]:
                l = l + t
            pb = jnp.concatenate([t.astype(BF16) for t in p], axis=1)
            cc = [_dot(pb, ld(ckv_u, (cb,), blk * per * 128, per * 128)) for cb in range(NCB)]
            if m_run is not None:
                al = jnp.exp((m_run - mx) * scale)
                cc = [c + a * al for c, a in zip(cc, acc)]
                l = l + l_run * al
            m_run, l_run, acc = mx, l, cc
        lsum = jnp.sum(l_run, axis=1, keepdims=True)
        return [_rb(c) for c in acc], 1.0 / lsum

    def attn_rest(q, first):
        if first:
            with _Scope('relayout_k'):
                relayout_k()
        qa = []
        for g in range(4):
            lhs = bd([q[g]])
            qa.append(jnp.concatenate(
                [_dot(lhs, ld(WKT, (g * 4 + cb,), 0, 1024)) for cb in range(NCB)], axis=1))
        if first:
            t = pin([x[:, cb * 128:(cb + 1) * 128] for x in qa for cb in range(NCB)], 'ckv0')
            qa = [jnp.concatenate(t[g * 4:(g + 1) * 4], axis=1) for g in range(4)]
        qa = jnp.concatenate(qa, axis=0).astype(BF16)
        if first:
            with _Scope('relayout_c'):
                relayout_c()
        cc, inv = softmax_ctx(qa, first)
        if first:
            t = pin([c[g * 8:(g + 1) * 8] for c in cc for g in range(4)]
                    + [jnp.broadcast_to(inv, (H, 128))[g * 8:(g + 1) * 8] for g in range(4)], 'g')
            cc = [jnp.concatenate(t[cb * 4:(cb + 1) * 4], axis=0) for cb in range(NCB)]
            inv = jnp.concatenate(t[16:20], axis=0)
            with _Scope('relayout_g'):
                relayout_f(g_v, GT)
            wait('u')
            with _Scope('relayout_u'):
                relayout_f(u_v, UT)
            wait('wuv')
            with _Scope('relayout_v'):
                relayout_v()
        if first or HV == 0:
            ctx = []
            for g in range(4):
                lhs = bd([c[g * 8:(g + 1) * 8] for c in cc])
                rhs = jnp.concatenate([ld(WV, (g * 8 + j,), 0, DC) for j in range(8)], axis=0)
                ctx.append(_rb(_dot(lhs, rhs) * inv[g * 8:(g + 1) * 8]))
            outs = [None] * NB
            wob = wo_b if first else [0, H]
            for i in range(len(wob) - 1):
                if first:
                    t = pin(ctx + [o for o in outs if o is not None] if i == 0 else outs, f'wo{i}')
                    if i == 0:
                        ctx = t[:4]
                    else:
                        outs = t
                g0, g1 = wob[i] // 8, wob[i + 1] // 8
                lhs = jnp.concatenate([bd([ctx[g]]) for g in range(g0, g1)], axis=1)
                for b in range(NB):
                    r = _dot(lhs, wo_v[pl.ds(g0 * 1024, (g1 - g0) * 1024), pl.ds(b * 128, 128)])
                    outs[b] = r if outs[b] is None else outs[b] + r
                if first and HV:
                    relayout_o(wob[i], wob[i + 1])
        else:
            outs = attn_tail_mixed(cc, inv)
        return [jnp.broadcast_to(jnp.sum(r, axis=0, keepdims=True), (8, 128)) for r in outs]

    def attn_tail_mixed(cc, inv):
        accv = [None] * NB
        invb = jnp.broadcast_to(inv, (H, 128))
        true_mask = invb[0:8] > -1.0
        zhist = []
        cn = [[cc[cb][g * 8:(g + 1) * 8] * invb[g * 8:(g + 1) * 8] for cb in range(NCB)]
              for g in range((HV + 7) // 8)]

        def vpu_head(h):
            xr = [jnp.broadcast_to(cn[h // 8][cb][h % 8:h % 8 + 1], (8, 128)) for cb in range(NCB)]
            if BACK and h >= BACK:
                xr = [jnp.where(true_mask, t, zhist[h - BACK]) for t in xr]
            for i in range(16):
                a = None
                for cb in range(NCB):
                    t = WVT[h * NCB + cb, pl.ds(i * 8, 8), :] * xr[cb]
                    a = t if a is None else a + t
                cv = jnp.broadcast_to(jnp.sum(a, axis=1, keepdims=True), (8, 128))
                for b in range(NB):
                    t = WO32[pl.ds(h * D + i * 8, 8), pl.ds(b * 128, 128)] * cv
                    accv[b] = t if accv[b] is None else accv[b] + t
            if BACK:
                z = accv[0]
                for b in range(1, NB):
                    z = jnp.maximum(z, accv[b])
                zhist.append(z)

        for h in range(HV):
            vpu_head(h)
        ctx = {}
        for g in range(HV // 8, 4):
            acc = None
            for h in range(max(HV, g * 8), g * 8 + 8):
                for cb in range(NCB):
                    lhs = jnp.where(row8 == h % 8, cc[cb][g * 8:(g + 1) * 8], 0.0)
                    t = _dot(lhs, ld(WV, (h,), cb * 128, 128))
                    acc = t if acc is None else acc + t
            ctx[g] = _rb(acc * invb[g * 8:(g + 1) * 8])
        outs = []
        lhs = {h: jnp.where(row8 == (h % 8), ctx[h // 8], 0.0) for h in range(HV, H)}
        for b in range(NB):
            acc = accv[b]
            for h in range(HV, H):
                acc = acc + _dot(lhs[h], ld(WOT, (b,), h * 128, 128))
            outs.append(acc)
        return outs

    def router(xn):
        wr = wr_v[...].reshape(1, M).astype(F32)
        r = None
        for b in range(NB):
            t = _rb(xn[b]) * wr[:, b * 128:(b + 1) * 128]
            r = t if r is None else r + t
        return jax.nn.sigmoid(jnp.sum(r, axis=1, keepdims=True))

    def down_block(hs, b):
        y = _dot(jnp.concatenate(hs[:-1], axis=1), wd_v[pl.ds(0, FF - 64), pl.ds(b * 128, 128)])
        return y + _dot(hs[-1][:, :64], wd_v[pl.ds(FF - 64, 64), pl.ds(b * 128, 128)])

    def finish(x):
        o_ref[0] = jnp.concatenate([p[0:1] for p in x], axis=1).astype(BF16)
        for name in cps:
            wait(name)

    with _Scope('p1_start'):
        wait('x')
        wait('wr')
        x0 = jnp.broadcast_to(x_v[0].astype(F32), (8, M))
        x0 = [x0[:, b * 128:(b + 1) * 128] for b in range(NB)]
        xn = _ln(x0)
        wait('wq')
    with _Scope('relayout_q'):
        relayout_q()
    with _Scope('A1'):
        q = None
        for b in range(NB):
            q = acc_list(q, q_block(_rb(xn[b]), b, with_ones=bool(OPT_LINQ)))
        if OPT_LINQ:
            cs = [t[8:16] for t in q]
            q = [t[0:8] for t in q]
        q = [_rb(t) for t in q]
        t = pin(q + cs, 'wuk')
        q, cs = t[:4], t[4:]
        t = pin(x0)
        x0 = t
        out = attn_rest(q, True)
        x1 = [a + b for a, b in zip(x0, out)]
    if STOP == 'A1':
        return finish(x1)
    with _Scope('B1'):
        xn1 = _ln(x1)
        sg = router(xn1)
        lhs = jnp.concatenate([_rb(t) for t in xn1], axis=1)
        if OPT_LINF:
            lhs = jnp.concatenate([lhs, jnp.ones((8, M), F32)], axis=0)
        hs, cg, cu = [], [], []
        for fb in range(NFB):
            g = _dot(lhs, ld(GT, (fb,), 0, M))
            u = _dot(lhs, ld(UT, (fb,), 0, M))
            if OPT_LINF:
                cg.append(g[8:16]); cu.append(u[8:16])
                g, u = g[0:8], u[0:8]
            hs.append(_rb(g * jax.nn.sigmoid(g) * u))
        base = [a + b for a, b in zip(x1, xn1)]
        x2 = [None] * NB
        if OPT_LINQ:
            qraw = [None] * 4
            deferred = []
            pivot = None
            xp = [None] * NB
            for i in range(len(wd_b) - 1):
                if i == 0:
                    t = pin(hs + base + xn1 + [jnp.broadcast_to(sg, (8, 128))] + cg + cu, 'wd0')
                    hs, base, xn1, sg = t[:NFB], t[NFB:NFB + 5], t[NFB + 5:NFB + 10], t[NFB + 10]
                    cg, cu = t[NFB + 11:2 * NFB + 11], t[2 * NFB + 11:]
                else:
                    done = [b for b in range(NB) if x2[b] is not None]
                    t = pin(qraw + [x2[b] for b in done] + [xp[b] for b in done]
                            + [jnp.broadcast_to(pivot, (8, 128))], f'wd{i}')
                    qraw = t[:4]
                    for n_, b in enumerate(done):
                        x2[b] = t[4 + n_]
                        xp[b] = t[4 + len(done) + n_]
                    pivot = t[-1]
                blks = list(range(wd_b[i], wd_b[i + 1]))
                with _Scope(f'wd{i}'):
                    for b in blks:
                        x2[b] = base[b] + (xn1[b] * 0.0 + down_block(hs, b) * sg)
                    if pivot is None:
                        s = x2[blks[0]]
                        for b in blks[1:]:
                            s = s + x2[b]
                        pivot = jnp.sum(s, axis=1, keepdims=True) * (1.0 / (128 * len(blks)))
                    for b in blks:
                        xp[b] = x2[b] - pivot
                    last = i == len(wd_b) - 2
                    for (bb, g) in deferred:
                        qraw[g] = qraw[g] + q_tile(_rb(xp[bb]), bb, g)
                    deferred = []
                    todo = [(b, g) for b in blks for g in range(4)]
                    if i == len(wd_b) - 3 and QDEF:
                        todo, deferred = todo[:-QDEF], todo[-QDEF:]
                    for (bb, g) in todo:
                        t = q_tile(_rb(xp[bb]), bb, g)
                        qraw[g] = t if qraw[g] is None else qraw[g] + t
        else:
            for i in range(len(wd_b) - 1):
                wait(f'wd{i}')
            for b in range(NB):
                x2[b] = base[b] + (xn1[b] * 0.0 + down_block(hs, b) * sg)
    if STOP == 'B1':
        return finish(x2)
    with _Scope('A2'):
        if OPT_LINQ:
            mu, rs = _stats(xp)
            q = [_rb((t - mu * c) * rs) for t, c in zip(qraw, cs)]
        else:
            xn = _ln(x2)
            q = None
            for b in range(NB):
                q = acc_list(q, q_block(_rb(xn[b]), b))
            q = [_rb(t) for t in q]
        out = attn_rest(q, False)
        x3 = [a + b for a, b in zip(x2, out)]
    with _Scope('B2'):
        if OPT_LINF:
            if OPT_LINQ:
                x3p = [a + b for a, b in zip(xp, out)]
            else:
                pv = jnp.sum(x2[0], axis=1, keepdims=True) * (1.0 / 128)
                x3p = [a - pv for a in x3]
            lhs = jnp.concatenate([_rb(t) for t in x3p], axis=1)
            mu, rs = _stats(x3p)
            xn3 = [(t - mu) * rs for t in x3p]
        else:
            xn3 = _ln(x3)
            lhs = jnp.concatenate([_rb(t) for t in xn3], axis=1)
        sg = router(xn3)
        xb3 = [lhs[:, b * 128:(b + 1) * 128] for b in range(NB)]
        gs, us = [None] * NFB, [None] * NFB

        def gu_tile(fb, b):
            g = _dot(xb3[b], ld(GT, (fb,), b * 128, 128))
            u = _dot(xb3[b], ld(UT, (fb,), b * 128, 128))
            gs[fb] = g if gs[fb] is None else gs[fb] + g
            us[fb] = u if us[fb] is None else us[fb] + u

        for b in range(NB):
            for fb in range(NF0):
                gu_tile(fb, b)
        hs = []
        hcs = {}
        accv = [None] * NB

        def vpu_down(fb, i0, i1):
            if fb not in hcs:
                hcs[fb] = jnp.broadcast_to(hs[fb][0:1], (128, 128)).T
            for i in range(i0, i1):
                wf = wd_v[pl.ds(fb * 128 + i * 8, 8), :].astype(F32)
                hv = hcs[fb][i * 8:(i + 1) * 8]
                for b in range(NB):
                    t = wf[:, b * 128:(b + 1) * 128] * hv
                    accv[b] = t if accv[b] is None else accv[b] + t

        for fb in range(NFB):
            v = fb - LAG
            if fb >= NF0:
                gs[fb] = None
                for b in range(NB):
                    t = _dot(xb3[b], ld(GT, (fb,), b * 128, 128))
                    gs[fb] = t if gs[fb] is None else gs[fb] + t
                    if 0 <= v < NV:
                        vpu_down(v, (16 * b) // 10, (16 * (b + 1)) // 10)
                us[fb] = None
                for b in range(NB):
                    t = _dot(xb3[b], ld(UT, (fb,), b * 128, 128))
                    us[fb] = t if us[fb] is None else us[fb] + t
                    if 0 <= v < NV:
                        vpu_down(v, (16 * (b + 5)) // 10, (16 * (b + 6)) // 10)
            g, u = gs[fb], us[fb]
            if OPT_LINF:
                g = (g - mu * cg[fb]) * rs
                u = (u - mu * cu[fb]) * rs
            hs.append(_rb(g * jax.nn.sigmoid(g) * u))
            if v + 1 < NV and v + 1 >= 0 and v + 1 <= fb:
                hcs[v + 1] = jnp.broadcast_to(hs[v + 1][0:1], (128, 128)).T
        for v in range(NFB - LAG, NV):
            vpu_down(v, 0, 16)
        x4 = []
        for b in range(NB):
            y = _dot(jnp.concatenate(hs[NV:-1], axis=1), wd_v[pl.ds(NV * 128, FF - 64 - NV * 128), pl.ds(b * 128, 128)])
            y = y + _dot(hs[-1][:, :64], wd_v[pl.ds(FF - 64, 64), pl.ds(b * 128, 128)])
            if NV:
                y = y + jnp.broadcast_to(jnp.sum(accv[b], axis=0, keepdims=True), (8, 128))
            x4.append(x3[b] + (xn3[b] + (xn3[b] * 0.0 + y * sg)))
    finish(x4)


@jax.jit
def pallas_interleave_layers__compressed_kv_cla__moe_arch_mod__decode_kernel(
    A_x, A_c_kv, A_w_q, A_w_uk, A_w_uv, A_w_o, B_x, B_w_r, B_w_gate, B_w_up, B_w_down,
):
    hbm = pl.BlockSpec(memory_space=pltpu.HBM)
    vm = pltpu.VMEM
    return pl.pallas_call(
        _kernel,
        out_shape=jax.ShapeDtypeStruct((1, 1, M), BF16),
        in_specs=[hbm] * 10,
        scratch_shapes=[
            vm((1, 1, M), BF16), vm((M,), BF16),
            vm((M * H, D), BF16), vm((DC * H, D), BF16), vm((NCB, SK, 128), BF16),
            vm((DC * H, D), BF16), vm((H * D, M), BF16),
            vm((FF, M), BF16), vm((FF, M), BF16), vm((FF, M), BF16),
            vm((NB, H * 64, 128), U32), vm((16, 512, 128), U32), vm((NKB, DC // 2, 128), U32),
            vm((H, DC // 2, 128), U32), vm((NFB, M // 2, 128), U32), vm((NFB, M // 2, 128), U32),
            vm((16 * NCB, 128, 128), F32), vm((16 * D, M), F32), vm((NB, H * 64, 128), U32),
            vm((128, 8, 128), F32),
            pltpu.SemaphoreType.DMA((N_SEM,)),
        ],
        compiler_params=pltpu.CompilerParams(vmem_limit_bytes=100 * 1024 * 1024, disable_semaphore_checks=bool(int(E('NOSEMCHK', '1')))),
        name="cla_moe_decode",
    )(A_x, A_w_q.reshape(M * H, D), A_w_uk.reshape(DC * H, D), A_c_kv.reshape(SK, DC),
      A_w_uv.reshape(DC * H, D), A_w_o.reshape(H * D, M), B_w_r, B_w_gate.T, B_w_up.T, B_w_down)
```

```python
import os
import jax
import numpy as np
import jax.numpy as jnp
import jax.experimental.pallas as pl
import jax.experimental.pallas.tpu as pltpu

F32 = jnp.float32
BF16 = jnp.bfloat16
U32 = jnp.uint32
U16 = jnp.uint16

M, H, D, SK, DC, FF = 640, 32, 128, 4096, 512, 1728
NB = M // 128
NCB = DC // 128
NKB = SK // 128
NFB = (FF + 127) // 128
EPS = 1e-5

E = os.environ.get
OPT_ONLINE = int(E('ONLINE', '1'))
OPT_LINQ = int(E('LINQ', '1'))
OPT_LINF = int(E('LINF', '1'))
STOP = E('STOP', '')
SCOPES = int(E('SCOPES', '0'))
WO_SPLIT = [int(t) for t in E('WOSPLIT', '24').split(',') if t]
WD_SPLIT = [int(t) for t in E('WDSPLIT', '2,4').split(',') if t]

NF0 = int(E('NF0', '3'))
QDEF = int(E('QDEF', '1'))
NV = int(E('NV', '0'))
HV = int(E('HV', '16'))
LAG = int(E('LAG', '4'))
ANCH = int(E('ANCH', '1'))
AOFF = int(E('AOFF', '4'))
BACK = int(E('BACK', '3'))
PINS = int(E('PINS', '1'))
S6LAST = int(E('S6LAST', '8'))
NGATE = int(E('NGATE', '4'))
ZB = [int(c) for c in E('ZB', '01234')]
VITER = int(E('VITER', '2'))
N_PIN = 160
N_SEM = int(E('NSEM', '16'))


def _rb(x):
    return x.astype(BF16).astype(F32)


def _dot(a, b):
    return jax.lax.dot_general(a, b, (((1,), (0,)), ((), ())), preferred_element_type=F32)


def _cat(xs, axis):
    return xs[0] if len(xs) == 1 else jnp.concatenate(xs, axis=axis)


def _stats(parts):
    s = parts[0]
    for p in parts[1:]:
        s = s + p
    m = jnp.sum(s, axis=1, keepdims=True) * (1.0 / M)
    c = [p - m for p in parts]
    v = c[0] * c[0]
    for p in c[1:]:
        v = v + p * p
    v = jnp.sum(v, axis=1, keepdims=True) * (1.0 / M)
    return m, jax.lax.rsqrt(v + EPS)


def _ln(parts):
    m, r = _stats(parts)
    return [(p - m) * r for p in parts]


class _Scope:
    def __init__(self, name):
        self.c = jax.named_scope(name) if SCOPES else None
    def __enter__(self):
        if self.c: self.c.__enter__()
    def __exit__(self, *a):
        if self.c: self.c.__exit__(*a)


def _kernel(x_hbm, wq_hbm, wuk_hbm, ckv_hbm, wuv_hbm, wo_hbm, wr_hbm, g_hbm, u_hbm, wd_hbm,
            o_ref,
            x_v, wr_v, wq_v, wuk_v, ckv_v, wuv_v, wo_v, g_v, u_v, wd_v,
            WQ, WKT, CT, WV, GT, UT, WVT, WO32, WOT, PIN, sems):
    cps = {}
    n = [0]

    def add(name, src, dst):
        cps[name] = pltpu.make_async_copy(src, dst, sems.at[n[0]])
        n[0] += 1

    add('wq', wq_hbm, wq_v)
    add('x', x_hbm, x_v)
    add('wr', wr_hbm, wr_v)
    add('wuk', wuk_hbm, wuk_v)
    for j in range(NCB):
        add(f'ckv{j}', ckv_hbm.at[:, pl.ds(128 * j, 128)], ckv_v.at[j])
    add('g', g_hbm, g_v)
    add('u', u_hbm, u_v)
    add('wuv', wuv_hbm, wuv_v)
    wo_b = [0] + WO_SPLIT + [H]
    for i in range(len(wo_b) - 1):
        sl = pl.ds(wo_b[i] * D, (wo_b[i + 1] - wo_b[i]) * D)
        add(f'wo{i}', wo_hbm.at[sl], wo_v.at[sl])
    wd_b = [0] + WD_SPLIT + [NB]
    for i in range(len(wd_b) - 1):
        sl = pl.ds(wd_b[i] * 128, (wd_b[i + 1] - wd_b[i]) * 128)
        add(f'wd{i}', wd_hbm.at[:, sl], wd_v.at[:, sl])
    assert n[0] <= N_SEM
    for c in cps.values():
        c.start()
    waited = set()

    def wait(name):
        if name not in waited:
            cps[name].wait()
            waited.add(name)

    wq_u, wuk_u, wuv_u, ckv_u = (r.bitcast(U32) for r in (wq_v, wuk_v, wuv_v, ckv_v))

    pin_n = [0]

    def pin(vals, *names):
        if not PINS:
            for nm in names:
                wait(nm)
            return vals
        k0 = pin_n[0]
        for i, v in enumerate(vals):
            PIN[k0 + i] = v
        pin_n[0] += len(vals)
        assert pin_n[0] <= N_PIN
        for nm in names:
            wait(nm)
        return [PIN[k0 + i] for i in range(len(vals))]

    def ld(uref, idx, r0, nrows):
        return pltpu.bitcast(uref[(*idx, pl.ds(r0 // 2, nrows // 2), slice(None))], BF16)

    def shuf(src_u, r0, s):
        a = src_u[pl.ds(r0 * 16 + s, 8, stride=16), :]
        b = src_u[pl.ds((r0 + 8) * 16 + s, 8, stride=16), :]
        xx = jnp.concatenate([a, b], axis=0)
        lo = pltpu.bitcast(xx.astype(U16), U32)
        hi = pltpu.bitcast((xx >> 16).astype(U16), U32)
        return lo, hi

    def relayout_q():
        for i in range(M // 16):
            b, m16 = divmod(i, 8)
            for s in range(16):
                lo, hi = shuf(wq_u, i * 16, s)
                WQ[b, pl.ds(2 * s * 64 + m16 * 8, 8), :] = lo
                WQ[b, pl.ds((2 * s + 1) * 64 + m16 * 8, 8), :] = hi

    def relayout_v():
        for i in range(DC // 16):
            for s in range(16):
                lo, hi = shuf(wuv_u, i * 16, s)
                WV[2 * s, pl.ds(i * 8, 8), :] = lo
                WV[2 * s + 1, pl.ds(i * 8, 8), :] = hi
        if HV:
            nit = VITER
            per = -(-HV // nit)
            def body(it, _):
                for k in range(per):
                    h = jnp.minimum(it * per + k, HV - 1)
                    for cb in range(NCB):
                        WVT[h * NCB + cb] = ld(WV, (h,), cb * 128, 128).T.astype(F32)
                return 0
            jax.lax.fori_loop(0, nit, body, 0)

    def relayout_o(h0, h1):
        for h in range(h0, h1):
            if h < HV:
                for i in range(16):
                    WO32[pl.ds(h * D + i * 8, 8), :] = wo_v[pl.ds(h * D + i * 8, 8), :].astype(F32)
            else:
                for b in range(NB):
                    WOT[b, pl.ds(h * 64, 64), :] = pltpu.bitcast(
                        wo_v[pl.ds(h * D, D), pl.ds(b * 128, 128)], U32)

    def relayout_k():
        for cb in range(NCB):
            for s in range(16):
                los, his = [], []
                for i in range(8):
                    lo, hi = shuf(wuk_u, cb * 128 + i * 16, s)
                    los.append(lo)
                    his.append(hi)
                for h, parts in ((2 * s, los), (2 * s + 1, his)):
                    t = pltpu.bitcast(jnp.concatenate(parts, axis=0), BF16).T
                    WKT[(h // 8) * 4 + cb, pl.ds((h % 8) * 64, 64), :] = pltpu.bitcast(t, U32)

    def relayout_c():
        for cb in range(NCB):
            wait(f'ckv{cb}')
            for kb in range(NKB):
                t = ld(ckv_u, (cb,), kb * 128, 128).T
                CT[kb, pl.ds(cb * 64, 64), :] = pltpu.bitcast(t, U32)

    def relayout_f(src, dst):
        for fb in range(NFB):
            for b in range(NB):
                if fb < NFB - 1:
                    t = src[pl.ds(fb * 128, 128), pl.ds(b * 128, 128)]
                else:
                    t = src[pl.ds(fb * 128, 64), pl.ds(b * 128, 128)]
                    t = jnp.concatenate([t, jnp.zeros((64, 128), BF16)], axis=0)
                dst[fb, pl.ds(b * 64, 64), :] = pltpu.bitcast(t.T, U32)

    row8 = jax.lax.broadcasted_iota(jnp.int32, (8, 128), 0)

    def bd(parts):
        return jnp.concatenate(
            [jnp.where(row8 == j, p, 0.0) for j in range(8) for p in parts], axis=1)

    ones8 = jnp.ones((8, 128), F32)
    scale = D ** -0.5

    def q_block(xb, b, with_ones=False):
        lhs = bd([xb])
        if with_ones:
            lhs = jnp.concatenate([lhs, bd([ones8])], axis=0)
        return [_dot(lhs, ld(WQ, (b,), g * 1024, 1024)) for g in range(4)]

    def q_tile(xb, b, g):
        return _dot(bd([xb]), ld(WQ, (b,), g * 1024, 1024))

    def acc_list(a, b):
        return b if a is None else [x + y for x, y in zip(a, b)]

    def softmax_ctx(qa, first):
        nblk = 2 if OPT_ONLINE else 1
        per = NKB // nblk
        ss = []
        for blk in range(nblk):
            ss.append([_dot(qa, ld(CT, (kb,), 0, DC)) for kb in range(blk * per, (blk + 1) * per)])
        m_run = l_run = acc = None
        for blk in range(nblk):
            s = ss[blk]
            mx = s[0]
            for t in s[1:]:
                mx = jnp.maximum(mx, t)
            mx = jnp.max(mx, axis=1, keepdims=True)
            if m_run is not None:
                mx = jnp.maximum(mx, m_run)
            p = [jnp.exp((t - mx) * scale) for t in s]
            l = p[0]
            for t in p[1:]:
                l = l + t
            pb = jnp.concatenate([t.astype(BF16) for t in p], axis=1)
            cc = [_dot(pb, ld(ckv_u, (cb,), blk * per * 128, per * 128)) for cb in range(NCB)]
            if m_run is not None:
                al = jnp.exp((m_run - mx) * scale)
                cc = [c + a * al for c, a in zip(cc, acc)]
                l = l + l_run * al
            m_run, l_run, acc = mx, l, cc
        lsum = jnp.sum(l_run, axis=1, keepdims=True)
        return acc, 1.0 / lsum

    def attn_rest(q, first):
        if first:
            with _Scope('relayout_k'):
                relayout_k()
        qa = []
        for g in range(4):
            lhs = bd([q[g]])
            qa.append(jnp.concatenate(
                [_dot(lhs, ld(WKT, (g * 4 + cb,), 0, 1024)) for cb in range(NCB)], axis=1))
        if first:
            t = pin([x[:, cb * 128:(cb + 1) * 128] for x in qa for cb in range(NCB)], 'ckv0')
            qa = [jnp.concatenate(t[g * 4:(g + 1) * 4], axis=1) for g in range(4)]
        qa = jnp.concatenate(qa, axis=0).astype(BF16)
        if first:
            with _Scope('relayout_c'):
                relayout_c()
        cc, inv = softmax_ctx(qa, first)
        if first:
            t = pin([c[g * 8:(g + 1) * 8] for c in cc for g in range(4)]
                    + [jnp.broadcast_to(inv, (H, 128))[g * 8:(g + 1) * 8] for g in range(4)], 'g')
            cc = [jnp.concatenate(t[cb * 4:(cb + 1) * 4], axis=0) for cb in range(NCB)]
            inv = jnp.concatenate(t[16:20], axis=0)
            with _Scope('relayout_g'):
                relayout_f(g_v, GT)
            wait('u')
            with _Scope('relayout_u'):
                relayout_f(u_v, UT)
            wait('wuv')
            with _Scope('relayout_v'):
                relayout_v()
        if first or HV == 0:
            ctx = []
            for g in range(4):
                lhs = bd([_rb(c[g * 8:(g + 1) * 8]) for c in cc])
                rhs = jnp.concatenate([ld(WV, (g * 8 + j,), 0, DC) for j in range(8)], axis=0)
                ctx.append(_rb(_dot(lhs, rhs) * inv[g * 8:(g + 1) * 8]))
            outs = [None] * NB
            wob = wo_b if first else [0, H]
            for i in range(len(wob) - 1):
                if first:
                    t = pin(ctx + [o for o in outs if o is not None] if i == 0 else outs, f'wo{i}')
                    if i == 0:
                        ctx = t[:4]
                    else:
                        outs = t
                g0, g1 = wob[i] // 8, wob[i + 1] // 8
                lhs = jnp.concatenate([bd([ctx[g]]) for g in range(g0, g1)], axis=1)
                for b in range(NB):
                    r = _dot(lhs, wo_v[pl.ds(g0 * 1024, (g1 - g0) * 1024), pl.ds(b * 128, 128)])
                    outs[b] = r if outs[b] is None else outs[b] + r
                if first and HV:
                    relayout_o(wob[i], wob[i + 1])
        else:
            outs = attn_tail_mixed(cc, inv)
        return [jnp.broadcast_to(jnp.sum(r, axis=0, keepdims=True), (8, 128)) for r in outs]

    def attn_tail_mixed(cc, inv):
        accv = [None] * NB
        invb = jnp.broadcast_to(inv, (H, 128))
        true_mask = invb[0:8] > -1.0
        zhist = []
        cn = [[cc[cb][g * 8:(g + 1) * 8] * invb[g * 8:(g + 1) * 8] for cb in range(NCB)]
              for g in range(4)]

        def vpu_head(h):
            xr = [jnp.broadcast_to(cn[h // 8][cb][h % 8:h % 8 + 1], (8, 128)) for cb in range(NCB)]
            if BACK and h >= BACK:
                xr = [jnp.where(true_mask, t, zhist[h - BACK]) if n_ < NGATE else t
                      for n_, t in enumerate(xr)]
            for i in range(16):
                a = None
                for cb in range(NCB):
                    t = WVT[h * NCB + cb, pl.ds(i * 8, 8), :] * xr[cb]
                    a = t if a is None else a + t
                cv = jnp.broadcast_to(jnp.sum(a, axis=1, keepdims=True), (8, 128))
                for b in range(NB):
                    t = WO32[pl.ds(h * D + i * 8, 8), pl.ds(b * 128, 128)] * cv
                    accv[b] = t if accv[b] is None else accv[b] + t
            if BACK:
                z = accv[ZB[0]]
                for b in ZB[1:]:
                    z = jnp.maximum(z, accv[b])
                zhist.append(z)

        for h in range(HV):
            vpu_head(h)
        ctx = {}
        for g in range(HV // 8, 4):
            acc = None
            for h in range(max(HV, g * 8), g * 8 + 8):
                for cb in range(NCB):
                    lhs = jnp.where(row8 == h % 8, _rb(cn[g][cb]), 0.0)
                    t = _dot(lhs, ld(WV, (h,), cb * 128, 128))
                    acc = t if acc is None else acc + t
            ctx[g] = _rb(acc)
        lhs = {h: jnp.where(row8 == (h % 8), ctx[h // 8], 0.0) for h in range(HV, H)}
        outs = [None] * NB
        mh = list(range(HV, H))
        segs = ([mh] if S6LAST == 0 else [mh[:-S6LAST], mh[-S6LAST:]])
        for si, seg in enumerate(segs):
            for b in range(NB):
                for h in seg:
                    t = _dot(lhs[h], ld(WOT, (b,), h * 128, 128))
                    outs[b] = t if outs[b] is None else outs[b] + t
        return [o + a for o, a in zip(outs, accv)]

    def router(xn):
        wr = wr_v[...].reshape(1, M).astype(F32)
        r = None
        for b in range(NB):
            t = _rb(xn[b]) * wr[:, b * 128:(b + 1) * 128]
            r = t if r is None else r + t
        return jax.nn.sigmoid(jnp.sum(r, axis=1, keepdims=True))

    def down_block(hs, b):
        y = _dot(jnp.concatenate(hs[:-1], axis=1), wd_v[pl.ds(0, FF - 64), pl.ds(b * 128, 128)])
        return y + _dot(hs[-1][:, :64], wd_v[pl.ds(FF - 64, 64), pl.ds(b * 128, 128)])

    def finish(x):
        o_ref[0] = jnp.concatenate([p[0:1] for p in x], axis=1).astype(BF16)
        for name in cps:
            wait(name)

    with _Scope('p1_start'):
        wait('x')
        wait('wr')
        x0 = jnp.broadcast_to(x_v[0].astype(F32), (8, M))
        x0 = [x0[:, b * 128:(b + 1) * 128] for b in range(NB)]
        xn = _ln(x0)
        wait('wq')
    with _Scope('relayout_q'):
        relayout_q()
    with _Scope('A1'):
        q = None
        for b in range(NB):
            q = acc_list(q, q_block(_rb(xn[b]), b, with_ones=bool(OPT_LINQ)))
        if OPT_LINQ:
            cs = [t[8:16] for t in q]
            q = [t[0:8] for t in q]
        q = [_rb(t) for t in q]
        t = pin(q + cs, 'wuk')
        q, cs = t[:4], t[4:]
        t = pin(x0)
        x0 = t
        out = attn_rest(q, True)
        x1 = [a + b for a, b in zip(x0, out)]
    if STOP == 'A1':
        return finish(x1)
    with _Scope('B1'):
        xn1 = _ln(x1)
        sg = router(xn1)
        lhs = jnp.concatenate([_rb(t) for t in xn1], axis=1)
        if OPT_LINF:
            lhs = jnp.concatenate([lhs, jnp.ones((8, M), F32)], axis=0)
        hs, cg, cu = [], [], []
        for fb in range(NFB):
            g = _dot(lhs, ld(GT, (fb,), 0, M))
            u = _dot(lhs, ld(UT, (fb,), 0, M))
            if OPT_LINF:
                cg.append(g[8:16]); cu.append(u[8:16])
                g, u = g[0:8], u[0:8]
            hs.append(_rb(g * jax.nn.sigmoid(g) * u))
        base = [a + b for a, b in zip(x1, xn1)]
        x2 = [None] * NB
        if OPT_LINQ:
            qraw = [None] * 4
            deferred = []
            pivot = None
            xp = [None] * NB
            for i in range(len(wd_b) - 1):
                if i == 0:
                    t = pin(hs + base + xn1 + [jnp.broadcast_to(sg, (8, 128))] + cg + cu, 'wd0')
                    hs, base, xn1, sg = t[:NFB], t[NFB:NFB + 5], t[NFB + 5:NFB + 10], t[NFB + 10]
                    cg, cu = t[NFB + 11:2 * NFB + 11], t[2 * NFB + 11:]
                else:
                    done = [b for b in range(NB) if x2[b] is not None]
                    t = pin(qraw + [x2[b] for b in done] + [xp[b] for b in done]
                            + [jnp.broadcast_to(pivot, (8, 128))], f'wd{i}')
                    qraw = t[:4]
                    for n_, b in enumerate(done):
                        x2[b] = t[4 + n_]
                        xp[b] = t[4 + len(done) + n_]
                    pivot = t[-1]
                blks = list(range(wd_b[i], wd_b[i + 1]))
                with _Scope(f'wd{i}'):
                    for b in blks:
                        x2[b] = base[b] + (xn1[b] * 0.0 + down_block(hs, b) * sg)
                    if pivot is None:
                        s = x2[blks[0]]
                        for b in blks[1:]:
                            s = s + x2[b]
                        pivot = jnp.sum(s, axis=1, keepdims=True) * (1.0 / (128 * len(blks)))
                    for b in blks:
                        xp[b] = x2[b] - pivot
                    last = i == len(wd_b) - 2
                    for (bb, g) in deferred:
                        qraw[g] = qraw[g] + q_tile(_rb(xp[bb]), bb, g)
                    deferred = []
                    todo = [(b, g) for b in blks for g in range(4)]
                    if i == len(wd_b) - 3 and QDEF:
                        todo, deferred = todo[:-QDEF], todo[-QDEF:]
                    for (bb, g) in todo:
                        t = q_tile(_rb(xp[bb]), bb, g)
                        qraw[g] = t if qraw[g] is None else qraw[g] + t
        else:
            for i in range(len(wd_b) - 1):
                wait(f'wd{i}')
            for b in range(NB):
                x2[b] = base[b] + (xn1[b] * 0.0 + down_block(hs, b) * sg)
    if STOP == 'B1':
        return finish(x2)
    with _Scope('A2'):
        if OPT_LINQ:
            mu, rs = _stats(xp)
            q = [_rb((t - mu * c) * rs) for t, c in zip(qraw, cs)]
        else:
            xn = _ln(x2)
            q = None
            for b in range(NB):
                q = acc_list(q, q_block(_rb(xn[b]), b))
            q = [_rb(t) for t in q]
        out = attn_rest(q, False)
        x3 = [a + b for a, b in zip(x2, out)]
    with _Scope('B2'):
        if OPT_LINF:
            if OPT_LINQ:
                x3p = [a + b for a, b in zip(xp, out)]
            else:
                pv = jnp.sum(x2[0], axis=1, keepdims=True) * (1.0 / 128)
                x3p = [a - pv for a in x3]
            lhs = jnp.concatenate([_rb(t) for t in x3p], axis=1)
            mu, rs = _stats(x3p)
            xn3 = [(t - mu) * rs for t in x3p]
        else:
            xn3 = _ln(x3)
            lhs = jnp.concatenate([_rb(t) for t in xn3], axis=1)
        sg = router(xn3)
        xb3 = [lhs[:, b * 128:(b + 1) * 128] for b in range(NB)]
        gs, us = [None] * NFB, [None] * NFB

        def gu_tile(fb, b):
            g = _dot(xb3[b], ld(GT, (fb,), b * 128, 128))
            u = _dot(xb3[b], ld(UT, (fb,), b * 128, 128))
            gs[fb] = g if gs[fb] is None else gs[fb] + g
            us[fb] = u if us[fb] is None else us[fb] + u

        for b in range(NB):
            for fb in range(NF0):
                gu_tile(fb, b)
        hs = []
        hcs = {}
        accv = [None] * NB

        def vpu_down(fb, i0, i1):
            if fb not in hcs:
                hcs[fb] = jnp.broadcast_to(hs[fb][0:1], (128, 128)).T
            for i in range(i0, i1):
                wf = wd_v[pl.ds(fb * 128 + i * 8, 8), :].astype(F32)
                hv = hcs[fb][i * 8:(i + 1) * 8]
                for b in range(NB):
                    t = wf[:, b * 128:(b + 1) * 128] * hv
                    accv[b] = t if accv[b] is None else accv[b] + t

        for fb in range(NFB):
            v = fb - LAG
            if fb >= NF0:
                gs[fb] = None
                for b in range(NB):
                    t = _dot(xb3[b], ld(GT, (fb,), b * 128, 128))
                    gs[fb] = t if gs[fb] is None else gs[fb] + t
                    if 0 <= v < NV:
                        vpu_down(v, (16 * b) // 10, (16 * (b + 1)) // 10)
                us[fb] = None
                for b in range(NB):
                    t = _dot(xb3[b], ld(UT, (fb,), b * 128, 128))
                    us[fb] = t if us[fb] is None else us[fb] + t
                    if 0 <= v < NV:
                        vpu_down(v, (16 * (b + 5)) // 10, (16 * (b + 6)) // 10)
            g, u = gs[fb], us[fb]
            if OPT_LINF:
                g = (g - mu * cg[fb]) * rs
                u = (u - mu * cu[fb]) * rs
            hs.append(_rb(g * jax.nn.sigmoid(g) * u))
            if v + 1 < NV and v + 1 >= 0 and v + 1 <= fb:
                hcs[v + 1] = jnp.broadcast_to(hs[v + 1][0:1], (128, 128)).T
        for v in range(NFB - LAG, NV):
            vpu_down(v, 0, 16)
        x4 = []
        for b in range(NB):
            y = _dot(jnp.concatenate(hs[NV:-1], axis=1), wd_v[pl.ds(NV * 128, FF - 64 - NV * 128), pl.ds(b * 128, 128)])
            y = y + _dot(hs[-1][:, :64], wd_v[pl.ds(FF - 64, 64), pl.ds(b * 128, 128)])
            if NV:
                y = y + jnp.broadcast_to(jnp.sum(accv[b], axis=0, keepdims=True), (8, 128))
            x4.append(x3[b] + (xn3[b] + (xn3[b] * 0.0 + y * sg)))
    finish(x4)


@jax.jit
def pallas_interleave_layers__compressed_kv_cla__moe_arch_mod__decode_kernel(
    A_x, A_c_kv, A_w_q, A_w_uk, A_w_uv, A_w_o, B_x, B_w_r, B_w_gate, B_w_up, B_w_down,
):
    hbm = pl.BlockSpec(memory_space=pltpu.HBM)
    vm = pltpu.VMEM
    return pl.pallas_call(
        _kernel,
        out_shape=jax.ShapeDtypeStruct((1, 1, M), BF16),
        in_specs=[hbm] * 10,
        scratch_shapes=[
            vm((1, 1, M), BF16), vm((M,), BF16),
            vm((M * H, D), BF16), vm((DC * H, D), BF16), vm((NCB, SK, 128), BF16),
            vm((DC * H, D), BF16), vm((H * D, M), BF16),
            vm((FF, M), BF16), vm((FF, M), BF16), vm((FF, M), BF16),
            vm((NB, H * 64, 128), U32), vm((16, 512, 128), U32), vm((NKB, DC // 2, 128), U32),
            vm((H, DC // 2, 128), U32), vm((NFB, M // 2, 128), U32), vm((NFB, M // 2, 128), U32),
            vm((16 * NCB, 128, 128), F32), vm((16 * D, M), F32), vm((NB, H * 64, 128), U32),
            vm((N_PIN, 8, 128), F32),
            pltpu.SemaphoreType.DMA((N_SEM,)),
        ],
        compiler_params=pltpu.CompilerParams(vmem_limit_bytes=100 * 1024 * 1024, disable_semaphore_checks=bool(int(E('NOSEMCHK', '1')))),
        name="cla_moe_decode",
    )(A_x, A_w_q.reshape(M * H, D), A_w_uk.reshape(DC * H, D), A_c_kv.reshape(SK, DC),
      A_w_uv.reshape(DC * H, D), A_w_o.reshape(H * D, M), B_w_r, B_w_gate.T, B_w_up.T, B_w_down)
```

```python
import os
import jax
import numpy as np
import jax.numpy as jnp
import jax.experimental.pallas as pl
import jax.experimental.pallas.tpu as pltpu

F32 = jnp.float32
BF16 = jnp.bfloat16
U32 = jnp.uint32
U16 = jnp.uint16

M, H, D, SK, DC, FF = 640, 32, 128, 4096, 512, 1728
NB = M // 128
NCB = DC // 128
NKB = SK // 128
NFB = (FF + 127) // 128
EPS = 1e-5

E = os.environ.get
OPT_ONLINE = int(E('ONLINE', '1'))
OPT_LINQ = int(E('LINQ', '1'))
OPT_LINF = int(E('LINF', '1'))
STOP = E('STOP', '')
SCOPES = int(E('SCOPES', '0'))
WO_SPLIT = [int(t) for t in E('WOSPLIT', '24').split(',') if t]
WD_SPLIT = [int(t) for t in E('WDSPLIT', '2,4').split(',') if t]

NF0 = int(E('NF0', '3'))
QDEF = int(E('QDEF', '1'))
NV = int(E('NV', '0'))
HV = int(E('HV', '16'))
LAG = int(E('LAG', '4'))
ANCH = int(E('ANCH', '1'))
AOFF = int(E('AOFF', '4'))
BACK = int(E('BACK', '3'))
PINS = int(E('PINS', '1'))
S6LAST = int(E('S6LAST', '8'))
NGATE = int(E('NGATE', '4'))
ZB = [int(c) for c in E('ZB', '01234')]
VITER = int(E('VITER', '2'))
NVF = int(E('NVF', '5'))
FBACK = int(E('FBACK', '0'))
FGATE = int(E('FGATE', '5'))
FLINK = int(E('FLINK', '15'))
FRCP = int(E('FRCP', '1'))
DLAST = int(E('DLAST', '1'))
N_PIN = 160
N_SEM = int(E('NSEM', '16'))


def _rb(x):
    return x.astype(BF16).astype(F32)


def _dot(a, b):
    return jax.lax.dot_general(a, b, (((1,), (0,)), ((), ())), preferred_element_type=F32)


def _cat(xs, axis):
    return xs[0] if len(xs) == 1 else jnp.concatenate(xs, axis=axis)


def _stats(parts):
    s = parts[0]
    for p in parts[1:]:
        s = s + p
    m = jnp.sum(s, axis=1, keepdims=True) * (1.0 / M)
    c = [p - m for p in parts]
    v = c[0] * c[0]
    for p in c[1:]:
        v = v + p * p
    v = jnp.sum(v, axis=1, keepdims=True) * (1.0 / M)
    return m, jax.lax.rsqrt(v + EPS)


def _ln(parts):
    m, r = _stats(parts)
    return [(p - m) * r for p in parts]


class _Scope:
    def __init__(self, name):
        self.c = jax.named_scope(name) if SCOPES else None
    def __enter__(self):
        if self.c: self.c.__enter__()
    def __exit__(self, *a):
        if self.c: self.c.__exit__(*a)


def _kernel(x_hbm, wq_hbm, wuk_hbm, ckv_hbm, wuv_hbm, wo_hbm, wr_hbm, g_hbm, u_hbm, wd_hbm,
            o_ref,
            x_v, wr_v, wq_v, wuk_v, ckv_v, wuv_v, wo_v, g_v, u_v, wd_v,
            WQ, WKT, CT, WV, GT, UT, WVT, WO32, WOT, G32, U32F, PIN, sems):
    cps = {}
    n = [0]

    def add(name, src, dst):
        cps[name] = pltpu.make_async_copy(src, dst, sems.at[n[0]])
        n[0] += 1

    add('wq', wq_hbm, wq_v)
    add('x', x_hbm, x_v)
    add('wr', wr_hbm, wr_v)
    add('wuk', wuk_hbm, wuk_v)
    for j in range(NCB):
        add(f'ckv{j}', ckv_hbm.at[:, pl.ds(128 * j, 128)], ckv_v.at[j])
    add('g', g_hbm, g_v)
    add('u', u_hbm, u_v)
    add('wuv', wuv_hbm, wuv_v)
    wo_b = [0] + WO_SPLIT + [H]
    for i in range(len(wo_b) - 1):
        sl = pl.ds(wo_b[i] * D, (wo_b[i + 1] - wo_b[i]) * D)
        add(f'wo{i}', wo_hbm.at[sl], wo_v.at[sl])
    wd_b = [0] + WD_SPLIT + [NB]
    for i in range(len(wd_b) - 1):
        sl = pl.ds(wd_b[i] * 128, (wd_b[i + 1] - wd_b[i]) * 128)
        add(f'wd{i}', wd_hbm.at[:, sl], wd_v.at[:, sl])
    assert n[0] <= N_SEM
    for c in cps.values():
        c.start()
    waited = set()

    def wait(name):
        if name not in waited:
            cps[name].wait()
            waited.add(name)

    wq_u, wuk_u, wuv_u, ckv_u = (r.bitcast(U32) for r in (wq_v, wuk_v, wuv_v, ckv_v))

    pin_n = [0]

    def pin(vals, *names):
        if not PINS:
            for nm in names:
                wait(nm)
            return vals
        k0 = pin_n[0]
        for i, v in enumerate(vals):
            PIN[k0 + i] = v
        pin_n[0] += len(vals)
        assert pin_n[0] <= N_PIN
        for nm in names:
            wait(nm)
        return [PIN[k0 + i] for i in range(len(vals))]

    def ld(uref, idx, r0, nrows):
        return pltpu.bitcast(uref[(*idx, pl.ds(r0 // 2, nrows // 2), slice(None))], BF16)

    def shuf(src_u, r0, s):
        a = src_u[pl.ds(r0 * 16 + s, 8, stride=16), :]
        b = src_u[pl.ds((r0 + 8) * 16 + s, 8, stride=16), :]
        xx = jnp.concatenate([a, b], axis=0)
        lo = pltpu.bitcast(xx.astype(U16), U32)
        hi = pltpu.bitcast((xx >> 16).astype(U16), U32)
        return lo, hi

    def relayout_q():
        for i in range(M // 16):
            b, m16 = divmod(i, 8)
            for s in range(16):
                lo, hi = shuf(wq_u, i * 16, s)
                WQ[b, pl.ds(2 * s * 64 + m16 * 8, 8), :] = lo
                WQ[b, pl.ds((2 * s + 1) * 64 + m16 * 8, 8), :] = hi

    def relayout_v():
        for i in range(DC // 16):
            for s in range(16):
                lo, hi = shuf(wuv_u, i * 16, s)
                WV[2 * s, pl.ds(i * 8, 8), :] = lo
                WV[2 * s + 1, pl.ds(i * 8, 8), :] = hi
        if HV:
            nit = VITER
            per = -(-HV // nit)
            def body(it, _):
                for k in range(per):
                    h = jnp.minimum(it * per + k, HV - 1)
                    for cb in range(NCB):
                        WVT[h * NCB + cb] = ld(WV, (h,), cb * 128, 128).T.astype(F32)
                return 0
            jax.lax.fori_loop(0, nit, body, 0)

    def relayout_o(h0, h1):
        for h in range(h0, h1):
            if h < HV:
                for i in range(16):
                    WO32[pl.ds(h * D + i * 8, 8), :] = wo_v[pl.ds(h * D + i * 8, 8), :].astype(F32)
            else:
                for b in range(NB):
                    WOT[b, pl.ds(h * 64, 64), :] = pltpu.bitcast(
                        wo_v[pl.ds(h * D, D), pl.ds(b * 128, 128)], U32)

    def relayout_k():
        for cb in range(NCB):
            for s in range(16):
                los, his = [], []
                for i in range(8):
                    lo, hi = shuf(wuk_u, cb * 128 + i * 16, s)
                    los.append(lo)
                    his.append(hi)
                for h, parts in ((2 * s, los), (2 * s + 1, his)):
                    t = pltpu.bitcast(jnp.concatenate(parts, axis=0), BF16).T
                    WKT[(h // 8) * 4 + cb, pl.ds((h % 8) * 64, 64), :] = pltpu.bitcast(t, U32)

    def relayout_c():
        for cb in range(NCB):
            wait(f'ckv{cb}')
            for kb in range(NKB):
                t = ld(ckv_u, (cb,), kb * 128, 128).T
                CT[kb, pl.ds(cb * 64, 64), :] = pltpu.bitcast(t, U32)

    def relayout_f(src, dst):
        for fb in range(NFB):
            for b in range(NB):
                if fb < NFB - 1:
                    t = src[pl.ds(fb * 128, 128), pl.ds(b * 128, 128)]
                else:
                    t = src[pl.ds(fb * 128, 64), pl.ds(b * 128, 128)]
                    t = jnp.concatenate([t, jnp.zeros((64, 128), BF16)], axis=0)
                dst[fb, pl.ds(b * 64, 64), :] = pltpu.bitcast(t.T, U32)

    row8 = jax.lax.broadcasted_iota(jnp.int32, (8, 128), 0)

    def bd(parts):
        return jnp.concatenate(
            [jnp.where(row8 == j, p, 0.0) for j in range(8) for p in parts], axis=1)

    ones8 = jnp.ones((8, 128), F32)
    scale = D ** -0.5

    def q_block(xb, b, with_ones=False):
        lhs = bd([xb])
        if with_ones:
            lhs = jnp.concatenate([lhs, bd([ones8])], axis=0)
        return [_dot(lhs, ld(WQ, (b,), g * 1024, 1024)) for g in range(4)]

    def q_tile(xb, b, g):
        return _dot(bd([xb]), ld(WQ, (b,), g * 1024, 1024))

    def acc_list(a, b):
        return b if a is None else [x + y for x, y in zip(a, b)]

    def softmax_ctx(qa, first):
        nblk = 2 if OPT_ONLINE else 1
        per = NKB // nblk
        ss = []
        for blk in range(nblk):
            ss.append([_dot(qa, ld(CT, (kb,), 0, DC)) for kb in range(blk * per, (blk + 1) * per)])
        m_run = l_run = acc = None
        for blk in range(nblk):
            s = ss[blk]
            mx = s[0]
            for t in s[1:]:
                mx = jnp.maximum(mx, t)
            mx = jnp.max(mx, axis=1, keepdims=True)
            if m_run is not None:
                mx = jnp.maximum(mx, m_run)
            p = [jnp.exp((t - mx) * scale) for t in s]
            l = p[0]
            for t in p[1:]:
                l = l + t
            pb = jnp.concatenate([t.astype(BF16) for t in p], axis=1)
            cc = [_dot(pb, ld(ckv_u, (cb,), blk * per * 128, per * 128)) for cb in range(NCB)]
            if m_run is not None:
                al = jnp.exp((m_run - mx) * scale)
                cc = [c + a * al for c, a in zip(cc, acc)]
                l = l + l_run * al
            m_run, l_run, acc = mx, l, cc
        lsum = jnp.sum(l_run, axis=1, keepdims=True)
        return acc, 1.0 / lsum

    def attn_rest(q, first):
        if first:
            with _Scope('relayout_k'):
                relayout_k()
        qa = []
        for g in range(4):
            lhs = bd([q[g]])
            qa.append(jnp.concatenate(
                [_dot(lhs, ld(WKT, (g * 4 + cb,), 0, 1024)) for cb in range(NCB)], axis=1))
        if first:
            t = pin([x[:, cb * 128:(cb + 1) * 128] for x in qa for cb in range(NCB)], 'ckv0')
            qa = [jnp.concatenate(t[g * 4:(g + 1) * 4], axis=1) for g in range(4)]
        qa = jnp.concatenate(qa, axis=0).astype(BF16)
        if first:
            with _Scope('relayout_c'):
                relayout_c()
        cc, inv = softmax_ctx(qa, first)
        if first:
            t = pin([c[g * 8:(g + 1) * 8] for c in cc for g in range(4)]
                    + [jnp.broadcast_to(inv, (H, 128))[g * 8:(g + 1) * 8] for g in range(4)], 'g')
            cc = [jnp.concatenate(t[cb * 4:(cb + 1) * 4], axis=0) for cb in range(NCB)]
            inv = jnp.concatenate(t[16:20], axis=0)
            with _Scope('relayout_g'):
                relayout_f(g_v, GT)
                for r in range(NVF * 16):
                    G32[pl.ds(r * 8, 8), :] = g_v[pl.ds(r * 8, 8), :].astype(F32)
            wait('u')
            with _Scope('relayout_u'):
                relayout_f(u_v, UT)
                for r in range(NVF * 16):
                    U32F[pl.ds(r * 8, 8), :] = u_v[pl.ds(r * 8, 8), :].astype(F32)
            wait('wuv')
            with _Scope('relayout_v'):
                relayout_v()
        if first or HV == 0:
            ctx = []
            for g in range(4):
                lhs = bd([_rb(c[g * 8:(g + 1) * 8]) for c in cc])
                rhs = jnp.concatenate([ld(WV, (g * 8 + j,), 0, DC) for j in range(8)], axis=0)
                ctx.append(_rb(_dot(lhs, rhs) * inv[g * 8:(g + 1) * 8]))
            outs = [None] * NB
            wob = wo_b if first else [0, H]
            for i in range(len(wob) - 1):
                if first:
                    t = pin(ctx + [o for o in outs if o is not None] if i == 0 else outs, f'wo{i}')
                    if i == 0:
                        ctx = t[:4]
                    else:
                        outs = t
                g0, g1 = wob[i] // 8, wob[i + 1] // 8
                lhs = jnp.concatenate([bd([ctx[g]]) for g in range(g0, g1)], axis=1)
                for b in range(NB):
                    r = _dot(lhs, wo_v[pl.ds(g0 * 1024, (g1 - g0) * 1024), pl.ds(b * 128, 128)])
                    outs[b] = r if outs[b] is None else outs[b] + r
                if first and HV:
                    relayout_o(wob[i], wob[i + 1])
        else:
            outs = attn_tail_mixed(cc, inv)
        return [jnp.broadcast_to(jnp.sum(r, axis=0, keepdims=True), (8, 128)) for r in outs]

    def attn_tail_mixed(cc, inv):
        accv = [None] * NB
        invb = jnp.broadcast_to(inv, (H, 128))
        true_mask = invb[0:8] > -1.0
        zhist = []
        cn = [[cc[cb][g * 8:(g + 1) * 8] * invb[g * 8:(g + 1) * 8] for cb in range(NCB)]
              for g in range(4)]

        def vpu_head(h):
            xr = [jnp.broadcast_to(cn[h // 8][cb][h % 8:h % 8 + 1], (8, 128)) for cb in range(NCB)]
            if BACK and h >= BACK:
                xr = [jnp.where(true_mask, t, zhist[h - BACK]) if n_ < NGATE else t
                      for n_, t in enumerate(xr)]
            for i in range(16):
                a = None
                for cb in range(NCB):
                    t = WVT[h * NCB + cb, pl.ds(i * 8, 8), :] * xr[cb]
                    a = t if a is None else a + t
                cv = jnp.broadcast_to(jnp.sum(a, axis=1, keepdims=True), (8, 128))
                for b in range(NB):
                    t = WO32[pl.ds(h * D + i * 8, 8), pl.ds(b * 128, 128)] * cv
                    accv[b] = t if accv[b] is None else accv[b] + t
            if BACK:
                z = accv[ZB[0]]
                for b in ZB[1:]:
                    z = jnp.maximum(z, accv[b])
                zhist.append(z)

        for h in range(HV):
            vpu_head(h)
        ctx = {}
        for g in range(HV // 8, 4):
            acc = None
            for h in range(max(HV, g * 8), g * 8 + 8):
                for cb in range(NCB):
                    lhs = jnp.where(row8 == h % 8, _rb(cn[g][cb]), 0.0)
                    t = _dot(lhs, ld(WV, (h,), cb * 128, 128))
                    acc = t if acc is None else acc + t
            ctx[g] = _rb(acc)
        lhs = {h: jnp.where(row8 == (h % 8), ctx[h // 8], 0.0) for h in range(HV, H)}
        outs = [None] * NB
        mh = list(range(HV, H))
        segs = ([mh] if S6LAST == 0 else [mh[:-S6LAST], mh[-S6LAST:]])
        for si, seg in enumerate(segs):
            for b in range(NB):
                for h in seg:
                    t = _dot(lhs[h], ld(WOT, (b,), h * 128, 128))
                    outs[b] = t if outs[b] is None else outs[b] + t
        return [o + a for o, a in zip(outs, accv)]

    def router(xn):
        wr = wr_v[...].reshape(1, M).astype(F32)
        r = None
        for b in range(NB):
            t = _rb(xn[b]) * wr[:, b * 128:(b + 1) * 128]
            r = t if r is None else r + t
        return jax.nn.sigmoid(jnp.sum(r, axis=1, keepdims=True))

    def down_block(hs, b):
        y = _dot(jnp.concatenate(hs[:-1], axis=1), wd_v[pl.ds(0, FF - 64), pl.ds(b * 128, 128)])
        return y + _dot(hs[-1][:, :64], wd_v[pl.ds(FF - 64, 64), pl.ds(b * 128, 128)])

    def finish(x):
        o_ref[0] = jnp.concatenate([p[0:1] for p in x], axis=1).astype(BF16)
        for name in cps:
            wait(name)

    with _Scope('p1_start'):
        wait('x')
        wait('wr')
        x0 = jnp.broadcast_to(x_v[0].astype(F32), (8, M))
        x0 = [x0[:, b * 128:(b + 1) * 128] for b in range(NB)]
        xn = _ln(x0)
        wait('wq')
    with _Scope('relayout_q'):
        relayout_q()
    with _Scope('A1'):
        q = None
        for b in range(NB):
            q = acc_list(q, q_block(_rb(xn[b]), b, with_ones=bool(OPT_LINQ)))
        if OPT_LINQ:
            cs = [t[8:16] for t in q]
            q = [t[0:8] for t in q]
        q = [_rb(t) for t in q]
        t = pin(q + cs, 'wuk')
        q, cs = t[:4], t[4:]
        t = pin(x0)
        x0 = t
        out = attn_rest(q, True)
        x1 = [a + b for a, b in zip(x0, out)]
    if STOP == 'A1':
        return finish(x1)
    with _Scope('B1'):
        xn1 = _ln(x1)
        sg = router(xn1)
        lhs = jnp.concatenate([_rb(t) for t in xn1], axis=1)
        if OPT_LINF:
            lhs = jnp.concatenate([lhs, jnp.ones((8, M), F32)], axis=0)
        hs, cg, cu = [], [], []
        for fb in range(NFB):
            g = _dot(lhs, ld(GT, (fb,), 0, M))
            u = _dot(lhs, ld(UT, (fb,), 0, M))
            if OPT_LINF:
                cg.append(g[8:16]); cu.append(u[8:16])
                g, u = g[0:8], u[0:8]
            hs.append(_rb(g * jax.nn.sigmoid(g) * u))
        base = [a + b for a, b in zip(x1, xn1)]
        x2 = [None] * NB
        if OPT_LINQ:
            qraw = [None] * 4
            deferred = []
            pivot = None
            xp = [None] * NB
            for i in range(len(wd_b) - 1):
                if i == 0:
                    t = pin(hs + base + xn1 + [jnp.broadcast_to(sg, (8, 128))] + cg + cu, 'wd0')
                    hs, base, xn1, sg = t[:NFB], t[NFB:NFB + 5], t[NFB + 5:NFB + 10], t[NFB + 10]
                    cg, cu = t[NFB + 11:2 * NFB + 11], t[2 * NFB + 11:]
                else:
                    done = [b for b in range(NB) if x2[b] is not None]
                    t = pin(qraw + [x2[b] for b in done] + [xp[b] for b in done]
                            + [jnp.broadcast_to(pivot, (8, 128))], f'wd{i}')
                    qraw = t[:4]
                    for n_, b in enumerate(done):
                        x2[b] = t[4 + n_]
                        xp[b] = t[4 + len(done) + n_]
                    pivot = t[-1]
                blks = list(range(wd_b[i], wd_b[i + 1]))
                with _Scope(f'wd{i}'):
                    for b in blks:
                        x2[b] = base[b] + (xn1[b] * 0.0 + down_block(hs, b) * sg)
                    if pivot is None:
                        s = x2[blks[0]]
                        for b in blks[1:]:
                            s = s + x2[b]
                        pivot = jnp.sum(s, axis=1, keepdims=True) * (1.0 / (128 * len(blks)))
                    for b in blks:
                        xp[b] = x2[b] - pivot
                    last = i == len(wd_b) - 2
                    for (bb, g) in deferred:
                        qraw[g] = qraw[g] + q_tile(_rb(xp[bb]), bb, g)
                    deferred = []
                    todo = [(b, g) for b in blks for g in range(4)]
                    if i == len(wd_b) - 3 and QDEF:
                        todo, deferred = todo[:-QDEF], todo[-QDEF:]
                    for (bb, g) in todo:
                        t = q_tile(_rb(xp[bb]), bb, g)
                        qraw[g] = t if qraw[g] is None else qraw[g] + t
        else:
            for i in range(len(wd_b) - 1):
                wait(f'wd{i}')
            for b in range(NB):
                x2[b] = base[b] + (xn1[b] * 0.0 + down_block(hs, b) * sg)
    if STOP == 'B1':
        return finish(x2)
    with _Scope('A2'):
        if OPT_LINQ:
            mu, rs = _stats(xp)
            q = [_rb((t - mu * c) * rs) for t, c in zip(qraw, cs)]
        else:
            xn = _ln(x2)
            q = None
            for b in range(NB):
                q = acc_list(q, q_block(_rb(xn[b]), b))
            q = [_rb(t) for t in q]
        out = attn_rest(q, False)
        x3 = [a + b for a, b in zip(x2, out)]
    with _Scope('B2'):
        if OPT_LINF:
            if OPT_LINQ:
                x3p = [a + b for a, b in zip(xp, out)]
            else:
                pv = jnp.sum(x2[0], axis=1, keepdims=True) * (1.0 / 128)
                x3p = [a - pv for a in x3]
            lhs = jnp.concatenate([_rb(t) for t in x3p], axis=1)
            mu, rs = _stats(x3p)
            xn3 = [(t - mu) * rs for t in x3p]
        else:
            xn3 = _ln(x3)
            lhs = jnp.concatenate([_rb(t) for t in xn3], axis=1)
        sg = router(xn3)
        xb3 = [lhs[:, b * 128:(b + 1) * 128] for b in range(NB)]
        gs, us = [None] * NFB, [None] * NFB
        mfb = list(range(NVF, NFB))

        def gu_tile(fb, b):
            g = _dot(xb3[b], ld(GT, (fb,), b * 128, 128))
            gs[fb] = g if gs[fb] is None else gs[fb] + g
            u = _dot(xb3[b], ld(UT, (fb,), b * 128, 128))
            us[fb] = u if us[fb] is None else us[fb] + u

        for b in range(NB):
            for fb in mfb[:NF0]:
                gu_tile(fb, b)
        for fb in mfb[NF0:]:
            for b in range(NB):
                gs[fb] = (lambda t, a: t if a is None else a + t)(
                    _dot(xb3[b], ld(GT, (fb,), b * 128, 128)), gs[fb])
            for b in range(NB):
                us[fb] = (lambda t, a: t if a is None else a + t)(
                    _dot(xb3[b], ld(UT, (fb,), b * 128, 128)), us[fb])

        true_mask3 = (pltpu.bitcast(x3p[0], jnp.int32) | 1) != 0
        link = []

        def vpu_col(W, fb):
            xr = x3p
            k = len(link)
            if FBACK and k >= FBACK:
                xr = [jnp.where(true_mask3, t, link[k - FBACK]) for t in xr[:FGATE]] + xr[FGATE:]
            a = []
            for i in range(16):
                t = None
                for b in range(NB):
                    p = W[pl.ds(fb * 128 + i * 8, 8), pl.ds(b * 128, 128)] * xr[b]
                    t = p if t is None else t + p
                a.append(t)
            z = a[FLINK]
            link.append(pl.reciprocal(z, approx=True) if FRCP else z)
            at = jnp.concatenate(a, axis=0).T
            parts = [at[i * 8:(i + 1) * 8] for i in range(16)]
            while len(parts) > 1:
                parts = [parts[i] + parts[i + 1] for i in range(0, len(parts), 2)]
            return jnp.broadcast_to(jnp.sum(parts[0], axis=0, keepdims=True), (8, 128))

        for fb in range(NVF):
            gs[fb] = vpu_col(G32, fb)
            us[fb] = vpu_col(U32F, fb)
        hs = []
        for fb in range(NFB):
            g = (gs[fb] - mu * cg[fb]) * rs
            u = (us[fb] - mu * cu[fb]) * rs
            hs.append(_rb(g * jax.nn.sigmoid(g) * u))
        ys = [None] * NB
        for seg in [sg_ for sg_ in (mfb[:len(mfb) - DLAST], mfb[len(mfb) - DLAST:] + list(range(NVF))) if sg_]:
            for b in range(NB):
                for fb in seg:
                    if fb == NFB - 1:
                        t = _dot(hs[fb][:, :64], wd_v[pl.ds(fb * 128, 64), pl.ds(b * 128, 128)])
                    else:
                        t = _dot(hs[fb], wd_v[pl.ds(fb * 128, 128), pl.ds(b * 128, 128)])
                    ys[b] = t if ys[b] is None else ys[b] + t
        x4 = [x3[b] + (xn3[b] + (xn3[b] * 0.0 + ys[b] * sg)) for b in range(NB)]
    finish(x4)


@jax.jit
def pallas_interleave_layers__compressed_kv_cla__moe_arch_mod__decode_kernel(
    A_x, A_c_kv, A_w_q, A_w_uk, A_w_uv, A_w_o, B_x, B_w_r, B_w_gate, B_w_up, B_w_down,
):
    hbm = pl.BlockSpec(memory_space=pltpu.HBM)
    vm = pltpu.VMEM
    return pl.pallas_call(
        _kernel,
        out_shape=jax.ShapeDtypeStruct((1, 1, M), BF16),
        in_specs=[hbm] * 10,
        scratch_shapes=[
            vm((1, 1, M), BF16), vm((M,), BF16),
            vm((M * H, D), BF16), vm((DC * H, D), BF16), vm((NCB, SK, 128), BF16),
            vm((DC * H, D), BF16), vm((H * D, M), BF16),
            vm((FF, M), BF16), vm((FF, M), BF16), vm((FF, M), BF16),
            vm((NB, H * 64, 128), U32), vm((16, 512, 128), U32), vm((NKB, DC // 2, 128), U32),
            vm((H, DC // 2, 128), U32), vm((NFB, M // 2, 128), U32), vm((NFB, M // 2, 128), U32),
            vm((16 * NCB, 128, 128), F32), vm((16 * D, M), F32), vm((NB, H * 64, 128), U32),
            vm((8 * 128, M), F32), vm((8 * 128, M), F32),
            vm((N_PIN, 8, 128), F32),
            pltpu.SemaphoreType.DMA((N_SEM,)),
        ],
        compiler_params=pltpu.CompilerParams(vmem_limit_bytes=100 * 1024 * 1024, disable_semaphore_checks=bool(int(E('NOSEMCHK', '1')))),
        name="cla_moe_decode",
    )(A_x, A_w_q.reshape(M * H, D), A_w_uk.reshape(DC * H, D), A_c_kv.reshape(SK, DC),
      A_w_uv.reshape(DC * H, D), A_w_o.reshape(H * D, M), B_w_r, B_w_gate.T, B_w_up.T, B_w_down)
```

```python
import os
import jax
import numpy as np
import jax.numpy as jnp
import jax.experimental.pallas as pl
import jax.experimental.pallas.tpu as pltpu

F32 = jnp.float32
BF16 = jnp.bfloat16
U32 = jnp.uint32
U16 = jnp.uint16
I32 = jnp.int32

M, H, D, SK, DC, FF = 640, 32, 128, 4096, 512, 1728
NB = M // 128
NCB = DC // 128
NKB = SK // 128
NFB = (FF + 127) // 128
EPS = 1e-5

E = os.environ.get
HQ = int(E('HQ', '10'))
QBACK = int(E('QBACK', '3'))
QDEF = int(E('QDEF', '8'))
HV = int(E('HV', '16'))
VBACK = int(E('VBACK', '3'))
S6LAST = int(E('S6LAST', '8'))
NVF = int(E('NVF', '5'))
NF0 = int(E('NF0', '3'))
DLAST = int(E('DLAST', '1'))
VITER = int(E('VITER', '2'))
STOP = E('STOP', '')
WO_SPLIT = [int(t) for t in E('WOSPLIT', '24').split(',') if t]
WD_SPLIT = [int(t) for t in E('WDSPLIT', '2,4').split(',') if t]
N_PIN = 176
N_SEM = 16


def _rb(x):
    return x.astype(BF16).astype(F32)


def _dot(a, b):
    return jax.lax.dot_general(a, b, (((1,), (0,)), ((), ())), preferred_element_type=F32)


def _acc(a, t):
    return t if a is None else a + t


def _stats(parts):
    s = parts[0]
    for p in parts[1:]:
        s = s + p
    m = jnp.sum(s, axis=1, keepdims=True) * (1.0 / M)
    c = [p - m for p in parts]
    v = c[0] * c[0]
    for p in c[1:]:
        v = v + p * p
    v = jnp.sum(v, axis=1, keepdims=True) * (1.0 / M)
    return m, jax.lax.rsqrt(v + EPS)


def _ln(parts):
    m, r = _stats(parts)
    return [(p - m) * r for p in parts]


def _rowsum(a):
    return jnp.broadcast_to(jnp.sum(a, axis=0, keepdims=True), (8, 128))


def _lanesum(a):
    return jnp.broadcast_to(jnp.sum(a, axis=1, keepdims=True), (8, 128))


def _kernel(x_hbm, wq_hbm, wuk_hbm, ckv_hbm, wuv_hbm, wo_hbm, wr_hbm, g_hbm, u_hbm, wd_hbm,
            o_ref,
            x_v, wr_v, wq_v, wuk_v, ckv_v, wuv_v, wo_v, g_v, u_v, wd_v,
            WQ, WKT, CT, WV, GT, UT,
            WQT32, WKT32, WVT32, WO32, WOT, G32, U32F, AE, PIN, sems):
    cps = {}

    def add(name, src, dst):
        cps[name] = pltpu.make_async_copy(src, dst, sems.at[len(cps)])

    add('wq', wq_hbm, wq_v)
    add('x', x_hbm, x_v)
    add('wr', wr_hbm, wr_v)
    add('wuk', wuk_hbm, wuk_v)
    for j in range(NCB):
        add(f'ckv{j}', ckv_hbm.at[:, pl.ds(128 * j, 128)], ckv_v.at[j])
    add('g', g_hbm, g_v)
    add('u', u_hbm, u_v)
    add('wuv', wuv_hbm, wuv_v)
    wo_b = [0] + WO_SPLIT + [H]
    for i in range(len(wo_b) - 1):
        sl = pl.ds(wo_b[i] * D, (wo_b[i + 1] - wo_b[i]) * D)
        add(f'wo{i}', wo_hbm.at[sl], wo_v.at[sl])
    wd_b = [0] + WD_SPLIT + [NB]
    for i in range(len(wd_b) - 1):
        sl = pl.ds(wd_b[i] * 128, (wd_b[i + 1] - wd_b[i]) * 128)
        add(f'wd{i}', wd_hbm.at[:, sl], wd_v.at[:, sl])
    assert len(cps) <= N_SEM
    for c in cps.values():
        c.start()
    waited = set()

    def wait(name):
        if name not in waited:
            cps[name].wait()
            waited.add(name)

    pin_n = [0]

    def pin(vals, *names):
        k0 = pin_n[0]
        for i, v in enumerate(vals):
            PIN[k0 + i] = v
        pin_n[0] += len(vals)
        assert pin_n[0] <= N_PIN
        for nm in names:
            wait(nm)
        return [PIN[k0 + i] for i in range(len(vals))]

    wq_u, wuk_u, wuv_u, ckv_u = (r.bitcast(U32) for r in (wq_v, wuk_v, wuv_v, ckv_v))

    def ld(uref, idx, r0, nrows):
        return pltpu.bitcast(uref[(*idx, pl.ds(r0 // 2, nrows // 2), slice(None))], BF16)

    def shuf(src_u, r0, s):
        a = src_u[pl.ds(r0 * 16 + s, 8, stride=16), :]
        b = src_u[pl.ds((r0 + 8) * 16 + s, 8, stride=16), :]
        xx = jnp.concatenate([a, b], axis=0)
        lo = pltpu.bitcast(xx.astype(U16), U32)
        hi = pltpu.bitcast((xx >> 16).astype(U16), U32)
        return lo, hi

    def relayout_q():
        for i in range(M // 16):
            b, m16 = divmod(i, 8)
            for s in range(16):
                lo, hi = shuf(wq_u, i * 16, s)
                WQ[b, pl.ds(2 * s * 64 + m16 * 8, 8), :] = lo
                WQ[b, pl.ds((2 * s + 1) * 64 + m16 * 8, 8), :] = hi
        for h in range(HQ):
            for b in range(NB):
                WQT32[h * NB + b] = ld(WQ, (b,), h * 128, 128).T.astype(F32)

    def relayout_k():
        for cb in range(NCB):
            for s in range(16):
                los, his = [], []
                for i in range(8):
                    lo, hi = shuf(wuk_u, cb * 128 + i * 16, s)
                    los.append(lo)
                    his.append(hi)
                for h, parts in ((2 * s, los), (2 * s + 1, his)):
                    t = pltpu.bitcast(jnp.concatenate(parts, axis=0), BF16).T
                    WKT[(h // 8) * 4 + cb, pl.ds((h % 8) * 64, 64), :] = pltpu.bitcast(t, U32)
                    if h < HQ:
                        WKT32[h * NCB + cb] = t.astype(F32)

    def relayout_c():
        for cb in range(NCB):
            wait(f'ckv{cb}')
            for kb in range(NKB):
                t = ld(ckv_u, (cb,), kb * 128, 128).T
                CT[kb, pl.ds(cb * 64, 64), :] = pltpu.bitcast(t, U32)

    def relayout_f(src, dst, dst32):
        for fb in range(NFB):
            for b in range(NB):
                if fb < NFB - 1:
                    t = src[pl.ds(fb * 128, 128), pl.ds(b * 128, 128)]
                else:
                    t = src[pl.ds(fb * 128, 64), pl.ds(b * 128, 128)]
                    t = jnp.concatenate([t, jnp.zeros((64, 128), BF16)], axis=0)
                dst[fb, pl.ds(b * 64, 64), :] = pltpu.bitcast(t.T, U32)
        for r in range(NVF * 16):
            dst32[pl.ds(r * 8, 8), :] = src[pl.ds(r * 8, 8), :].astype(F32)

    def relayout_v():
        for i in range(DC // 16):
            for s in range(16):
                lo, hi = shuf(wuv_u, i * 16, s)
                WV[2 * s, pl.ds(i * 8, 8), :] = lo
                WV[2 * s + 1, pl.ds(i * 8, 8), :] = hi
        if HV:
            per = -(-HV // VITER)

            def body(it, _):
                for k in range(per):
                    h = jnp.minimum(it * per + k, HV - 1)
                    for cb in range(NCB):
                        WVT32[h * NCB + cb] = ld(WV, (h,), cb * 128, 128).T.astype(F32)
                return 0
            jax.lax.fori_loop(0, VITER, body, 0)

    def relayout_o(h0, h1):
        for h in range(h0, h1):
            if h < HV:
                for i in range(16):
                    WO32[pl.ds(h * D + i * 8, 8), :] = wo_v[pl.ds(h * D + i * 8, 8), :].astype(F32)
            else:
                for b in range(NB):
                    WOT[b, pl.ds((h - HV) * 64, 64), :] = pltpu.bitcast(
                        wo_v[pl.ds(h * D, D), pl.ds(b * 128, 128)], U32)

    row8 = jax.lax.broadcasted_iota(I32, (8, 128), 0)

    def row_sel(v, j):
        return jnp.where(row8 == j, v, 0.0)

    def bd(v):
        return jnp.concatenate([row_sel(v, j) for j in range(8)], axis=1)

    def always(v):
        return (pltpu.bitcast(v, I32) | 1) != 0

    scale = D ** -0.5

    def softmax_ctx(qa):
        nblk = 2
        per = NKB // nblk
        ss = [[_dot(qa, ld(CT, (kb,), 0, DC)) for kb in range(blk * per, (blk + 1) * per)]
              for blk in range(nblk)]
        m_run = l_run = acc = None
        for blk in range(nblk):
            s = ss[blk]
            mx = s[0]
            for t in s[1:]:
                mx = jnp.maximum(mx, t)
            mx = jnp.max(mx, axis=1, keepdims=True)
            if m_run is not None:
                mx = jnp.maximum(mx, m_run)
            p = [jnp.exp((t - mx) * scale) for t in s]
            l = p[0]
            for t in p[1:]:
                l = l + t
            pb = jnp.concatenate([t.astype(BF16) for t in p], axis=1)
            cc = [_dot(pb, ld(ckv_u, (cb,), blk * per * 128, per * 128)) for cb in range(NCB)]
            if m_run is not None:
                al = jnp.exp((m_run - mx) * scale)
                cc = [c + a * al for c, a in zip(cc, acc)]
                l = l + l_run * al
            m_run, l_run, acc = mx, l, cc
        return acc, 1.0 / jnp.sum(l_run, axis=1, keepdims=True)

    def finish(x):
        o_ref[0] = jnp.concatenate([p[0:1] for p in x], axis=1).astype(BF16)
        for name in cps:
            wait(name)

    wait('x')
    wait('wr')
    x0 = jnp.broadcast_to(x_v[0].astype(F32), (8, M))
    x0 = [x0[:, b * 128:(b + 1) * 128] for b in range(NB)]
    wr = wr_v[...].reshape(1, M).astype(F32)

    def router(xn):
        r = None
        for b in range(NB):
            r = _acc(r, _rb(xn[b]) * wr[:, b * 128:(b + 1) * 128])
        return jax.nn.sigmoid(jnp.sum(r, axis=1, keepdims=True))

    xn = _ln(x0)
    wait('wq')
    relayout_q()
    ones_bd = bd(jnp.ones((8, 128), F32))
    q = [None] * 4
    for b in range(NB):
        lhs = jnp.concatenate([bd(_rb(xn[b])), ones_bd], axis=0)
        for g in range(4):
            q[g] = _acc(q[g], _dot(lhs, ld(WQ, (b,), g * 1024, 1024)))
    cs = [t[8:16] for t in q]
    q = [_rb(t[0:8]) for t in q]
    t = pin(q + cs + x0, 'wuk')
    q, cs, x0 = t[:4], t[4:8], t[8:]
    relayout_k()
    qa, csk = [], []
    for g in range(4):
        lhs = jnp.concatenate([bd(q[g]), bd(cs[g])], axis=0)
        for cb in range(NCB):
            r = _dot(lhs, ld(WKT, (g * 4 + cb,), 0, 1024))
            qa.append(r[0:8])
            csk.append(r[8:16])
    t = pin(qa + csk, 'ckv0')
    qa, csk = t[:16], t[16:]
    qa = jnp.concatenate([jnp.concatenate(qa[g * 4:(g + 1) * 4], axis=1) for g in range(4)], axis=0)
    relayout_c()
    cc, inv = softmax_ctx(qa.astype(BF16))
    invb = jnp.broadcast_to(inv, (H, 128))
    t = pin([c[g * 8:(g + 1) * 8] for c in cc for g in range(4)]
            + [invb[g * 8:(g + 1) * 8] for g in range(4)], 'g')
    cc, inv = t[:16], t[16:]
    relayout_f(g_v, GT, G32)
    wait('u')
    relayout_f(u_v, UT, U32F)
    wait('wuv')
    relayout_v()
    ctx = []
    for g in range(4):
        lhs = jnp.concatenate([row_sel(_rb(cc[cb * 4 + g]), j) for j in range(8) for cb in range(NCB)], axis=1)
        rhs = jnp.concatenate([ld(WV, (g * 8 + j,), 0, DC) for j in range(8)], axis=0)
        ctx.append(_rb(_dot(lhs, rhs) * inv[g]))
    outs = [None] * NB
    for i in range(len(wo_b) - 1):
        if i == 0:
            ctx = pin(ctx, 'wo0')
        else:
            outs = pin(outs, f'wo{i}')
        g0, g1 = wo_b[i] // 8, wo_b[i + 1] // 8
        lhs = jnp.concatenate([bd(ctx[g]) for g in range(g0, g1)], axis=1)
        for b in range(NB):
            outs[b] = _acc(outs[b], _dot(lhs, wo_v[pl.ds(g0 * 1024, (g1 - g0) * 1024), pl.ds(b * 128, 128)]))
        relayout_o(wo_b[i], wo_b[i + 1])
    x1 = [a + _rowsum(o) for a, o in zip(x0, outs)]
    if STOP == 'A1':
        return finish(x1)

    xn1 = _ln(x1)
    sg = router(xn1)
    lhs = jnp.concatenate([jnp.concatenate([_rb(t) for t in xn1], axis=1), jnp.ones((8, M), F32)], axis=0)
    hs, cg, cu = [], [], []
    for fb in range(NFB):
        g = _dot(lhs, ld(GT, (fb,), 0, M))
        u = _dot(lhs, ld(UT, (fb,), 0, M))
        cg.append(g[8:16])
        cu.append(u[8:16])
        g, u = g[0:8], u[0:8]
        hs.append(_rb(g * jax.nn.sigmoid(g) * u))
    base = [a + b for a, b in zip(x1, xn1)]

    def down_tile(hs, fb, b):
        if fb == NFB - 1:
            return _dot(hs[fb][:, :64], wd_v[pl.ds(fb * 128, 64), pl.ds(b * 128, 128)])
        return _dot(hs[fb], wd_v[pl.ds(fb * 128, 128), pl.ds(b * 128, 128)])

    x2, xp = [None] * NB, [None] * NB
    qraw = [None] * 4
    deferred = []
    pivot = None
    nseg = len(wd_b) - 1
    for i in range(nseg):
        if i == 0:
            t = pin(hs + base + xn1 + [jnp.broadcast_to(sg, (8, 128))] + cg + cu, 'wd0')
            hs, base, xn1, sg = t[:NFB], t[NFB:NFB + 5], t[NFB + 5:NFB + 10], t[NFB + 10]
            cg, cu = t[NFB + 11:2 * NFB + 11], t[2 * NFB + 11:]
        else:
            done = [b for b in range(NB) if x2[b] is not None]
            gl = [g for g in range(4) if qraw[g] is not None]
            t = pin([qraw[g] for g in gl] + [x2[b] for b in done] + [xp[b] for b in done]
                    + [jnp.broadcast_to(pivot, (8, 128))], f'wd{i}')
            for n_, g in enumerate(gl):
                qraw[g] = t[n_]
            for n_, b in enumerate(done):
                x2[b] = t[len(gl) + n_]
                xp[b] = t[len(gl) + len(done) + n_]
            pivot = t[-1]
        blks = list(range(wd_b[i], wd_b[i + 1]))
        for b in blks:
            y = None
            for fb in range(NFB):
                y = _acc(y, down_tile(hs, fb, b))
            x2[b] = base[b] + (xn1[b] * 0.0 + y * sg)
        if pivot is None:
            s = x2[blks[0]]
            for b in blks[1:]:
                s = s + x2[b]
            pivot = jnp.sum(s, axis=1, keepdims=True) * (1.0 / (128 * len(blks)))
        for b in blks:
            xp[b] = x2[b] - pivot
        todo = deferred + [(b, h) for b in blks for h in range(HQ, H)]
        deferred = []
        if i == nseg - 2 and QDEF:
            todo, deferred = todo[:-QDEF], todo[-QDEF:]
        for (b, h) in todo:
            qraw[h // 8] = _acc(qraw[h // 8], _dot(row_sel(_rb(xp[b]), h % 8), ld(WQ, (b,), h * 128, 128)))
        if i < nseg - 1:
            for h in range(HQ):
                for r in range(16):
                    a = None if i == 0 else AE[h * 16 + r]
                    for b in blks:
                        a = _acc(a, WQT32[h * NB + b, pl.ds(r * 8, 8), :] * xp[b])
                    AE[h * 16 + r] = a
    if STOP == 'B1':
        return finish(x2)

    mu, rs = _stats(xp)
    qa = [[None] * NCB for _ in range(4)]
    for h in range(HQ, H):
        g = h // 8
        lhs = row_sel(_rb(qraw[g]), h % 8)
        for cb in range(NCB):
            qa[g][cb] = _acc(qa[g][cb], _dot(lhs, ld(WKT, (g * 4 + cb,), (h % 8) * 128, 128)))
    tmask = always(xp[wd_b[-2]])
    zq = []
    for h in range(HQ):
        xr = {b: xp[b] for b in range(wd_b[-2], NB)}
        if QBACK and h >= QBACK:
            xr = {b: jnp.where(tmask, v, zq[h - QBACK]) for b, v in xr.items()}
        acc = [None] * NCB
        for r in range(16):
            a = AE[h * 16 + r]
            for b, v in xr.items():
                a = a + WQT32[h * NB + b, pl.ds(r * 8, 8), :] * v
            cv = _lanesum(a)
            for cb in range(NCB):
                acc[cb] = _acc(acc[cb], WKT32[h * NCB + cb, pl.ds(r * 8, 8), :] * cv)
        z = acc[0]
        for cb in range(1, NCB):
            z = jnp.maximum(z, acc[cb])
        zq.append(z)
        for cb in range(NCB):
            prev = qa[h // 8][cb]
            qa[h // 8][cb] = jnp.where(row8 == h % 8, _rowsum(acc[cb]), 0.0 if prev is None else prev) \
                if (h // 8) * 8 + 7 >= HQ or prev is not None else row_sel(_rowsum(acc[cb]), h % 8)
    qa = jnp.concatenate(
        [jnp.concatenate([(qa[g][cb] - mu * csk[g * 4 + cb]) * rs for cb in range(NCB)], axis=1)
         for g in range(4)], axis=0)
    cc, inv = softmax_ctx(qa.astype(BF16))

    invb = jnp.broadcast_to(inv, (H, 128))
    cn = [[cc[cb][g * 8:(g + 1) * 8] * invb[g * 8:(g + 1) * 8] for cb in range(NCB)] for g in range(4)]
    vmask = always(invb[0:8])
    accv = [None] * NB
    zv = []
    for h in range(HV):
        xr = [jnp.broadcast_to(cn[h // 8][cb][h % 8:h % 8 + 1], (8, 128)) for cb in range(NCB)]
        if VBACK and h >= VBACK:
            xr = [jnp.where(vmask, v, zv[h - VBACK]) for v in xr]
        for r in range(16):
            a = None
            for cb in range(NCB):
                a = _acc(a, WVT32[h * NCB + cb, pl.ds(r * 8, 8), :] * xr[cb])
            cv = _lanesum(a)
            for b in range(NB):
                accv[b] = _acc(accv[b], WO32[pl.ds(h * D + r * 8, 8), pl.ds(b * 128, 128)] * cv)
        z = accv[0]
        for b in range(1, NB):
            z = jnp.maximum(z, accv[b])
        zv.append(z)
    ctx = {}
    for g in range(HV // 8, 4):
        acc = None
        for h in range(max(HV, g * 8), g * 8 + 8):
            for cb in range(NCB):
                acc = _acc(acc, _dot(row_sel(_rb(cn[g][cb]), h % 8), ld(WV, (h,), cb * 128, 128)))
        ctx[g] = _rb(acc)
    mh = list(range(HV, H))
    lhs6 = {h: row_sel(ctx[h // 8], h % 8) for h in mh}
    outs = [None] * NB
    for seg in ([mh[:-S6LAST], mh[-S6LAST:]] if S6LAST else [mh]):
        for b in range(NB):
            for h in seg:
                outs[b] = _acc(outs[b], _dot(lhs6[h], ld(WOT, (b,), (h - HV) * 128, 128)))
    out = [_rowsum(o if a is None else o + a) for o, a in zip(outs, accv)]

    x3 = [a + b for a, b in zip(x2, out)]
    x3p = [a + b for a, b in zip(xp, out)]
    xb3 = [_rb(t) for t in x3p]
    mu, rs = _stats(x3p)
    xn3 = [(t - mu) * rs for t in x3p]
    sg = router(xn3)
    gs, us = [None] * NFB, [None] * NFB
    mfb = list(range(NVF, NFB))
    for b in range(NB):
        for fb in mfb[:NF0]:
            gs[fb] = _acc(gs[fb], _dot(xb3[b], ld(GT, (fb,), b * 128, 128)))
            us[fb] = _acc(us[fb], _dot(xb3[b], ld(UT, (fb,), b * 128, 128)))
    for fb in mfb[NF0:]:
        for b in range(NB):
            gs[fb] = _acc(gs[fb], _dot(xb3[b], ld(GT, (fb,), b * 128, 128)))
        for b in range(NB):
            us[fb] = _acc(us[fb], _dot(xb3[b], ld(UT, (fb,), b * 128, 128)))

    def vpu_col(W, fb):
        a = []
        for i in range(16):
            t = None
            for b in range(NB):
                t = _acc(t, W[pl.ds(fb * 128 + i * 8, 8), pl.ds(b * 128, 128)] * x3p[b])
            a.append(t)
        at = jnp.concatenate(a, axis=0).T
        parts = [at[i * 8:(i + 1) * 8] for i in range(16)]
        while len(parts) > 1:
            parts = [parts[i] + parts[i + 1] for i in range(0, len(parts), 2)]
        return _rowsum(parts[0])

    for fb in range(NVF):
        gs[fb] = vpu_col(G32, fb)
        us[fb] = vpu_col(U32F, fb)
    hs = []
    for fb in range(NFB):
        g = (gs[fb] - mu * cg[fb]) * rs
        u = (us[fb] - mu * cu[fb]) * rs
        hs.append(_rb(g * jax.nn.sigmoid(g) * u))
    ys = [None] * NB
    for seg in (mfb[:len(mfb) - DLAST], mfb[len(mfb) - DLAST:] + list(range(NVF))):
        for b in range(NB):
            for fb in seg:
                ys[b] = _acc(ys[b], down_tile(hs, fb, b))
    finish([x3[b] + (xn3[b] + (xn3[b] * 0.0 + ys[b] * sg)) for b in range(NB)])


@jax.jit
def pallas_interleave_layers__compressed_kv_cla__moe_arch_mod__decode_kernel(
    A_x, A_c_kv, A_w_q, A_w_uk, A_w_uv, A_w_o, B_x, B_w_r, B_w_gate, B_w_up, B_w_down,
):
    hbm = pl.BlockSpec(memory_space=pltpu.HBM)
    vm = pltpu.VMEM
    one = lambda n: max(n, 1)
    return pl.pallas_call(
        _kernel,
        out_shape=jax.ShapeDtypeStruct((1, 1, M), BF16),
        in_specs=[hbm] * 10,
        scratch_shapes=[
            vm((1, 1, M), BF16), vm((M,), BF16),
            vm((M * H, D), BF16), vm((DC * H, D), BF16), vm((NCB, SK, 128), BF16),
            vm((DC * H, D), BF16), vm((H * D, M), BF16),
            vm((FF, M), BF16), vm((FF, M), BF16), vm((FF, M), BF16),
            vm((NB, H * 64, 128), U32), vm((16, 512, 128), U32), vm((NKB, DC // 2, 128), U32),
            vm((H, DC // 2, 128), U32), vm((NFB, M // 2, 128), U32), vm((NFB, M // 2, 128), U32),
            vm((one(HQ) * NB, 128, 128), F32), vm((one(HQ) * NCB, 128, 128), F32),
            vm((one(HV) * NCB, 128, 128), F32), vm((one(HV) * D, M), F32),
            vm((NB, (H - HV) * 64, 128), U32),
            vm((one(NVF) * 128, M), F32), vm((one(NVF) * 128, M), F32),
            vm((one(HQ) * 16, 8, 128), F32), vm((N_PIN, 8, 128), F32),
            pltpu.SemaphoreType.DMA((N_SEM,)),
        ],
        compiler_params=pltpu.CompilerParams(
            vmem_limit_bytes=110 * 1024 * 1024, disable_semaphore_checks=True),
        name="cla_moe_decode",
    )(A_x, A_w_q.reshape(M * H, D), A_w_uk.reshape(DC * H, D), A_c_kv.reshape(SK, DC),
      A_w_uv.reshape(DC * H, D), A_w_o.reshape(H * D, M), B_w_r, B_w_gate.T, B_w_up.T, B_w_down)
```

```python
import os
import jax
import numpy as np
import jax.numpy as jnp
import jax.experimental.pallas as pl
import jax.experimental.pallas.tpu as pltpu

F32 = jnp.float32
BF16 = jnp.bfloat16
U32 = jnp.uint32
U16 = jnp.uint16
I32 = jnp.int32

M, H, D, SK, DC, FF = 640, 32, 128, 4096, 512, 1728
NB = M // 128
NCB = DC // 128
NKB = SK // 128
NFB = (FF + 127) // 128
EPS = 1e-5

E = os.environ.get
HQ = int(E('HQ', '12'))
QBACK = int(E('QBACK', '5'))
QDEF = int(E('QDEF', '8'))
HV = int(E('HV', '17'))
VBACK = int(E('VBACK', '3'))
S6LAST = int(E('S6LAST', '8'))
NVF = int(E('NVF', '6'))
NF0 = int(E('NF0', '3'))
DLAST = int(E('DLAST', '1'))
FBACK = int(E('FBACK', '0'))
DORD = int(E('DORD', '1'))
DTAIL = int(E('DTAIL', '0'))
KB0 = int(E('KB0', '6'))
S2ORD = int(E('S2ORD', '12'))
VITER = int(E('VITER', '2'))
STOP = E('STOP', '')
WO_SPLIT = [int(t) for t in E('WOSPLIT', '16,24').split(',') if t]
WD_SPLIT = [int(t) for t in E('WDSPLIT', '2,4').split(',') if t]
N_PIN = 176
N_SEM = 18


def _rb(x):
    return x.astype(BF16).astype(F32)


def _dot(a, b):
    return jax.lax.dot_general(a, b, (((1,), (0,)), ((), ())), preferred_element_type=F32)


def _acc(a, t):
    return t if a is None else a + t


def _stats(parts):
    s = parts[0]
    for p in parts[1:]:
        s = s + p
    m = jnp.sum(s, axis=1, keepdims=True) * (1.0 / M)
    c = [p - m for p in parts]
    v = c[0] * c[0]
    for p in c[1:]:
        v = v + p * p
    v = jnp.sum(v, axis=1, keepdims=True) * (1.0 / M)
    return m, jax.lax.rsqrt(v + EPS)


def _ln(parts):
    m, r = _stats(parts)
    return [(p - m) * r for p in parts]


def _rowsum(a):
    return jnp.broadcast_to(jnp.sum(a, axis=0, keepdims=True), (8, 128))


def _lanesum(a):
    return jnp.broadcast_to(jnp.sum(a, axis=1, keepdims=True), (8, 128))


def _kernel(x_hbm, wq_hbm, wuk_hbm, ckv_hbm, wuv_hbm, wo_hbm, wr_hbm, g_hbm, u_hbm, wd_hbm,
            o_ref,
            x_v, wr_v, wq_v, wuk_v, ckv_v, wuv_v, wo_v, g_v, u_v, wd_v,
            WQ, WKT, CT, WV, GT, UT,
            WQT32, WKT32, WVT32, WO32, WOT, G32, U32F, AE, PIN, sems):
    cps = {}

    def add(name, src, dst):
        cps[name] = pltpu.make_async_copy(src, dst, sems.at[len(cps)])

    add('wq', wq_hbm, wq_v)
    add('x', x_hbm, x_v)
    add('wr', wr_hbm, wr_v)
    add('wuk', wuk_hbm, wuk_v)
    for j in range(NCB):
        add(f'ckv{j}', ckv_hbm.at[:, pl.ds(128 * j, 128)], ckv_v.at[j])
    add('g', g_hbm, g_v)
    add('u', u_hbm, u_v)
    add('wuv', wuv_hbm, wuv_v)
    wo_b = [0] + WO_SPLIT + [H]
    for i in range(len(wo_b) - 1):
        sl = pl.ds(wo_b[i] * D, (wo_b[i + 1] - wo_b[i]) * D)
        add(f'wo{i}', wo_hbm.at[sl], wo_v.at[sl])
    wd_b = [0] + WD_SPLIT + [NB]
    for i in range(len(wd_b) - 1):
        sl = pl.ds(wd_b[i] * 128, (wd_b[i + 1] - wd_b[i]) * 128)
        add(f'wd{i}', wd_hbm.at[:, sl], wd_v.at[:, sl])
    assert len(cps) <= N_SEM
    for c in cps.values():
        c.start()
    waited = set()

    def wait(name):
        if name not in waited:
            cps[name].wait()
            waited.add(name)

    pin_n = [0]

    def pin(vals, *names):
        k0 = pin_n[0]
        for i, v in enumerate(vals):
            PIN[k0 + i] = v
        pin_n[0] += len(vals)
        assert pin_n[0] <= N_PIN
        for nm in names:
            wait(nm)
        return [PIN[k0 + i] for i in range(len(vals))]

    wq_u, wuk_u, wuv_u, ckv_u = (r.bitcast(U32) for r in (wq_v, wuk_v, wuv_v, ckv_v))

    def ld(uref, idx, r0, nrows):
        return pltpu.bitcast(uref[(*idx, pl.ds(r0 // 2, nrows // 2), slice(None))], BF16)

    def shuf(src_u, r0, s):
        a = src_u[pl.ds(r0 * 16 + s, 8, stride=16), :]
        b = src_u[pl.ds((r0 + 8) * 16 + s, 8, stride=16), :]
        xx = jnp.concatenate([a, b], axis=0)
        lo = pltpu.bitcast(xx.astype(U16), U32)
        hi = pltpu.bitcast((xx >> 16).astype(U16), U32)
        return lo, hi

    def relayout_q():
        for i in range(M // 16):
            b, m16 = divmod(i, 8)
            for s in range(16):
                lo, hi = shuf(wq_u, i * 16, s)
                WQ[b, pl.ds(2 * s * 64 + m16 * 8, 8), :] = lo
                WQ[b, pl.ds((2 * s + 1) * 64 + m16 * 8, 8), :] = hi
        for h in range(HQ):
            for b in range(NB):
                WQT32[h * NB + b] = ld(WQ, (b,), h * 128, 128).T.astype(F32)

    def relayout_k():
        for cb in range(NCB):
            for s in range(16):
                los, his = [], []
                for i in range(8):
                    lo, hi = shuf(wuk_u, cb * 128 + i * 16, s)
                    los.append(lo)
                    his.append(hi)
                for h, parts in ((2 * s, los), (2 * s + 1, his)):
                    t = pltpu.bitcast(jnp.concatenate(parts, axis=0), BF16).T
                    WKT[(h // 8) * 4 + cb, pl.ds((h % 8) * 64, 64), :] = pltpu.bitcast(t, U32)
                    if h < HQ:
                        WKT32[h * NCB + cb] = t.astype(F32)

    def relayout_c():
        for cb in range(NCB):
            wait(f'ckv{cb}')
            for kb in range(NKB):
                t = ld(ckv_u, (cb,), kb * 128, 128).T
                CT[kb, pl.ds(cb * 64, 64), :] = pltpu.bitcast(t, U32)

    def relayout_f(src, dst, dst32):
        for fb in range(NFB):
            for b in range(NB):
                if fb < NFB - 1:
                    t = src[pl.ds(fb * 128, 128), pl.ds(b * 128, 128)]
                else:
                    t = src[pl.ds(fb * 128, 64), pl.ds(b * 128, 128)]
                    t = jnp.concatenate([t, jnp.zeros((64, 128), BF16)], axis=0)
                dst[fb, pl.ds(b * 64, 64), :] = pltpu.bitcast(t.T, U32)
        for r in range(NVF * 16):
            dst32[pl.ds(r * 8, 8), :] = src[pl.ds(r * 8, 8), :].astype(F32)

    def relayout_v():
        for i in range(DC // 16):
            for s in range(16):
                lo, hi = shuf(wuv_u, i * 16, s)
                WV[2 * s, pl.ds(i * 8, 8), :] = lo
                WV[2 * s + 1, pl.ds(i * 8, 8), :] = hi
        if HV:
            per = -(-HV // VITER)

            def body(it, _):
                for k in range(per):
                    h = jnp.minimum(it * per + k, HV - 1)
                    for cb in range(NCB):
                        WVT32[h * NCB + cb] = ld(WV, (h,), cb * 128, 128).T.astype(F32)
                return 0
            jax.lax.fori_loop(0, VITER, body, 0)

    def relayout_o(h0, h1):
        for h in range(h0, h1):
            if h < HV:
                for i in range(16):
                    WO32[pl.ds(h * D + i * 8, 8), :] = wo_v[pl.ds(h * D + i * 8, 8), :].astype(F32)
            else:
                for b in range(NB):
                    WOT[b, pl.ds((h - HV) * 64, 64), :] = pltpu.bitcast(
                        wo_v[pl.ds(h * D, D), pl.ds(b * 128, 128)], U32)

    row8 = jax.lax.broadcasted_iota(I32, (8, 128), 0)

    def row_sel(v, j):
        return jnp.where(row8 == j, v, 0.0)

    def bd(v):
        return jnp.concatenate([row_sel(v, j) for j in range(8)], axis=1)

    def always(v):
        return (pltpu.bitcast(v, I32) | 1) != 0

    scale = D ** -0.5

    def softmax_ctx(qa, kb0=0):
        nblk = 2
        per = NKB // nblk
        sall = [None] * NKB
        qc = [qa[:, cb * 128:(cb + 1) * 128] for cb in range(NCB)]
        for cb in range(NCB):
            for kb in range(kb0):
                sall[kb] = _acc(sall[kb], _dot(qc[cb], ld(CT, (kb,), cb * 128, 128)))
        for kb in range(kb0, NKB):
            sall[kb] = _dot(qa, ld(CT, (kb,), 0, DC))
        ss = [sall[blk * per:(blk + 1) * per] for blk in range(nblk)]
        m_run = l_run = acc = None
        for blk in range(nblk):
            s = ss[blk]
            mx = s[0]
            for t in s[1:]:
                mx = jnp.maximum(mx, t)
            mx = jnp.max(mx, axis=1, keepdims=True)
            if m_run is not None:
                mx = jnp.maximum(mx, m_run)
            p = [jnp.exp((t - mx) * scale) for t in s]
            l = p[0]
            for t in p[1:]:
                l = l + t
            pb = jnp.concatenate([t.astype(BF16) for t in p], axis=1)
            cc = [_dot(pb, ld(ckv_u, (cb,), blk * per * 128, per * 128)) for cb in range(NCB)]
            if m_run is not None:
                al = jnp.exp((m_run - mx) * scale)
                cc = [c + a * al for c, a in zip(cc, acc)]
                l = l + l_run * al
            m_run, l_run, acc = mx, l, cc
        return acc, 1.0 / jnp.sum(l_run, axis=1, keepdims=True)

    def finish(x):
        o_ref[0] = jnp.concatenate([p[0:1] for p in x], axis=1).astype(BF16)
        for name in cps:
            wait(name)

    wait('x')
    wait('wr')
    x0 = jnp.broadcast_to(x_v[0].astype(F32), (8, M))
    x0 = [x0[:, b * 128:(b + 1) * 128] for b in range(NB)]
    wr = wr_v[...].reshape(1, M).astype(F32)

    def router(xn):
        r = None
        for b in range(NB):
            r = _acc(r, _rb(xn[b]) * wr[:, b * 128:(b + 1) * 128])
        return jax.nn.sigmoid(jnp.sum(r, axis=1, keepdims=True))

    xn = _ln(x0)
    wait('wq')
    relayout_q()
    ones_bd = bd(jnp.ones((8, 128), F32))
    q = [None] * 4
    for b in range(NB):
        lhs = jnp.concatenate([bd(xn[b]), ones_bd], axis=0)
        for g in range(4):
            q[g] = _acc(q[g], _dot(lhs, ld(WQ, (b,), g * 1024, 1024)))
    cs = [t[8:16] for t in q]
    q = [t[0:8] for t in q]
    t = pin(q + cs + x0, 'wuk')
    q, cs, x0 = t[:4], t[4:8], t[8:]
    relayout_k()
    qa, csk = [], []
    for g in range(4):
        lhs = jnp.concatenate([bd(q[g]), bd(cs[g])], axis=0)
        for cb in range(NCB):
            r = _dot(lhs, ld(WKT, (g * 4 + cb,), 0, 1024))
            qa.append(r[0:8])
            csk.append(r[8:16])
    t = pin(qa + csk, 'ckv0')
    qa, csk = t[:16], t[16:]
    qa = jnp.concatenate([jnp.concatenate(qa[g * 4:(g + 1) * 4], axis=1) for g in range(4)], axis=0)
    relayout_c()
    cc, inv = softmax_ctx(qa.astype(BF16))
    invb = jnp.broadcast_to(inv, (H, 128))
    t = pin([c[g * 8:(g + 1) * 8] for c in cc for g in range(4)]
            + [invb[g * 8:(g + 1) * 8] for g in range(4)], 'g')
    cc, inv = t[:16], t[16:]
    relayout_f(g_v, GT, G32)
    wait('u')
    relayout_f(u_v, UT, U32F)
    wait('wuv')
    relayout_v()
    ctx = []
    for g in range(4):
        lhs = jnp.concatenate([row_sel(cc[cb * 4 + g], j) for j in range(8) for cb in range(NCB)], axis=1)
        rhs = jnp.concatenate([ld(WV, (g * 8 + j,), 0, DC) for j in range(8)], axis=0)
        ctx.append(_dot(lhs, rhs) * inv[g])
    outs = [None] * NB
    for i in range(len(wo_b) - 1):
        if i == 0:
            ctx = pin(ctx, 'wo0')
        else:
            outs = pin(outs, f'wo{i}')
        hh = list(range(wo_b[i], wo_b[i + 1]))
        lhs = jnp.concatenate([row_sel(ctx[h // 8], h % 8) for h in hh], axis=1)
        for b in range(NB):
            outs[b] = _acc(outs[b], _dot(lhs, wo_v[pl.ds(hh[0] * D, len(hh) * D), pl.ds(b * 128, 128)]))
        relayout_o(wo_b[i], wo_b[i + 1])
    x1 = [a + _rowsum(o) for a, o in zip(x0, outs)]
    if STOP == 'A1':
        return finish(x1)

    xn1 = _ln(x1)
    sg = router(xn1)
    lhs = jnp.concatenate([jnp.concatenate(xn1, axis=1), jnp.ones((8, M), F32)], axis=0)
    hs, cg, cu = [], [], []
    for fb in range(NFB):
        g = _dot(lhs, ld(GT, (fb,), 0, M))
        u = _dot(lhs, ld(UT, (fb,), 0, M))
        cg.append(g[8:16])
        cu.append(u[8:16])
        g, u = g[0:8], u[0:8]
        hs.append(g * jax.nn.sigmoid(g) * u)
    base = [a + b for a, b in zip(x1, xn1)]

    def down_tile(hs, fb, b):
        if fb == NFB - 1:
            return _dot(hs[fb][:, :64], wd_v[pl.ds(fb * 128, 64), pl.ds(b * 128, 128)])
        return _dot(hs[fb], wd_v[pl.ds(fb * 128, 128), pl.ds(b * 128, 128)])

    x2, xp = [None] * NB, [None] * NB
    qraw = [None] * 4
    deferred = []
    pivot = None
    nseg = len(wd_b) - 1
    for i in range(nseg):
        if i == 0:
            t = pin(hs + base + xn1 + [jnp.broadcast_to(sg, (8, 128))] + cg + cu, 'wd0')
            hs, base, xn1, sg = t[:NFB], t[NFB:NFB + 5], t[NFB + 5:NFB + 10], t[NFB + 10]
            cg, cu = t[NFB + 11:2 * NFB + 11], t[2 * NFB + 11:]
        else:
            done = [b for b in range(NB) if x2[b] is not None]
            gl = [g for g in range(4) if qraw[g] is not None]
            t = pin([qraw[g] for g in gl] + [x2[b] for b in done] + [xp[b] for b in done]
                    + [jnp.broadcast_to(pivot, (8, 128))], f'wd{i}')
            for n_, g in enumerate(gl):
                qraw[g] = t[n_]
            for n_, b in enumerate(done):
                x2[b] = t[len(gl) + n_]
                xp[b] = t[len(gl) + len(done) + n_]
            pivot = t[-1]
        blks = list(range(wd_b[i], wd_b[i + 1]))
        for b in blks:
            y = None
            for fb in range(NFB):
                y = _acc(y, down_tile(hs, fb, b))
            x2[b] = base[b] + (xn1[b] * 0.0 + y * sg)
        if pivot is None:
            s = x2[blks[0]]
            for b in blks[1:]:
                s = s + x2[b]
            pivot = jnp.sum(s, axis=1, keepdims=True) * (1.0 / (128 * len(blks)))
        for b in blks:
            xp[b] = x2[b] - pivot
        todo = deferred + [(b, h) for b in blks for h in range(HQ, H)]
        deferred = []
        if i == nseg - 2 and QDEF:
            todo, deferred = todo[:-QDEF], todo[-QDEF:]
        for (b, h) in todo:
            qraw[h // 8] = _acc(qraw[h // 8], _dot(row_sel(xp[b], h % 8), ld(WQ, (b,), h * 128, 128)))
        if i < nseg - 1:
            for h in range(HQ):
                for r in range(16):
                    a = None if i == 0 else AE[h * 16 + r]
                    for b in blks:
                        a = _acc(a, WQT32[h * NB + b, pl.ds(r * 8, 8), :] * xp[b])
                    AE[h * 16 + r] = a
    if STOP == 'B1':
        return finish(x2)

    mu, rs = _stats(xp)
    qa = [[None] * NCB for _ in range(4)]
    s2 = [(h, cb) for h in range(HQ, H) for cb in range(NCB)]
    if S2ORD:
        s2 = s2[:S2ORD * NCB] + [(h, cb) for cb in range(NCB) for h in range(HQ + S2ORD, H)]
    for h, cb in s2:
        g = h // 8
        qa[g][cb] = _acc(qa[g][cb], _dot(row_sel(qraw[g], h % 8), ld(WKT, (g * 4 + cb,), (h % 8) * 128, 128)))
    tmask = always(xp[wd_b[-2]])
    zq = []
    for h in range(HQ):
        xr = {b: xp[b] for b in range(wd_b[-2], NB)}
        if QBACK and h >= QBACK:
            xr = {b: jnp.where(tmask, v, zq[h - QBACK]) for b, v in xr.items()}
        acc = [None] * NCB
        for r in range(16):
            a = AE[h * 16 + r]
            for b, v in xr.items():
                a = a + WQT32[h * NB + b, pl.ds(r * 8, 8), :] * v
            cv = _lanesum(a)
            for cb in range(NCB):
                acc[cb] = _acc(acc[cb], WKT32[h * NCB + cb, pl.ds(r * 8, 8), :] * cv)
        z = acc[0]
        for cb in range(1, NCB):
            z = jnp.maximum(z, acc[cb])
        zq.append(z)
        for cb in range(NCB):
            prev = qa[h // 8][cb]
            qa[h // 8][cb] = jnp.where(row8 == h % 8, _rowsum(acc[cb]), 0.0 if prev is None else prev) \
                if (h // 8) * 8 + 7 >= HQ or prev is not None else row_sel(_rowsum(acc[cb]), h % 8)
    qa = jnp.concatenate(
        [jnp.concatenate([(qa[g][cb] - mu * csk[g * 4 + cb]) * rs for cb in range(NCB)], axis=1)
         for g in range(4)], axis=0)
    cc, inv = softmax_ctx(qa.astype(BF16), KB0)

    invb = jnp.broadcast_to(inv, (H, 128))
    cn = [[cc[cb][g * 8:(g + 1) * 8] * invb[g * 8:(g + 1) * 8] for cb in range(NCB)] for g in range(4)]
    vmask = always(invb[0:8])
    accv = [None] * NB
    zv = []
    for h in range(HV):
        xr = [jnp.broadcast_to(cn[h // 8][cb][h % 8:h % 8 + 1], (8, 128)) for cb in range(NCB)]
        if VBACK and h >= VBACK:
            xr = [jnp.where(vmask, v, zv[h - VBACK]) for v in xr]
        for r in range(16):
            a = None
            for cb in range(NCB):
                a = _acc(a, WVT32[h * NCB + cb, pl.ds(r * 8, 8), :] * xr[cb])
            cv = _lanesum(a)
            for b in range(NB):
                accv[b] = _acc(accv[b], WO32[pl.ds(h * D + r * 8, 8), pl.ds(b * 128, 128)] * cv)
        z = accv[0]
        for b in range(1, NB):
            z = jnp.maximum(z, accv[b])
        zv.append(z)
    ctx = {}
    for g in range(HV // 8, 4):
        acc = None
        for h in range(max(HV, g * 8), g * 8 + 8):
            for cb in range(NCB):
                acc = _acc(acc, _dot(row_sel(cn[g][cb], h % 8), ld(WV, (h,), cb * 128, 128)))
        ctx[g] = acc
    mh = list(range(HV, H))
    lhs6 = {h: row_sel(ctx[h // 8], h % 8) for h in mh}
    outs = [None] * NB
    for seg in ([mh[:-S6LAST], mh[-S6LAST:]] if S6LAST else [mh]):
        for b in range(NB):
            for h in seg:
                outs[b] = _acc(outs[b], _dot(lhs6[h], ld(WOT, (b,), (h - HV) * 128, 128)))
    out = [_rowsum(o if a is None else o + a) for o, a in zip(outs, accv)]

    x3 = [a + b for a, b in zip(x2, out)]
    x3p = [a + b for a, b in zip(xp, out)]
    xb3 = x3p
    mu, rs = _stats(x3p)
    xn3 = [(t - mu) * rs for t in x3p]
    sg = router(xn3)
    gs, us = [None] * NFB, [None] * NFB
    mfb = list(range(NVF, NFB))
    for b in range(NB):
        for fb in mfb[:NF0]:
            gs[fb] = _acc(gs[fb], _dot(xb3[b], ld(GT, (fb,), b * 128, 128)))
            us[fb] = _acc(us[fb], _dot(xb3[b], ld(UT, (fb,), b * 128, 128)))
    for fb in mfb[NF0:]:
        for b in range(NB):
            gs[fb] = _acc(gs[fb], _dot(xb3[b], ld(GT, (fb,), b * 128, 128)))
        for b in range(NB):
            us[fb] = _acc(us[fb], _dot(xb3[b], ld(UT, (fb,), b * 128, 128)))

    fmask = always(x3p[0])
    link = []

    def vpu_col(W, fb):
        xr = x3p
        k = len(link)
        if FBACK and k >= FBACK:
            xr = [jnp.where(fmask, v, link[k - FBACK]) for v in xr]
        a = []
        for i in range(16):
            t = None
            for b in range(NB):
                t = _acc(t, W[pl.ds(fb * 128 + i * 8, 8), pl.ds(b * 128, 128)] * xr[b])
            a.append(t)
        link.append(_lanesum(a[15]))
        at = jnp.concatenate(a, axis=0).T
        parts = [at[i * 8:(i + 1) * 8] for i in range(16)]
        while len(parts) > 1:
            parts = [parts[i] + parts[i + 1] for i in range(0, len(parts), 2)]
        return _rowsum(parts[0])

    for fb in range(NVF):
        gs[fb] = vpu_col(G32, fb)
        us[fb] = vpu_col(U32F, fb)
    hs = []
    for fb in range(NFB):
        g = (gs[fb] - mu * cg[fb]) * rs
        u = (us[fb] - mu * cu[fb]) * rs
        hs.append(g * jax.nn.sigmoid(g) * u)
    ys = [None] * NB
    if DORD == 0:
        for seg in (mfb[:len(mfb) - DLAST], mfb[len(mfb) - DLAST:] + list(range(NVF))):
            for b in range(NB):
                for fb in seg:
                    ys[b] = _acc(ys[b], down_tile(hs, fb, b))
    else:
        for b in range(NB):
            for fb in mfb[:len(mfb) - DLAST]:
                ys[b] = _acc(ys[b], down_tile(hs, fb, b))
        late = mfb[len(mfb) - DLAST:] + list(range(NVF))
        nfo = len(late) - DTAIL
        for fb in late[:nfo]:
            for b in range(NB):
                ys[b] = _acc(ys[b], down_tile(hs, fb, b))
        for b in range(NB):
            for fb in late[nfo:]:
                ys[b] = _acc(ys[b], down_tile(hs, fb, b))
    finish([x3[b] + (xn3[b] + (xn3[b] * 0.0 + ys[b] * sg)) for b in range(NB)])


@jax.jit
def pallas_interleave_layers__compressed_kv_cla__moe_arch_mod__decode_kernel(
    A_x, A_c_kv, A_w_q, A_w_uk, A_w_uv, A_w_o, B_x, B_w_r, B_w_gate, B_w_up, B_w_down,
):
    hbm = pl.BlockSpec(memory_space=pltpu.HBM)
    vm = pltpu.VMEM
    one = lambda n: max(n, 1)
    return pl.pallas_call(
        _kernel,
        out_shape=jax.ShapeDtypeStruct((1, 1, M), BF16),
        in_specs=[hbm] * 10,
        scratch_shapes=[
            vm((1, 1, M), BF16), vm((M,), BF16),
            vm((M * H, D), BF16), vm((DC * H, D), BF16), vm((NCB, SK, 128), BF16),
            vm((DC * H, D), BF16), vm((H * D, M), BF16),
            vm((FF, M), BF16), vm((FF, M), BF16), vm((FF, M), BF16),
            vm((NB, H * 64, 128), U32), vm((16, 512, 128), U32), vm((NKB, DC // 2, 128), U32),
            vm((H, DC // 2, 128), U32), vm((NFB, M // 2, 128), U32), vm((NFB, M // 2, 128), U32),
            vm((one(HQ) * NB, 128, 128), F32), vm((one(HQ) * NCB, 128, 128), F32),
            vm((one(HV) * NCB, 128, 128), F32), vm((one(HV) * D, M), F32),
            vm((NB, (H - HV) * 64, 128), U32),
            vm((one(NVF) * 128, M), F32), vm((one(NVF) * 128, M), F32),
            vm((one(HQ) * 16, 8, 128), F32), vm((N_PIN, 8, 128), F32),
            pltpu.SemaphoreType.DMA((N_SEM,)),
        ],
        compiler_params=pltpu.CompilerParams(
            vmem_limit_bytes=110 * 1024 * 1024, disable_semaphore_checks=True),
        name="cla_moe_decode",
    )(A_x, A_w_q.reshape(M * H, D), A_w_uk.reshape(DC * H, D), A_c_kv.reshape(SK, DC),
      A_w_uv.reshape(DC * H, D), A_w_o.reshape(H * D, M), B_w_r, B_w_gate.T, B_w_up.T, B_w_down)
```

```python
import jax
import numpy as np
import jax.numpy as jnp
import jax.experimental.pallas as pl
import jax.experimental.pallas.tpu as pltpu

F32 = jnp.float32
BF16 = jnp.bfloat16
U32 = jnp.uint32
U16 = jnp.uint16
I32 = jnp.int32

M, H, D, SK, DC, FF = 640, 32, 128, 4096, 512, 1728
NB = M // 128
NCB = DC // 128
NKB = SK // 128
NFB = (FF + 127) // 128
EPS = 1e-5

HQ, QBACK = 12, 5
HV, VBACK = 17, 3
NVF = 6
NY = 10
QDEF, KB0, S2ORD, S6LAST, NF0, DLAST = 4, 6, 12, 8, 3, 1
WO_SPLIT = [16, 24]
WD_SPLIT = [2, 4]
PAD = 32
N_PIN = 176
N_SEM = 17


def _rb(x):
    return x.astype(BF16).astype(F32)


def _dot(a, b):
    return jax.lax.dot_general(a, b, (((1,), (0,)), ((), ())), preferred_element_type=F32)


def _acc(a, t):
    return t if a is None else a + t


def _stats(parts):
    s = parts[0]
    for p in parts[1:]:
        s = s + p
    m = jnp.sum(s, axis=1, keepdims=True) * (1.0 / M)
    c = [p - m for p in parts]
    v = c[0] * c[0]
    for p in c[1:]:
        v = v + p * p
    v = jnp.sum(v, axis=1, keepdims=True) * (1.0 / M)
    return m, jax.lax.rsqrt(v + EPS)


def _ln(parts):
    m, r = _stats(parts)
    return [(p - m) * r for p in parts]


def _rowsum(a):
    return jnp.broadcast_to(jnp.sum(a, axis=0, keepdims=True), (8, 128))


def _lanesum(a):
    return jnp.broadcast_to(jnp.sum(a, axis=1, keepdims=True), (8, 128))


def _kernel(x_hbm, wq_hbm, wuk_hbm, ckv_hbm, wuv_hbm, wo_hbm, wr_hbm, g_hbm, u_hbm, wd_hbm,
            o_ref,
            x_v, wr_v, wq_v, wuk_v, ckv_v, wuv_v, wo_v, g_v, u_v, wd_v,
            WQ, WKT, CT, WV, GT, UT,
            WQT32, WKT32, WVT32, WO32, WOT, G32, U32F, AE, HC, PIN, sems):
    cps = {}

    def add(name, src, dst):
        cps[name] = pltpu.make_async_copy(src, dst, sems.at[len(cps)])

    add('wq', wq_hbm, wq_v.at[pl.ds(0, M * H)])
    add('x', x_hbm, x_v)
    add('wr', wr_hbm, wr_v)
    add('wuk', wuk_hbm, wuk_v.at[pl.ds(0, DC * H)])
    for j in range(NCB):
        add(f'ckv{j}', ckv_hbm.at[:, pl.ds(128 * j, 128)], ckv_v.at[j])
    add('g', g_hbm, g_v)
    add('u', u_hbm, u_v)
    add('wuv', wuv_hbm, wuv_v.at[pl.ds(0, DC * H)])
    wo_b = [0] + WO_SPLIT + [H]
    for i in range(len(wo_b) - 1):
        sl = pl.ds(wo_b[i] * D, (wo_b[i + 1] - wo_b[i]) * D)
        add(f'wo{i}', wo_hbm.at[sl], wo_v.at[sl])
    wd_b = [0] + WD_SPLIT + [NB]
    for i in range(len(wd_b) - 1):
        sl = pl.ds(wd_b[i] * 128, (wd_b[i + 1] - wd_b[i]) * 128)
        add(f'wd{i}', wd_hbm.at[:, sl], wd_v.at[:, sl])
    assert len(cps) <= N_SEM
    for c in cps.values():
        c.start()
    waited = set()

    def wait(name):
        if name not in waited:
            cps[name].wait()
            waited.add(name)

    pin_n = [0]

    def pin(vals, *names):
        k0 = pin_n[0]
        for i, v in enumerate(vals):
            PIN[k0 + i] = v
        pin_n[0] += len(vals)
        assert pin_n[0] <= N_PIN
        for nm in names:
            wait(nm)
        return [PIN[k0 + i] for i in range(len(vals))]

    wq_u, wuk_u, wuv_u, ckv_u = (r.bitcast(U32) for r in (wq_v, wuk_v, wuv_v, ckv_v))

    def ld(uref, idx, r0, nrows):
        return pltpu.bitcast(uref[(*idx, pl.ds(r0 // 2, nrows // 2), slice(None))], BF16)

    def shuf(src_u, r0, s):
        a = src_u[pl.ds(r0 * 16 + s, 8, stride=16), :]
        b = src_u[pl.ds((r0 + 8) * 16 + s, 8, stride=16), :]
        xx = jnp.concatenate([a, b], axis=0)
        lo = pltpu.bitcast(xx.astype(U16), U32)
        hi = pltpu.bitcast((xx >> 16).astype(U16), U32)
        return lo, hi

    def relayout_q():
        for i in range(M // 16):
            b, m16 = divmod(i, 8)
            for s in range(16):
                lo, hi = shuf(wq_u, i * 16, s)
                WQ[b, pl.ds(2 * s * 64 + m16 * 8, 8), :] = lo
                WQ[b, pl.ds((2 * s + 1) * 64 + m16 * 8, 8), :] = hi
        for h in range(HQ):
            for b in range(NB):
                WQT32[h * NB + b] = ld(WQ, (b,), h * 128, 128).T.astype(F32)

    def relayout_k():
        for cb in range(NCB):
            for s in range(16):
                los, his = [], []
                for i in range(8):
                    lo, hi = shuf(wuk_u, cb * 128 + i * 16, s)
                    los.append(lo)
                    his.append(hi)
                for h, parts in ((2 * s, los), (2 * s + 1, his)):
                    t = pltpu.bitcast(jnp.concatenate(parts, axis=0), BF16).T
                    WKT[(h // 8) * 4 + cb, pl.ds((h % 8) * 64, 64), :] = pltpu.bitcast(t, U32)
                    if h < HQ:
                        WKT32[h * NCB + cb] = t.astype(F32)

    def relayout_c():
        for cb in range(NCB):
            wait(f'ckv{cb}')
            for kb in range(NKB):
                t = ld(ckv_u, (cb,), kb * 128, 128).T
                CT[kb, pl.ds(cb * 64, 64), :] = pltpu.bitcast(t, U32)

    def relayout_f(src, dst, dst32):
        for fb in range(NFB):
            for b in range(NB):
                if fb < NFB - 1:
                    t = src[pl.ds(fb * 128, 128), pl.ds(b * 128, 128)]
                else:
                    t = src[pl.ds(fb * 128, 64), pl.ds(b * 128, 128)]
                    t = jnp.concatenate([t, jnp.zeros((64, 128), BF16)], axis=0)
                dst[fb, pl.ds(b * 64, 64), :] = pltpu.bitcast(t.T, U32)
        for r in range(NVF * 16):
            dst32[pl.ds(r * 8, 8), :] = src[pl.ds(r * 8, 8), :].astype(F32)

    def relayout_v():
        for i in range(DC // 16):
            for s in range(16):
                lo, hi = shuf(wuv_u, i * 16, s)
                WV[2 * s, pl.ds(i * 8, 8), :] = lo
                WV[2 * s + 1, pl.ds(i * 8, 8), :] = hi
        if HV:
            per = -(-HV // 2)

            def body(it, _):
                for k in range(per):
                    h = jnp.minimum(it * per + k, HV - 1)
                    for cb in range(NCB):
                        WVT32[h * NCB + cb] = ld(WV, (h,), cb * 128, 128).T.astype(F32)
                return 0
            jax.lax.fori_loop(0, 2, body, 0)

    def relayout_o(h0, h1):
        for h in range(h0, h1):
            if h < HV:
                for i in range(16):
                    WO32[pl.ds(h * D + i * 8, 8), :] = wo_v[pl.ds(h * D + i * 8, 8), :].astype(F32)
            else:
                for b in range(NB):
                    WOT[b, pl.ds((h - HV) * 64, 64), :] = pltpu.bitcast(
                        wo_v[pl.ds(h * D, D), pl.ds(b * 128, 128)], U32)

    row8 = jax.lax.broadcasted_iota(I32, (8, 128), 0)

    def row_sel(v, j):
        return jnp.where(row8 == j, v, 0.0)

    def bd(v):
        return jnp.concatenate([row_sel(v, j) for j in range(8)], axis=1)

    def always(v):
        return (pltpu.bitcast(v, I32) | 1) != 0

    scale = D ** -0.5

    def softmax_ctx(qa, kb0=0):
        nblk = 2
        per = NKB // nblk
        sall = [None] * NKB
        qc = [qa[:, cb * 128:(cb + 1) * 128] for cb in range(NCB)]
        for cb in range(NCB):
            for kb in range(kb0):
                sall[kb] = _acc(sall[kb], _dot(qc[cb], ld(CT, (kb,), cb * 128, 128)))
        for kb in range(kb0, NKB):
            sall[kb] = _dot(qa, ld(CT, (kb,), 0, DC))
        ss = [sall[blk * per:(blk + 1) * per] for blk in range(nblk)]
        m_run = l_run = acc = None
        for blk in range(nblk):
            s = ss[blk]
            mx = s[0]
            for t in s[1:]:
                mx = jnp.maximum(mx, t)
            mx = jnp.max(mx, axis=1, keepdims=True)
            if m_run is not None:
                mx = jnp.maximum(mx, m_run)
            p = [jnp.exp((t - mx) * scale) for t in s]
            l = p[0]
            for t in p[1:]:
                l = l + t
            pb = jnp.concatenate([t.astype(BF16) for t in p], axis=1)
            cc = [_dot(pb, ld(ckv_u, (cb,), blk * per * 128, per * 128)) for cb in range(NCB)]
            if m_run is not None:
                al = jnp.exp((m_run - mx) * scale)
                cc = [c + a * al for c, a in zip(cc, acc)]
                l = l + l_run * al
            m_run, l_run, acc = mx, l, cc
        return acc, 1.0 / jnp.sum(l_run, axis=1, keepdims=True)

    def finish(x):
        for b in range(NB):
            o_ref[0, :, pl.ds(b * 128, 128)] = x[b][0:1].astype(BF16)
        for name in cps:
            wait(name)

    wait('x')
    wait('wr')
    x0 = jnp.broadcast_to(x_v[0].astype(F32), (8, M))
    x0 = [x0[:, b * 128:(b + 1) * 128] for b in range(NB)]
    wr = wr_v[...].reshape(1, M).astype(F32)

    def router(xn):
        r = None
        for b in range(NB):
            r = _acc(r, _rb(xn[b]) * wr[:, b * 128:(b + 1) * 128])
        return jax.nn.sigmoid(jnp.sum(r, axis=1, keepdims=True))

    xn = _ln(x0)
    wait('wq')
    relayout_q()
    ones_bd = bd(jnp.ones((8, 128), F32))
    q = [None] * 4
    for b in range(NB):
        lhs = jnp.concatenate([bd(xn[b]), ones_bd], axis=0)
        for g in range(4):
            q[g] = _acc(q[g], _dot(lhs, ld(WQ, (b,), g * 1024, 1024)))
    cs = [t[8:16] for t in q]
    q = [t[0:8] for t in q]
    t = pin(q + cs + x0, 'wuk')
    q, cs, x0 = t[:4], t[4:8], t[8:]
    relayout_k()
    qa, csk = [], []
    for g in range(4):
        lhs = jnp.concatenate([bd(q[g]), bd(cs[g])], axis=0)
        for cb in range(NCB):
            r = _dot(lhs, ld(WKT, (g * 4 + cb,), 0, 1024))
            qa.append(r[0:8])
            csk.append(r[8:16])
    t = pin(qa + csk, 'ckv0')
    qa, csk = t[:16], t[16:]
    qa = jnp.concatenate([jnp.concatenate(qa[g * 4:(g + 1) * 4], axis=1) for g in range(4)], axis=0)
    relayout_c()
    cc, inv = softmax_ctx(qa.astype(BF16))
    invb = jnp.broadcast_to(inv, (H, 128))
    t = pin([c[g * 8:(g + 1) * 8] for c in cc for g in range(4)]
            + [invb[g * 8:(g + 1) * 8] for g in range(4)], 'g')
    cc, inv = t[:16], t[16:]
    relayout_f(g_v, GT, G32)
    wait('u')
    relayout_f(u_v, UT, U32F)
    wait('wuv')
    relayout_v()
    ctx = []
    for g in range(4):
        lhs = jnp.concatenate([row_sel(cc[cb * 4 + g], j) for j in range(8) for cb in range(NCB)], axis=1)
        rhs = jnp.concatenate([ld(WV, (g * 8 + j,), 0, DC) for j in range(8)], axis=0)
        ctx.append(_dot(lhs, rhs) * inv[g])
    outs = [None] * NB
    for i in range(len(wo_b) - 1):
        if i == 0:
            ctx = pin(ctx, 'wo0')
        else:
            outs = pin(outs, f'wo{i}')
        hh = list(range(wo_b[i], wo_b[i + 1]))
        lhs = jnp.concatenate([row_sel(ctx[h // 8], h % 8) for h in hh], axis=1)
        for b in range(NB):
            outs[b] = _acc(outs[b], _dot(lhs, wo_v[pl.ds(hh[0] * D, len(hh) * D), pl.ds(b * 128, 128)]))
        relayout_o(wo_b[i], wo_b[i + 1])
    x1 = [a + _rowsum(o) for a, o in zip(x0, outs)]

    xn1 = _ln(x1)
    sg = router(xn1)
    lhs = jnp.concatenate([jnp.concatenate(xn1, axis=1), jnp.ones((8, M), F32)], axis=0)
    hs, cg, cu = [], [], []
    for fb in range(NFB):
        g = _dot(lhs, ld(GT, (fb,), 0, M))
        u = _dot(lhs, ld(UT, (fb,), 0, M))
        cg.append(g[8:16])
        cu.append(u[8:16])
        g, u = g[0:8], u[0:8]
        hs.append(g * jax.nn.sigmoid(g) * u)
    base = [a + b for a, b in zip(x1, xn1)]

    def down_tile(hs, fb, b):
        if fb == NFB - 1:
            return _dot(hs[fb][:, :64], wd_v[pl.ds(fb * 128, 64), pl.ds(b * 128, 128)])
        return _dot(hs[fb], wd_v[pl.ds(fb * 128, 128), pl.ds(b * 128, 128)])

    x2, xp = [None] * NB, [None] * NB
    qraw = [None] * 4
    deferred = []
    pivot = None
    nseg = len(wd_b) - 1
    for i in range(nseg):
        if i == 0:
            t = pin(hs + base + xn1 + [jnp.broadcast_to(sg, (8, 128))] + cg + cu, 'wd0')
            hs, base, xn1, sg = t[:NFB], t[NFB:NFB + 5], t[NFB + 5:NFB + 10], t[NFB + 10]
            cg, cu = t[NFB + 11:2 * NFB + 11], t[2 * NFB + 11:]
        else:
            done = [b for b in range(NB) if x2[b] is not None]
            gl = [g for g in range(4) if qraw[g] is not None]
            t = pin([qraw[g] for g in gl] + [x2[b] for b in done] + [xp[b] for b in done]
                    + [jnp.broadcast_to(pivot, (8, 128))], f'wd{i}')
            for n_, g in enumerate(gl):
                qraw[g] = t[n_]
            for n_, b in enumerate(done):
                x2[b] = t[len(gl) + n_]
                xp[b] = t[len(gl) + len(done) + n_]
            pivot = t[-1]
        blks = list(range(wd_b[i], wd_b[i + 1]))
        if i == 0:
            for fb in range(NY):
                HC[pl.ds(fb * 128, 128), :] = jnp.broadcast_to(hs[fb][0:1], (128, 128)).T
        for b in blks:
            y = None
            nv = NY if i == nseg - 1 else 0
            for fb in range(nv, NFB):
                y = _acc(y, down_tile(hs, fb, b))
            if nv:
                parts = [None] * 4
                for r in range(nv * 16):
                    t = wd_v[pl.ds(r * 8, 8), pl.ds(b * 128, 128)].astype(F32) * HC[pl.ds(r * 8, 8), :]
                    parts[r % 4] = _acc(parts[r % 4], t)
                y = y + _rowsum((parts[0] + parts[1]) + (parts[2] + parts[3]))
            x2[b] = base[b] + (xn1[b] * 0.0 + y * sg)
        if pivot is None:
            s = x2[blks[0]]
            for b in blks[1:]:
                s = s + x2[b]
            pivot = jnp.sum(s, axis=1, keepdims=True) * (1.0 / (128 * len(blks)))
        for b in blks:
            xp[b] = x2[b] - pivot
        todo = deferred + [(b, h) for b in blks for h in range(HQ, H)]
        deferred = []
        if i == nseg - 2 and QDEF:
            todo, deferred = todo[:-QDEF], todo[-QDEF:]
        for (b, h) in todo:
            qraw[h // 8] = _acc(qraw[h // 8], _dot(row_sel(xp[b], h % 8), ld(WQ, (b,), h * 128, 128)))
        if i < nseg - 1:
            for h in range(HQ):
                for r in range(16):
                    a = None if i == 0 else AE[h * 16 + r]
                    for b in blks:
                        a = _acc(a, WQT32[h * NB + b, pl.ds(r * 8, 8), :] * xp[b])
                    AE[h * 16 + r] = a

    mu, rs = _stats(xp)
    xc = [t - mu for t in xp]
    qa = [[None] * NCB for _ in range(4)]
    s2 = [(h, cb) for h in range(HQ, H) for cb in range(NCB)]
    if S2ORD:
        s2 = s2[:S2ORD * NCB] + [(h, cb) for cb in range(NCB) for h in range(HQ + S2ORD, H)]
    for h, cb in s2:
        g = h // 8
        qa[g][cb] = _acc(qa[g][cb], _dot(row_sel(qraw[g], h % 8), ld(WKT, (g * 4 + cb,), (h % 8) * 128, 128)))
    tmask = always(xp[wd_b[-2]])
    zq = []
    for h in range(HQ):
        xr = {b: xp[b] for b in range(wd_b[-2], NB)}
        if QBACK and h >= QBACK:
            xr = {b: jnp.where(tmask, v, zq[h - QBACK]) for b, v in xr.items()}
        acc = [None] * NCB
        for r in range(16):
            a = AE[h * 16 + r]
            for b, v in xr.items():
                a = a + WQT32[h * NB + b, pl.ds(r * 8, 8), :] * v
            cv = _lanesum(a)
            for cb in range(NCB):
                acc[cb] = _acc(acc[cb], WKT32[h * NCB + cb, pl.ds(r * 8, 8), :] * cv)
        z = acc[0]
        for cb in range(1, NCB):
            z = jnp.maximum(z, acc[cb])
        zq.append(z)
        for cb in range(NCB):
            prev = qa[h // 8][cb]
            qa[h // 8][cb] = jnp.where(row8 == h % 8, _rowsum(acc[cb]), 0.0 if prev is None else prev) \
                if (h // 8) * 8 + 7 >= HQ or prev is not None else row_sel(_rowsum(acc[cb]), h % 8)
    qa = jnp.concatenate(
        [jnp.concatenate([(qa[g][cb] - mu * csk[g * 4 + cb]) * rs for cb in range(NCB)], axis=1)
         for g in range(4)], axis=0)
    cc, inv = softmax_ctx(qa.astype(BF16), KB0)

    invb = jnp.broadcast_to(inv, (H, 128))
    cn = [[cc[cb][g * 8:(g + 1) * 8] * invb[g * 8:(g + 1) * 8] for cb in range(NCB)] for g in range(4)]
    vmask = always(invb[0:8])
    accv = [None] * NB
    zv = []
    for h in range(HV):
        xr = [jnp.broadcast_to(cn[h // 8][cb][h % 8:h % 8 + 1], (8, 128)) for cb in range(NCB)]
        if VBACK and h >= VBACK:
            xr = [jnp.where(vmask, v, zv[h - VBACK]) for v in xr]
        for r in range(16):
            a = None
            for cb in range(NCB):
                a = _acc(a, WVT32[h * NCB + cb, pl.ds(r * 8, 8), :] * xr[cb])
            cv = _lanesum(a)
            for b in range(NB):
                accv[b] = _acc(accv[b], WO32[pl.ds(h * D + r * 8, 8), pl.ds(b * 128, 128)] * cv)
        z = accv[0]
        for b in range(1, NB):
            z = jnp.maximum(z, accv[b])
        zv.append(z)
    mh = list(range(HV, H))
    ctx = {}
    for g in range(HV // 8, 4):
        acc = None
        for h in range(max(HV, g * 8), g * 8 + 8):
            for cb in range(NCB):
                acc = _acc(acc, _dot(row_sel(cn[g][cb], h % 8), ld(WV, (h,), cb * 128, 128)))
        ctx[g] = acc
    lhs6 = {h: row_sel(ctx[h // 8], h % 8) for h in mh}
    outs = [None] * NB
    for seg in (mh[:-S6LAST], mh[-S6LAST:]):
        for b in range(NB):
            for h in seg:
                outs[b] = _acc(outs[b], _dot(lhs6[h], ld(WOT, (b,), (h - HV) * 128, 128)))
    out = [_rowsum(o if a is None else o + a) for o, a in zip(outs, accv)]

    x3 = [a + b for a, b in zip(x2, out)]
    x3p = [a + b for a, b in zip(xc, out)]
    mu, rs = _stats(x3p)
    xn3 = [(t - mu) * rs for t in x3p]
    sg = router(xn3)
    gs, us = [None] * NFB, [None] * NFB
    mfb = list(range(NVF, NFB))
    for b in range(NB):
        for fb in mfb[:NF0]:
            gs[fb] = _acc(gs[fb], _dot(x3p[b], ld(GT, (fb,), b * 128, 128)))
            us[fb] = _acc(us[fb], _dot(x3p[b], ld(UT, (fb,), b * 128, 128)))
    for fb in mfb[NF0:]:
        for b in range(NB):
            gs[fb] = _acc(gs[fb], _dot(x3p[b], ld(GT, (fb,), b * 128, 128)))
        for b in range(NB):
            us[fb] = _acc(us[fb], _dot(x3p[b], ld(UT, (fb,), b * 128, 128)))

    def vpu_col(W, fb):
        a = []
        for i in range(16):
            t = None
            for b in range(NB):
                t = _acc(t, W[pl.ds(fb * 128 + i * 8, 8), pl.ds(b * 128, 128)] * x3p[b])
            a.append(t)
        at = jnp.concatenate(a, axis=0).T
        parts = [at[i * 8:(i + 1) * 8] for i in range(16)]
        while len(parts) > 1:
            parts = [parts[i] + parts[i + 1] for i in range(0, len(parts), 2)]
        return _rowsum(parts[0])

    for fb in range(NVF):
        gs[fb] = vpu_col(G32, fb)
        us[fb] = vpu_col(U32F, fb)
    hs = []
    for fb in range(NFB):
        g = (gs[fb] - mu * cg[fb]) * rs
        u = (us[fb] - mu * cu[fb]) * rs
        hs.append(g * jax.nn.sigmoid(g) * u)
    ys = [None] * NB
    for b in range(NB):
        for fb in mfb[:-DLAST]:
            ys[b] = _acc(ys[b], down_tile(hs, fb, b))
    for fb in mfb[-DLAST:] + list(range(NVF)):
        for b in range(NB):
            ys[b] = _acc(ys[b], down_tile(hs, fb, b))
    base = [x3[b] + (xn3[b] + xn3[b] * 0.0) for b in range(NB)]
    finish([base[b] + ys[b] * sg for b in range(NB)])


@jax.jit
def pallas_interleave_layers__compressed_kv_cla__moe_arch_mod__decode_kernel(
    A_x, A_c_kv, A_w_q, A_w_uk, A_w_uv, A_w_o, B_x, B_w_r, B_w_gate, B_w_up, B_w_down,
):
    hbm = pl.BlockSpec(memory_space=pltpu.HBM)
    vm = pltpu.VMEM
    return pl.pallas_call(
        _kernel,
        out_shape=jax.ShapeDtypeStruct((1, 1, M), BF16),
        in_specs=[hbm] * 10,
        scratch_shapes=[
            vm((1, 1, M), BF16), vm((M,), BF16),
            vm((M * H + PAD, D), BF16), vm((DC * H + PAD, D), BF16), vm((NCB, SK, 128), BF16),
            vm((DC * H + PAD, D), BF16), vm((H * D, M), BF16),
            vm((FF, M), BF16), vm((FF, M), BF16), vm((FF, M), BF16),
            vm((NB, H * 64, 128), U32), vm((16, 512, 128), U32), vm((NKB, DC // 2, 128), U32),
            vm((H, DC // 2, 128), U32), vm((NFB, M // 2, 128), U32), vm((NFB, M // 2, 128), U32),
            vm((HQ * NB, 128, 128), F32), vm((HQ * NCB, 128, 128), F32),
            vm((HV * NCB, 128, 128), F32), vm((HV * D, M), F32),
            vm((NB, (H - HV) * 64, 128), U32),
            vm((NVF * 128, M), F32), vm((NVF * 128, M), F32),
            vm((HQ * 16, 8, 128), F32), vm((NY * 128, 128), F32), vm((N_PIN, 8, 128), F32),
            pltpu.SemaphoreType.DMA((N_SEM,)),
        ],
        compiler_params=pltpu.CompilerParams(
            vmem_limit_bytes=110 * 1024 * 1024, disable_semaphore_checks=True),
        name="cla_moe_decode",
    )(A_x, A_w_q.reshape(M * H, D), A_w_uk.reshape(DC * H, D), A_c_kv.reshape(SK, DC),
      A_w_uv.reshape(DC * H, D), A_w_o.reshape(H * D, M), B_w_r, B_w_gate.T, B_w_up.T, B_w_down)
```

```python
import jax
import numpy as np
import jax.numpy as jnp
import jax.experimental.pallas as pl
import jax.experimental.pallas.tpu as pltpu

F32 = jnp.float32
BF16 = jnp.bfloat16
U32 = jnp.uint32
U16 = jnp.uint16
I32 = jnp.int32

M, H, D, SK, DC, FF = 640, 32, 128, 4096, 512, 1728
NB = M // 128
NCB = DC // 128
NKB = SK // 128
NFB = (FF + 127) // 128
EPS = 1e-5

HQ, QBACK = 12, 5
HV, VBACK = 17, 3
NVF = 7
NY = 10
QDEF, KB0, S2ORD, S6LAST, NF0 = 4, 6, 12, 8, 3
WO_SPLIT = [16, 24]
WD_SPLIT = [2, 4]
PAD = 32
N_PIN = 176
N_SEM = 17


def _rb(x):
    return x.astype(BF16).astype(F32)


def _dot(a, b):
    return jax.lax.dot_general(a, b, (((1,), (0,)), ((), ())), preferred_element_type=F32)


def _acc(a, t):
    return t if a is None else a + t


def _stats(parts):
    s = parts[0]
    for p in parts[1:]:
        s = s + p
    m = jnp.sum(s, axis=1, keepdims=True) * (1.0 / M)
    c = [p - m for p in parts]
    v = c[0] * c[0]
    for p in c[1:]:
        v = v + p * p
    v = jnp.sum(v, axis=1, keepdims=True) * (1.0 / M)
    return m, jax.lax.rsqrt(v + EPS)


def _stats1(parts):
    s, v = parts[0], parts[0] * parts[0]
    for p in parts[1:]:
        s, v = s + p, v + p * p
    m = jnp.sum(s, axis=1, keepdims=True) * (1.0 / M)
    v = jnp.sum(v, axis=1, keepdims=True) * (1.0 / M) - m * m
    return m, jax.lax.rsqrt(jnp.maximum(v, 0.0) + EPS)


def _ln(parts):
    m, r = _stats(parts)
    return [(p - m) * r for p in parts]


def _rowsum(a):
    return jnp.broadcast_to(jnp.sum(a, axis=0, keepdims=True), (8, 128))


def _lanesum(a):
    return jnp.broadcast_to(jnp.sum(a, axis=1, keepdims=True), (8, 128))


def _kernel(x_hbm, wq_hbm, wuk_hbm, ckv_hbm, wuv_hbm, wo_hbm, wr_hbm, g_hbm, u_hbm, wd_hbm,
            o_ref,
            x_v, wr_v, wq_v, wuk_v, ckv_v, wuv_v, wo_v, g_v, u_v, wd_v,
            WQ, WKT, CT, WV, GT, UT,
            WQT32, WKT32, WVT32, WO32, WOT, G32, U32F, AE, HC, PIN, sems):
    cps = {}

    def add(name, src, dst):
        cps[name] = pltpu.make_async_copy(src, dst, sems.at[len(cps)])

    add('wq', wq_hbm, wq_v.at[pl.ds(0, M * H)])
    add('x', x_hbm, x_v)
    add('wr', wr_hbm, wr_v)
    add('wuk', wuk_hbm, wuk_v.at[pl.ds(0, DC * H)])
    for j in range(NCB):
        add(f'ckv{j}', ckv_hbm.at[:, pl.ds(128 * j, 128)], ckv_v.at[j])
    add('g', g_hbm, g_v)
    add('u', u_hbm, u_v)
    add('wuv', wuv_hbm, wuv_v.at[pl.ds(0, DC * H)])
    wo_b = [0] + WO_SPLIT + [H]
    for i in range(len(wo_b) - 1):
        sl = pl.ds(wo_b[i] * D, (wo_b[i + 1] - wo_b[i]) * D)
        add(f'wo{i}', wo_hbm.at[sl], wo_v.at[sl])
    wd_b = [0] + WD_SPLIT + [NB]
    for i in range(len(wd_b) - 1):
        sl = pl.ds(wd_b[i] * 128, (wd_b[i + 1] - wd_b[i]) * 128)
        add(f'wd{i}', wd_hbm.at[:, sl], wd_v.at[:, sl])
    assert len(cps) <= N_SEM
    for c in cps.values():
        c.start()
    waited = set()

    def wait(name):
        if name not in waited:
            cps[name].wait()
            waited.add(name)

    pin_n = [0]

    def pin(vals, *names):
        k0 = pin_n[0]
        for i, v in enumerate(vals):
            PIN[k0 + i] = v
        pin_n[0] += len(vals)
        assert pin_n[0] <= N_PIN
        for nm in names:
            wait(nm)
        return [PIN[k0 + i] for i in range(len(vals))]

    wq_u, wuk_u, wuv_u, ckv_u = (r.bitcast(U32) for r in (wq_v, wuk_v, wuv_v, ckv_v))

    def ld(uref, idx, r0, nrows):
        return pltpu.bitcast(uref[(*idx, pl.ds(r0 // 2, nrows // 2), slice(None))], BF16)

    def shuf(src_u, r0, s):
        a = src_u[pl.ds(r0 * 16 + s, 8, stride=16), :]
        b = src_u[pl.ds((r0 + 8) * 16 + s, 8, stride=16), :]
        xx = jnp.concatenate([a, b], axis=0)
        lo = pltpu.bitcast(xx.astype(U16), U32)
        hi = pltpu.bitcast((xx >> 16).astype(U16), U32)
        return lo, hi

    def relayout_q():
        for i in range(M // 16):
            b, m16 = divmod(i, 8)
            for s in range(16):
                lo, hi = shuf(wq_u, i * 16, s)
                WQ[b, pl.ds(2 * s * 64 + m16 * 8, 8), :] = lo
                WQ[b, pl.ds((2 * s + 1) * 64 + m16 * 8, 8), :] = hi
        for h in range(HQ):
            for b in range(NB):
                WQT32[h * NB + b] = ld(WQ, (b,), h * 128, 128).T.astype(F32)

    def relayout_k():
        for cb in range(NCB):
            for s in range(16):
                los, his = [], []
                for i in range(8):
                    lo, hi = shuf(wuk_u, cb * 128 + i * 16, s)
                    los.append(lo)
                    his.append(hi)
                for h, parts in ((2 * s, los), (2 * s + 1, his)):
                    t = pltpu.bitcast(jnp.concatenate(parts, axis=0), BF16).T
                    WKT[(h // 8) * 4 + cb, pl.ds((h % 8) * 64, 64), :] = pltpu.bitcast(t, U32)
                    if h < HQ:
                        WKT32[h * NCB + cb] = t.astype(F32)

    def relayout_c():
        for cb in range(NCB):
            wait(f'ckv{cb}')
            for kb in range(NKB):
                t = ld(ckv_u, (cb,), kb * 128, 128).T
                CT[kb, pl.ds(cb * 64, 64), :] = pltpu.bitcast(t, U32)

    def relayout_f(src, dst, dst32):
        for fb in range(NFB):
            for b in range(NB):
                if fb < NFB - 1:
                    t = src[pl.ds(fb * 128, 128), pl.ds(b * 128, 128)]
                else:
                    t = src[pl.ds(fb * 128, 64), pl.ds(b * 128, 128)]
                    t = jnp.concatenate([t, jnp.zeros((64, 128), BF16)], axis=0)
                dst[fb, pl.ds(b * 64, 64), :] = pltpu.bitcast(t.T, U32)
        for r in range(NVF * 16):
            dst32[pl.ds(r * 8, 8), :] = src[pl.ds(r * 8, 8), :].astype(F32)

    def relayout_v():
        for i in range(DC // 16):
            for s in range(16):
                lo, hi = shuf(wuv_u, i * 16, s)
                WV[2 * s, pl.ds(i * 8, 8), :] = lo
                WV[2 * s + 1, pl.ds(i * 8, 8), :] = hi
        if HV:
            per = -(-HV // 2)

            def body(it, _):
                for k in range(per):
                    h = jnp.minimum(it * per + k, HV - 1)
                    for cb in range(NCB):
                        WVT32[h * NCB + cb] = ld(WV, (h,), cb * 128, 128).T.astype(F32)
                return 0
            jax.lax.fori_loop(0, 2, body, 0)

    def relayout_o(h0, h1):
        for h in range(h0, h1):
            if h < HV:
                for i in range(16):
                    WO32[pl.ds(h * D + i * 8, 8), :] = wo_v[pl.ds(h * D + i * 8, 8), :].astype(F32)
            else:
                for b in range(NB):
                    WOT[b, pl.ds((h - HV) * 64, 64), :] = pltpu.bitcast(
                        wo_v[pl.ds(h * D, D), pl.ds(b * 128, 128)], U32)

    row8 = jax.lax.broadcasted_iota(I32, (8, 128), 0)

    def row_sel(v, j):
        return jnp.where(row8 == j, v, 0.0)

    def bd(v):
        return jnp.concatenate([row_sel(v, j) for j in range(8)], axis=1)

    def always(v):
        return (pltpu.bitcast(v, I32) | 1) != 0

    scale = D ** -0.5

    def softmax_ctx(qa, kb0=0):
        nblk = 2
        per = NKB // nblk
        sall = [None] * NKB
        qc = [qa[:, cb * 128:(cb + 1) * 128] for cb in range(NCB)]
        for cb in range(NCB):
            for kb in range(kb0):
                sall[kb] = _acc(sall[kb], _dot(qc[cb], ld(CT, (kb,), cb * 128, 128)))
        for kb in range(kb0, NKB):
            sall[kb] = _dot(qa, ld(CT, (kb,), 0, DC))
        ss = [sall[blk * per:(blk + 1) * per] for blk in range(nblk)]
        m_run = l_run = acc = None
        for blk in range(nblk):
            s = ss[blk]
            mx = s[0]
            for t in s[1:]:
                mx = jnp.maximum(mx, t)
            mx = jnp.max(mx, axis=1, keepdims=True)
            if m_run is not None:
                mx = jnp.maximum(mx, m_run)
            p = [jnp.exp((t - mx) * scale) for t in s]
            l = p[0]
            for t in p[1:]:
                l = l + t
            pb = jnp.concatenate([t.astype(BF16) for t in p], axis=1)
            cc = [_dot(pb, ld(ckv_u, (cb,), blk * per * 128, per * 128)) for cb in range(NCB)]
            if m_run is not None:
                al = jnp.exp((m_run - mx) * scale)
                cc = [c + a * al for c, a in zip(cc, acc)]
                l = l + l_run * al
            m_run, l_run, acc = mx, l, cc
        return acc, 1.0 / jnp.sum(l_run, axis=1, keepdims=True)

    def finish(x):
        for b in range(NB):
            o_ref[0, :, pl.ds(b * 128, 128)] = x[b][0:1].astype(BF16)
        for name in cps:
            wait(name)

    wait('x')
    wait('wr')
    x0 = jnp.broadcast_to(x_v[0].astype(F32), (8, M))
    x0 = [x0[:, b * 128:(b + 1) * 128] for b in range(NB)]
    wr = wr_v[...].reshape(1, M).astype(F32)

    def router(xn):
        r = None
        for b in range(NB):
            r = _acc(r, _rb(xn[b]) * wr[:, b * 128:(b + 1) * 128])
        return jax.nn.sigmoid(jnp.sum(r, axis=1, keepdims=True))

    xn = _ln(x0)
    wait('wq')
    relayout_q()
    ones_bd = bd(jnp.ones((8, 128), F32))
    q = [None] * 4
    for b in range(NB):
        lhs = jnp.concatenate([bd(xn[b]), ones_bd], axis=0)
        for g in range(4):
            q[g] = _acc(q[g], _dot(lhs, ld(WQ, (b,), g * 1024, 1024)))
    cs = [t[8:16] for t in q]
    q = [t[0:8] for t in q]
    t = pin(q + cs + x0, 'wuk')
    q, cs, x0 = t[:4], t[4:8], t[8:]
    relayout_k()
    qa, csk = [], []
    for g in range(4):
        lhs = jnp.concatenate([bd(q[g]), bd(cs[g])], axis=0)
        for cb in range(NCB):
            r = _dot(lhs, ld(WKT, (g * 4 + cb,), 0, 1024))
            qa.append(r[0:8])
            csk.append(r[8:16])
    t = pin(qa + csk, 'ckv0')
    qa, csk = t[:16], t[16:]
    qa = jnp.concatenate([jnp.concatenate(qa[g * 4:(g + 1) * 4], axis=1) for g in range(4)], axis=0)
    relayout_c()
    cc, inv = softmax_ctx(qa.astype(BF16))
    invb = jnp.broadcast_to(inv, (H, 128))
    t = pin([c[g * 8:(g + 1) * 8] for c in cc for g in range(4)]
            + [invb[g * 8:(g + 1) * 8] for g in range(4)], 'g')
    cc, inv = t[:16], t[16:]
    relayout_f(g_v, GT, G32)
    wait('u')
    relayout_f(u_v, UT, U32F)
    wait('wuv')
    relayout_v()
    ctx = []
    for g in range(4):
        lhs = jnp.concatenate([row_sel(cc[cb * 4 + g], j) for j in range(8) for cb in range(NCB)], axis=1)
        rhs = jnp.concatenate([ld(WV, (g * 8 + j,), 0, DC) for j in range(8)], axis=0)
        ctx.append(_dot(lhs, rhs) * inv[g])
    outs = [None] * NB
    for i in range(len(wo_b) - 1):
        if i == 0:
            ctx = pin(ctx, 'wo0')
        else:
            outs = pin(outs, f'wo{i}')
        hh = list(range(wo_b[i], wo_b[i + 1]))
        lhs = jnp.concatenate([row_sel(ctx[h // 8], h % 8) for h in hh], axis=1)
        for b in range(NB):
            outs[b] = _acc(outs[b], _dot(lhs, wo_v[pl.ds(hh[0] * D, len(hh) * D), pl.ds(b * 128, 128)]))
        relayout_o(wo_b[i], wo_b[i + 1])
    x1 = [a + _rowsum(o) for a, o in zip(x0, outs)]

    xn1 = _ln(x1)
    sg = router(xn1)
    lhs = jnp.concatenate([jnp.concatenate(xn1, axis=1), jnp.ones((8, M), F32)], axis=0)
    hs, cg, cu = [], [], []
    for fb in range(NFB):
        g = _dot(lhs, ld(GT, (fb,), 0, M))
        u = _dot(lhs, ld(UT, (fb,), 0, M))
        cg.append(g[8:16])
        cu.append(u[8:16])
        g, u = g[0:8], u[0:8]
        hs.append(g * jax.nn.sigmoid(g) * u)
    base = [a + b for a, b in zip(x1, xn1)]

    def down_tile(hs, fb, b):
        if fb == NFB - 1:
            return _dot(hs[fb][:, :64], wd_v[pl.ds(fb * 128, 64), pl.ds(b * 128, 128)])
        return _dot(hs[fb], wd_v[pl.ds(fb * 128, 128), pl.ds(b * 128, 128)])

    x2, xp = [None] * NB, [None] * NB
    qraw = [None] * 4
    deferred = []
    pivot = None
    nseg = len(wd_b) - 1
    for i in range(nseg):
        if i == 0:
            t = pin(hs + base + xn1 + [jnp.broadcast_to(sg, (8, 128))] + cg + cu, 'wd0')
            hs, base, xn1, sg = t[:NFB], t[NFB:NFB + 5], t[NFB + 5:NFB + 10], t[NFB + 10]
            cg, cu = t[NFB + 11:2 * NFB + 11], t[2 * NFB + 11:]
        else:
            done = [b for b in range(NB) if x2[b] is not None]
            gl = [g for g in range(4) if qraw[g] is not None]
            t = pin([qraw[g] for g in gl] + [x2[b] for b in done] + [xp[b] for b in done]
                    + [jnp.broadcast_to(pivot, (8, 128))], f'wd{i}')
            for n_, g in enumerate(gl):
                qraw[g] = t[n_]
            for n_, b in enumerate(done):
                x2[b] = t[len(gl) + n_]
                xp[b] = t[len(gl) + len(done) + n_]
            pivot = t[-1]
        blks = list(range(wd_b[i], wd_b[i + 1]))
        if i == 0:
            for fb in range(NY):
                HC[pl.ds(fb * 128, 128), :] = jnp.broadcast_to(hs[fb][0:1], (128, 128)).T
        for b in blks:
            y = None
            nv = NY if i == nseg - 1 else 0
            for fb in range(nv, NFB):
                y = _acc(y, down_tile(hs, fb, b))
            if nv:
                parts = [None] * 4
                for r in range(nv * 16):
                    t = wd_v[pl.ds(r * 8, 8), pl.ds(b * 128, 128)].astype(F32) * HC[pl.ds(r * 8, 8), :]
                    parts[r % 4] = _acc(parts[r % 4], t)
                y = y + _rowsum((parts[0] + parts[1]) + (parts[2] + parts[3]))
            x2[b] = base[b] + (xn1[b] * 0.0 + y * sg)
        if pivot is None:
            s = x2[blks[0]]
            for b in blks[1:]:
                s = s + x2[b]
            pivot = jnp.sum(s, axis=1, keepdims=True) * (1.0 / (128 * len(blks)))
        for b in blks:
            xp[b] = x2[b] - pivot
        todo = deferred + [(b, h) for b in blks for h in range(HQ, H)]
        deferred = []
        if i == nseg - 2 and QDEF:
            todo, deferred = todo[:-QDEF], todo[-QDEF:]
        for (b, h) in todo:
            qraw[h // 8] = _acc(qraw[h // 8], _dot(row_sel(xp[b], h % 8), ld(WQ, (b,), h * 128, 128)))
        if i < nseg - 1:
            for h in range(HQ):
                for r in range(16):
                    a = None if i == 0 else AE[h * 16 + r]
                    for b in blks:
                        a = _acc(a, WQT32[h * NB + b, pl.ds(r * 8, 8), :] * xp[b])
                    AE[h * 16 + r] = a

    mu, rs = _stats(xp)
    xc = [t - mu for t in xp]
    qa = [[None] * NCB for _ in range(4)]
    s2 = [(h, cb) for h in range(HQ, H) for cb in range(NCB)]
    if S2ORD:
        s2 = s2[:S2ORD * NCB] + [(h, cb) for cb in range(NCB) for h in range(HQ + S2ORD, H)]
    for h, cb in s2:
        g = h // 8
        qa[g][cb] = _acc(qa[g][cb], _dot(row_sel(qraw[g], h % 8), ld(WKT, (g * 4 + cb,), (h % 8) * 128, 128)))
    tmask = always(xp[wd_b[-2]])
    zq = []
    for h in range(HQ):
        xr = {b: xp[b] for b in range(wd_b[-2], NB)}
        if QBACK and h >= QBACK:
            xr = {b: jnp.where(tmask, v, zq[h - QBACK]) for b, v in xr.items()}
        acc = [None] * NCB
        for r in range(16):
            a = AE[h * 16 + r]
            for b, v in xr.items():
                a = a + WQT32[h * NB + b, pl.ds(r * 8, 8), :] * v
            cv = _lanesum(a)
            for cb in range(NCB):
                acc[cb] = _acc(acc[cb], WKT32[h * NCB + cb, pl.ds(r * 8, 8), :] * cv)
        z = acc[0]
        for cb in range(1, NCB):
            z = jnp.maximum(z, acc[cb])
        zq.append(z)
        for cb in range(NCB):
            prev = qa[h // 8][cb]
            qa[h // 8][cb] = jnp.where(row8 == h % 8, _rowsum(acc[cb]), 0.0 if prev is None else prev)
    qa = jnp.concatenate(
        [jnp.concatenate([(qa[g][cb] - mu * csk[g * 4 + cb]) * rs for cb in range(NCB)], axis=1)
         for g in range(4)], axis=0)
    cc, inv = softmax_ctx(qa.astype(BF16), KB0)

    invb = jnp.broadcast_to(inv, (H, 128))
    cn = [[cc[cb][g * 8:(g + 1) * 8] * invb[g * 8:(g + 1) * 8] for cb in range(NCB)] for g in range(4)]
    vmask = always(invb[0:8])
    accv = [None] * NB
    zv = []
    for h in range(HV):
        xr = [jnp.broadcast_to(cn[h // 8][cb][h % 8:h % 8 + 1], (8, 128)) for cb in range(NCB)]
        if VBACK and h >= VBACK:
            xr = [jnp.where(vmask, v, zv[h - VBACK]) for v in xr]
        for r in range(16):
            a = None
            for cb in range(NCB):
                a = _acc(a, WVT32[h * NCB + cb, pl.ds(r * 8, 8), :] * xr[cb])
            cv = _lanesum(a)
            for b in range(NB):
                accv[b] = _acc(accv[b], WO32[pl.ds(h * D + r * 8, 8), pl.ds(b * 128, 128)] * cv)
        z = accv[0]
        for b in range(1, NB):
            z = jnp.maximum(z, accv[b])
        zv.append(z)
    mh = list(range(HV, H))
    ctx = {}
    for g in range(HV // 8, 4):
        acc = None
        for h in range(max(HV, g * 8), g * 8 + 8):
            for cb in range(NCB):
                acc = _acc(acc, _dot(row_sel(cn[g][cb], h % 8), ld(WV, (h,), cb * 128, 128)))
        ctx[g] = acc
    lhs6 = {h: row_sel(ctx[h // 8], h % 8) for h in mh}
    outs = [None] * NB
    for seg in (mh[:-S6LAST], mh[-S6LAST:]):
        for b in range(NB):
            for h in seg:
                outs[b] = _acc(outs[b], _dot(lhs6[h], ld(WOT, (b,), (h - HV) * 128, 128)))
    out = [_rowsum(o if a is None else o + a) for o, a in zip(outs, accv)]

    x3 = [a + b for a, b in zip(x2, out)]
    x3p = [a + b for a, b in zip(xc, out)]
    mu, rs = _stats1(x3p)
    xn3 = [(t - mu) * rs for t in x3p]
    sg = router(xn3)
    gs, us = [None] * NFB, [None] * NFB
    mfb = list(range(NVF, NFB))
    for b in range(NB):
        for fb in mfb[:NF0]:
            gs[fb] = _acc(gs[fb], _dot(x3p[b], ld(GT, (fb,), b * 128, 128)))
            us[fb] = _acc(us[fb], _dot(x3p[b], ld(UT, (fb,), b * 128, 128)))
    for fb in mfb[NF0:]:
        for b in range(NB):
            gs[fb] = _acc(gs[fb], _dot(x3p[b], ld(GT, (fb,), b * 128, 128)))
        for b in range(NB):
            us[fb] = _acc(us[fb], _dot(x3p[b], ld(UT, (fb,), b * 128, 128)))

    def vpu_col(W, fb):
        a = []
        for i in range(16):
            t = None
            for b in range(NB):
                t = _acc(t, W[pl.ds(fb * 128 + i * 8, 8), pl.ds(b * 128, 128)] * x3p[b])
            a.append(t)
        at = jnp.concatenate(a, axis=0).T
        parts = [at[i * 8:(i + 1) * 8] for i in range(16)]
        while len(parts) > 1:
            parts = [parts[i] + parts[i + 1] for i in range(0, len(parts), 2)]
        return _rowsum(parts[0])

    for fb in range(NVF):
        gs[fb] = vpu_col(G32, fb)
        us[fb] = vpu_col(U32F, fb)
    hs = [None] * NFB
    ys = [None] * NB
    for fb in mfb + list(range(NVF)):
        g = (gs[fb] - mu * cg[fb]) * rs
        u = (us[fb] - mu * cu[fb]) * rs
        hs[fb] = g * jax.nn.sigmoid(g) * u
        for b in range(NB):
            ys[b] = _acc(ys[b], down_tile(hs, fb, b))
    base = [x3[b] + (xn3[b] + xn3[b] * 0.0) for b in range(NB)]
    finish([base[b] + ys[b] * sg for b in range(NB)])


@jax.jit
def pallas_interleave_layers__compressed_kv_cla__moe_arch_mod__decode_kernel(
    A_x, A_c_kv, A_w_q, A_w_uk, A_w_uv, A_w_o, B_x, B_w_r, B_w_gate, B_w_up, B_w_down,
):
    hbm = pl.BlockSpec(memory_space=pltpu.HBM)
    vm = pltpu.VMEM
    return pl.pallas_call(
        _kernel,
        out_shape=jax.ShapeDtypeStruct((1, 1, M), BF16),
        in_specs=[hbm] * 10,
        scratch_shapes=[
            vm((1, 1, M), BF16), vm((M,), BF16),
            vm((M * H + PAD, D), BF16), vm((DC * H + PAD, D), BF16), vm((NCB, SK, 128), BF16),
            vm((DC * H + PAD, D), BF16), vm((H * D, M), BF16),
            vm((FF, M), BF16), vm((FF, M), BF16), vm((FF, M), BF16),
            vm((NB, H * 64, 128), U32), vm((16, 512, 128), U32), vm((NKB, DC // 2, 128), U32),
            vm((H, DC // 2, 128), U32), vm((NFB, M // 2, 128), U32), vm((NFB, M // 2, 128), U32),
            vm((HQ * NB, 128, 128), F32), vm((HQ * NCB, 128, 128), F32),
            vm((HV * NCB, 128, 128), F32), vm((HV * D, M), F32),
            vm((NB, (H - HV) * 64, 128), U32),
            vm((NVF * 128, M), F32), vm((NVF * 128, M), F32),
            vm((HQ * 16, 8, 128), F32), vm((NY * 128, 128), F32), vm((N_PIN, 8, 128), F32),
            pltpu.SemaphoreType.DMA((N_SEM,)),
        ],
        compiler_params=pltpu.CompilerParams(
            vmem_limit_bytes=110 * 1024 * 1024, disable_semaphore_checks=True),
        name="cla_moe_decode",
    )(A_x, A_w_q.reshape(M * H, D), A_w_uk.reshape(DC * H, D), A_c_kv.reshape(SK, DC),
      A_w_uv.reshape(DC * H, D), A_w_o.reshape(H * D, M), B_w_r, B_w_gate.T, B_w_up.T, B_w_down)
```

```python
import jax
import numpy as np
import jax.numpy as jnp
import jax.experimental.pallas as pl
import jax.experimental.pallas.tpu as pltpu

F32 = jnp.float32
BF16 = jnp.bfloat16
U32 = jnp.uint32
U16 = jnp.uint16
I32 = jnp.int32

M, H, D, SK, DC, FF = 640, 32, 128, 4096, 512, 1728
NB = M // 128
NCB = DC // 128
NKB = SK // 128
NFB = (FF + 127) // 128
EPS = 1e-5

HQ, QBACK = 12, 5
HV, VBACK = 17, 3
NVF = 7
NY = 10
QDEF, KB0, S2ORD, S6LAST, NF0 = 4, 6, 12, 8, 3
SM_SPLIT = 20
WO_SPLIT = [16, 24]
WD_SPLIT = [2, 4]
PAD = 32
N_PIN = 176
N_SEM = 17


def _rb(x):
    return x.astype(BF16).astype(F32)


def _dot(a, b):
    return jax.lax.dot_general(a, b, (((1,), (0,)), ((), ())), preferred_element_type=F32)


def _acc(a, t):
    return t if a is None else a + t


def _stats(parts):
    s = parts[0]
    for p in parts[1:]:
        s = s + p
    m = jnp.sum(s, axis=1, keepdims=True) * (1.0 / M)
    c = [p - m for p in parts]
    v = c[0] * c[0]
    for p in c[1:]:
        v = v + p * p
    v = jnp.sum(v, axis=1, keepdims=True) * (1.0 / M)
    return m, jax.lax.rsqrt(v + EPS)


def _stats1(parts):
    s, v = parts[0], parts[0] * parts[0]
    for p in parts[1:]:
        s, v = s + p, v + p * p
    m = jnp.sum(s, axis=1, keepdims=True) * (1.0 / M)
    v = jnp.sum(v, axis=1, keepdims=True) * (1.0 / M) - m * m
    return m, jax.lax.rsqrt(jnp.maximum(v, 0.0) + EPS)


def _ln(parts):
    m, r = _stats(parts)
    return [(p - m) * r for p in parts]


def _rowsum(a):
    return jnp.broadcast_to(jnp.sum(a, axis=0, keepdims=True), (8, 128))


def _lanesum(a):
    return jnp.broadcast_to(jnp.sum(a, axis=1, keepdims=True), (8, 128))


def _kernel(x_hbm, wq_hbm, wuk_hbm, ckv_hbm, wuv_hbm, wo_hbm, wr_hbm, g_hbm, u_hbm, wd_hbm,
            o_ref,
            x_v, wr_v, wq_v, wuk_v, ckv_v, wuv_v, wo_v, g_v, u_v, wd_v,
            WQ, WKT, CT, WV, GT, UT,
            WQT32, WKT32, WVT32, WO32, WOT, G32, U32F, AE, HC, PIN, sems):
    cps = {}

    def add(name, src, dst):
        cps[name] = pltpu.make_async_copy(src, dst, sems.at[len(cps)])

    add('wq', wq_hbm, wq_v.at[pl.ds(0, M * H)])
    add('x', x_hbm, x_v)
    add('wr', wr_hbm, wr_v)
    add('wuk', wuk_hbm, wuk_v.at[pl.ds(0, DC * H)])
    for j in range(NCB):
        add(f'ckv{j}', ckv_hbm.at[:, pl.ds(128 * j, 128)], ckv_v.at[j])
    add('g', g_hbm, g_v)
    add('u', u_hbm, u_v)
    add('wuv', wuv_hbm, wuv_v.at[pl.ds(0, DC * H)])
    wo_b = [0] + WO_SPLIT + [H]
    for i in range(len(wo_b) - 1):
        sl = pl.ds(wo_b[i] * D, (wo_b[i + 1] - wo_b[i]) * D)
        add(f'wo{i}', wo_hbm.at[sl], wo_v.at[sl])
    wd_b = [0] + WD_SPLIT + [NB]
    for i in range(len(wd_b) - 1):
        sl = pl.ds(wd_b[i] * 128, (wd_b[i + 1] - wd_b[i]) * 128)
        add(f'wd{i}', wd_hbm.at[:, sl], wd_v.at[:, sl])
    assert len(cps) <= N_SEM
    for c in cps.values():
        c.start()
    waited = set()

    def wait(name):
        if name not in waited:
            cps[name].wait()
            waited.add(name)

    pin_n = [0]

    def pin(vals, *names):
        k0 = pin_n[0]
        for i, v in enumerate(vals):
            PIN[k0 + i] = v
        pin_n[0] += len(vals)
        assert pin_n[0] <= N_PIN
        for nm in names:
            wait(nm)
        return [PIN[k0 + i] for i in range(len(vals))]

    wq_u, wuk_u, wuv_u, ckv_u = (r.bitcast(U32) for r in (wq_v, wuk_v, wuv_v, ckv_v))

    def ld(uref, idx, r0, nrows):
        return pltpu.bitcast(uref[(*idx, pl.ds(r0 // 2, nrows // 2), slice(None))], BF16)

    def shuf(src_u, r0, s):
        a = src_u[pl.ds(r0 * 16 + s, 8, stride=16), :]
        b = src_u[pl.ds((r0 + 8) * 16 + s, 8, stride=16), :]
        xx = jnp.concatenate([a, b], axis=0)
        lo = pltpu.bitcast(xx.astype(U16), U32)
        hi = pltpu.bitcast((xx >> 16).astype(U16), U32)
        return lo, hi

    def relayout_q():
        for i in range(M // 16):
            b, m16 = divmod(i, 8)
            for s in range(16):
                lo, hi = shuf(wq_u, i * 16, s)
                WQ[b, pl.ds(2 * s * 64 + m16 * 8, 8), :] = lo
                WQ[b, pl.ds((2 * s + 1) * 64 + m16 * 8, 8), :] = hi
        for h in range(HQ):
            for b in range(NB):
                WQT32[h * NB + b] = ld(WQ, (b,), h * 128, 128).T.astype(F32)

    def relayout_k():
        for cb in range(NCB):
            for s in range(16):
                los, his = [], []
                for i in range(8):
                    lo, hi = shuf(wuk_u, cb * 128 + i * 16, s)
                    los.append(lo)
                    his.append(hi)
                for h, parts in ((2 * s, los), (2 * s + 1, his)):
                    t = pltpu.bitcast(jnp.concatenate(parts, axis=0), BF16).T
                    WKT[(h // 8) * 4 + cb, pl.ds((h % 8) * 64, 64), :] = pltpu.bitcast(t, U32)
                    if h < HQ:
                        WKT32[h * NCB + cb] = t.astype(F32)

    def relayout_c():
        for cb in range(NCB):
            wait(f'ckv{cb}')
            for kb in range(NKB):
                t = ld(ckv_u, (cb,), kb * 128, 128).T
                CT[kb, pl.ds(cb * 64, 64), :] = pltpu.bitcast(t, U32)

    def relayout_f(src, dst, dst32):
        for fb in range(NFB):
            for b in range(NB):
                if fb < NFB - 1:
                    t = src[pl.ds(fb * 128, 128), pl.ds(b * 128, 128)]
                else:
                    t = src[pl.ds(fb * 128, 64), pl.ds(b * 128, 128)]
                    t = jnp.concatenate([t, jnp.zeros((64, 128), BF16)], axis=0)
                dst[fb, pl.ds(b * 64, 64), :] = pltpu.bitcast(t.T, U32)
        for r in range(NVF * 16):
            dst32[pl.ds(r * 8, 8), :] = src[pl.ds(r * 8, 8), :].astype(F32)

    def relayout_v():
        for i in range(DC // 16):
            for s in range(16):
                lo, hi = shuf(wuv_u, i * 16, s)
                WV[2 * s, pl.ds(i * 8, 8), :] = lo
                WV[2 * s + 1, pl.ds(i * 8, 8), :] = hi
        if HV:
            per = -(-HV // 2)

            def body(it, _):
                for k in range(per):
                    h = jnp.minimum(it * per + k, HV - 1)
                    for cb in range(NCB):
                        WVT32[h * NCB + cb] = ld(WV, (h,), cb * 128, 128).T.astype(F32)
                return 0
            jax.lax.fori_loop(0, 2, body, 0)

    def relayout_o(h0, h1):
        for h in range(h0, h1):
            if h < HV:
                for i in range(16):
                    WO32[pl.ds(h * D + i * 8, 8), :] = wo_v[pl.ds(h * D + i * 8, 8), :].astype(F32)
            else:
                for b in range(NB):
                    WOT[b, pl.ds((h - HV) * 64, 64), :] = pltpu.bitcast(
                        wo_v[pl.ds(h * D, D), pl.ds(b * 128, 128)], U32)

    row8 = jax.lax.broadcasted_iota(I32, (8, 128), 0)

    def row_sel(v, j):
        return jnp.where(row8 == j, v, 0.0)

    def bd(v):
        return jnp.concatenate([row_sel(v, j) for j in range(8)], axis=1)

    def always(v):
        return (pltpu.bitcast(v, I32) | 1) != 0

    scale = D ** -0.5

    def softmax_ctx(qa, kb0=0):
        bnd = (0, SM_SPLIT, NKB)
        nblk = 2
        sall = [None] * NKB
        qc = [qa[:, cb * 128:(cb + 1) * 128] for cb in range(NCB)]
        for cb in range(NCB):
            for kb in range(kb0):
                sall[kb] = _acc(sall[kb], _dot(qc[cb], ld(CT, (kb,), cb * 128, 128)))
        for kb in range(kb0, NKB):
            sall[kb] = _dot(qa, ld(CT, (kb,), 0, DC))
        ss = [sall[bnd[blk]:bnd[blk + 1]] for blk in range(nblk)]
        m_run = l_run = acc = None
        for blk in range(nblk):
            s = ss[blk]
            mx = s[0]
            for t in s[1:]:
                mx = jnp.maximum(mx, t)
            mx = jnp.max(mx, axis=1, keepdims=True)
            if m_run is not None:
                mx = jnp.maximum(mx, m_run)
            p = [jnp.exp((t - mx) * scale) for t in s]
            l = p[0]
            for t in p[1:]:
                l = l + t
            pb = jnp.concatenate([t.astype(BF16) for t in p], axis=1)
            cc = [_dot(pb, ld(ckv_u, (cb,), bnd[blk] * 128, (bnd[blk + 1] - bnd[blk]) * 128)) for cb in range(NCB)]
            if m_run is not None:
                al = jnp.exp((m_run - mx) * scale)
                cc = [c + a * al for c, a in zip(cc, acc)]
                l = l + l_run * al
            m_run, l_run, acc = mx, l, cc
        return acc, 1.0 / jnp.sum(l_run, axis=1, keepdims=True)

    def finish(x):
        for b in range(NB):
            o_ref[0, :, pl.ds(b * 128, 128)] = x[b][0:1].astype(BF16)
        for name in cps:
            wait(name)

    wait('x')
    wait('wr')
    x0 = jnp.broadcast_to(x_v[0].astype(F32), (8, M))
    x0 = [x0[:, b * 128:(b + 1) * 128] for b in range(NB)]
    wr = wr_v[...].reshape(1, M).astype(F32)

    def router(xn):
        r = None
        for b in range(NB):
            r = _acc(r, _rb(xn[b]) * wr[:, b * 128:(b + 1) * 128])
        return jax.nn.sigmoid(jnp.sum(r, axis=1, keepdims=True))

    xn = _ln(x0)
    wait('wq')
    relayout_q()
    ones_bd = bd(jnp.ones((8, 128), F32))
    q = [None] * 4
    for b in range(NB):
        lhs = jnp.concatenate([bd(xn[b]), ones_bd], axis=0)
        for g in range(4):
            q[g] = _acc(q[g], _dot(lhs, ld(WQ, (b,), g * 1024, 1024)))
    cs = [t[8:16] for t in q]
    q = [t[0:8] for t in q]
    t = pin(q + cs + x0, 'wuk')
    q, cs, x0 = t[:4], t[4:8], t[8:]
    relayout_k()
    qa, csk = [], []
    for g in range(4):
        lhs = jnp.concatenate([bd(q[g]), bd(cs[g])], axis=0)
        for cb in range(NCB):
            r = _dot(lhs, ld(WKT, (g * 4 + cb,), 0, 1024))
            qa.append(r[0:8])
            csk.append(r[8:16])
    t = pin(qa + csk, 'ckv0')
    qa, csk = t[:16], t[16:]
    qa = jnp.concatenate([jnp.concatenate(qa[g * 4:(g + 1) * 4], axis=1) for g in range(4)], axis=0)
    relayout_c()
    cc, inv = softmax_ctx(qa.astype(BF16))
    invb = jnp.broadcast_to(inv, (H, 128))
    t = pin([c[g * 8:(g + 1) * 8] for c in cc for g in range(4)]
            + [invb[g * 8:(g + 1) * 8] for g in range(4)], 'g')
    cc, inv = t[:16], t[16:]
    relayout_f(g_v, GT, G32)
    wait('u')
    relayout_f(u_v, UT, U32F)
    wait('wuv')
    relayout_v()
    ctx = []
    for g in range(4):
        lhs = jnp.concatenate([row_sel(cc[cb * 4 + g], j) for j in range(8) for cb in range(NCB)], axis=1)
        rhs = jnp.concatenate([ld(WV, (g * 8 + j,), 0, DC) for j in range(8)], axis=0)
        ctx.append(_dot(lhs, rhs) * inv[g])
    outs = [None] * NB
    for i in range(len(wo_b) - 1):
        if i == 0:
            ctx = pin(ctx, 'wo0')
        else:
            outs = pin(outs, f'wo{i}')
        hh = list(range(wo_b[i], wo_b[i + 1]))
        lhs = jnp.concatenate([row_sel(ctx[h // 8], h % 8) for h in hh], axis=1)
        for b in range(NB):
            outs[b] = _acc(outs[b], _dot(lhs, wo_v[pl.ds(hh[0] * D, len(hh) * D), pl.ds(b * 128, 128)]))
        relayout_o(wo_b[i], wo_b[i + 1])
    x1 = [a + _rowsum(o) for a, o in zip(x0, outs)]

    xn1 = _ln(x1)
    sg = router(xn1)
    lhs = jnp.concatenate([jnp.concatenate(xn1, axis=1), jnp.ones((8, M), F32)], axis=0)
    hs, cg, cu = [], [], []
    for fb in range(NFB):
        g = _dot(lhs, ld(GT, (fb,), 0, M))
        u = _dot(lhs, ld(UT, (fb,), 0, M))
        cg.append(g[8:16])
        cu.append(u[8:16])
        g, u = g[0:8], u[0:8]
        hs.append(g * jax.nn.sigmoid(g) * u)
    base = [a + b for a, b in zip(x1, xn1)]

    def down_tile(hs, fb, b):
        if fb == NFB - 1:
            return _dot(hs[fb][:, :64], wd_v[pl.ds(fb * 128, 64), pl.ds(b * 128, 128)])
        return _dot(hs[fb], wd_v[pl.ds(fb * 128, 128), pl.ds(b * 128, 128)])

    x2, xp = [None] * NB, [None] * NB
    qraw = [None] * 4
    deferred = []
    pivot = None
    nseg = len(wd_b) - 1
    for i in range(nseg):
        if i == 0:
            t = pin(hs + base + xn1 + [jnp.broadcast_to(sg, (8, 128))] + cg + cu, 'wd0')
            hs, base, xn1, sg = t[:NFB], t[NFB:NFB + 5], t[NFB + 5:NFB + 10], t[NFB + 10]
            cg, cu = t[NFB + 11:2 * NFB + 11], t[2 * NFB + 11:]
        else:
            done = [b for b in range(NB) if x2[b] is not None]
            gl = [g for g in range(4) if qraw[g] is not None]
            t = pin([qraw[g] for g in gl] + [x2[b] for b in done] + [xp[b] for b in done]
                    + [jnp.broadcast_to(pivot, (8, 128))], f'wd{i}')
            for n_, g in enumerate(gl):
                qraw[g] = t[n_]
            for n_, b in enumerate(done):
                x2[b] = t[len(gl) + n_]
                xp[b] = t[len(gl) + len(done) + n_]
            pivot = t[-1]
        blks = list(range(wd_b[i], wd_b[i + 1]))
        if i == 0:
            for fb in range(NY):
                HC[pl.ds(fb * 128, 128), :] = jnp.broadcast_to(hs[fb][0:1], (128, 128)).T
        for b in blks:
            y = None
            nv = NY if i == nseg - 1 else 0
            for fb in range(nv, NFB):
                y = _acc(y, down_tile(hs, fb, b))
            if nv:
                parts = [None] * 4
                for r in range(nv * 16):
                    t = wd_v[pl.ds(r * 8, 8), pl.ds(b * 128, 128)].astype(F32) * HC[pl.ds(r * 8, 8), :]
                    parts[r % 4] = _acc(parts[r % 4], t)
                y = y + _rowsum((parts[0] + parts[1]) + (parts[2] + parts[3]))
            x2[b] = base[b] + (xn1[b] * 0.0 + y * sg)
        if pivot is None:
            s = x2[blks[0]]
            for b in blks[1:]:
                s = s + x2[b]
            pivot = jnp.sum(s, axis=1, keepdims=True) * (1.0 / (128 * len(blks)))
        for b in blks:
            xp[b] = x2[b] - pivot
        todo = deferred + [(b, h) for b in blks for h in range(HQ, H)]
        deferred = []
        if i == nseg - 2 and QDEF:
            todo, deferred = todo[:-QDEF], todo[-QDEF:]
        for (b, h) in todo:
            qraw[h // 8] = _acc(qraw[h // 8], _dot(row_sel(xp[b], h % 8), ld(WQ, (b,), h * 128, 128)))
        if i < nseg - 1:
            for h in range(HQ):
                for r in range(16):
                    a = None if i == 0 else AE[h * 16 + r]
                    for b in blks:
                        a = _acc(a, WQT32[h * NB + b, pl.ds(r * 8, 8), :] * xp[b])
                    AE[h * 16 + r] = a

    mu, rs = _stats(xp)
    xc = [t - mu for t in xp]
    qa = [[None] * NCB for _ in range(4)]
    s2 = [(h, cb) for h in range(HQ, H) for cb in range(NCB)]
    if S2ORD:
        s2 = s2[:S2ORD * NCB] + [(h, cb) for cb in range(NCB) for h in range(HQ + S2ORD, H)]
    for h, cb in s2:
        g = h // 8
        qa[g][cb] = _acc(qa[g][cb], _dot(row_sel(qraw[g], h % 8), ld(WKT, (g * 4 + cb,), (h % 8) * 128, 128)))
    tmask = always(xp[wd_b[-2]])
    zq = []
    for h in range(HQ):
        xr = {b: xp[b] for b in range(wd_b[-2], NB)}
        if QBACK and h >= QBACK:
            xr = {b: jnp.where(tmask, v, zq[h - QBACK]) for b, v in xr.items()}
        acc = [None] * NCB
        for r in range(16):
            a = AE[h * 16 + r]
            for b, v in xr.items():
                a = a + WQT32[h * NB + b, pl.ds(r * 8, 8), :] * v
            cv = _lanesum(a)
            for cb in range(NCB):
                acc[cb] = _acc(acc[cb], WKT32[h * NCB + cb, pl.ds(r * 8, 8), :] * cv)
        z = acc[0]
        for cb in range(1, NCB):
            z = jnp.maximum(z, acc[cb])
        zq.append(z)
        for cb in range(NCB):
            prev = qa[h // 8][cb]
            qa[h // 8][cb] = jnp.where(row8 == h % 8, _rowsum(acc[cb]), 0.0 if prev is None else prev)
    qa = jnp.concatenate(
        [jnp.concatenate([(qa[g][cb] - mu * csk[g * 4 + cb]) * rs for cb in range(NCB)], axis=1)
         for g in range(4)], axis=0)
    cc, inv = softmax_ctx(qa.astype(BF16), KB0)

    invb = jnp.broadcast_to(inv, (H, 128))
    cn = [[cc[cb][g * 8:(g + 1) * 8] * invb[g * 8:(g + 1) * 8] for cb in range(NCB)] for g in range(4)]
    vmask = always(invb[0:8])
    accv = [None] * NB
    zv = []
    for h in range(HV):
        xr = [jnp.broadcast_to(cn[h // 8][cb][h % 8:h % 8 + 1], (8, 128)) for cb in range(NCB)]
        if VBACK and h >= VBACK:
            xr = [jnp.where(vmask, v, zv[h - VBACK]) for v in xr]
        for r in range(16):
            a = None
            for cb in range(NCB):
                a = _acc(a, WVT32[h * NCB + cb, pl.ds(r * 8, 8), :] * xr[cb])
            cv = _lanesum(a)
            for b in range(NB):
                accv[b] = _acc(accv[b], WO32[pl.ds(h * D + r * 8, 8), pl.ds(b * 128, 128)] * cv)
        z = accv[0]
        for b in range(1, NB):
            z = jnp.maximum(z, accv[b])
        zv.append(z)
    mh = list(range(HV, H))
    ctx = {}
    for g in range(HV // 8, 4):
        acc = None
        for h in range(max(HV, g * 8), g * 8 + 8):
            for cb in range(NCB):
                acc = _acc(acc, _dot(row_sel(cn[g][cb], h % 8), ld(WV, (h,), cb * 128, 128)))
        ctx[g] = acc
    lhs6 = {h: row_sel(ctx[h // 8], h % 8) for h in mh}
    outs = [None] * NB
    for seg in (mh[:-S6LAST], mh[-S6LAST:]):
        for b in range(NB):
            for h in seg:
                outs[b] = _acc(outs[b], _dot(lhs6[h], ld(WOT, (b,), (h - HV) * 128, 128)))
    out = [_rowsum(o if a is None else o + a) for o, a in zip(outs, accv)]

    x3 = [a + b for a, b in zip(x2, out)]
    x3p = [a + b for a, b in zip(xc, out)]
    mu, rs = _stats1(x3p)
    xn3 = [(t - mu) * rs for t in x3p]
    sg = router(xn3)
    gs, us = [None] * NFB, [None] * NFB
    mfb = list(range(NVF, NFB))
    for b in range(NB):
        for fb in mfb[:NF0]:
            gs[fb] = _acc(gs[fb], _dot(x3p[b], ld(GT, (fb,), b * 128, 128)))
            us[fb] = _acc(us[fb], _dot(x3p[b], ld(UT, (fb,), b * 128, 128)))
    for fb in mfb[NF0:]:
        for b in range(NB):
            gs[fb] = _acc(gs[fb], _dot(x3p[b], ld(GT, (fb,), b * 128, 128)))
        for b in range(NB):
            us[fb] = _acc(us[fb], _dot(x3p[b], ld(UT, (fb,), b * 128, 128)))

    def vpu_col(W, fb):
        a = []
        for i in range(16):
            t = None
            for b in range(NB):
                t = _acc(t, W[pl.ds(fb * 128 + i * 8, 8), pl.ds(b * 128, 128)] * x3p[b])
            a.append(t)
        at = jnp.concatenate(a, axis=0).T
        parts = [at[i * 8:(i + 1) * 8] for i in range(16)]
        while len(parts) > 1:
            parts = [parts[i] + parts[i + 1] for i in range(0, len(parts), 2)]
        return _rowsum(parts[0])

    for fb in range(NVF):
        gs[fb] = vpu_col(G32, fb)
        us[fb] = vpu_col(U32F, fb)
    hs = [None] * NFB
    ys = [None] * NB
    for fb in mfb + list(range(NVF)):
        g = (gs[fb] - mu * cg[fb]) * rs
        u = (us[fb] - mu * cu[fb]) * rs
        hs[fb] = g * jax.nn.sigmoid(g) * u
        for b in range(NB):
            ys[b] = _acc(ys[b], down_tile(hs, fb, b))
    base = [x3[b] + (xn3[b] + xn3[b] * 0.0) for b in range(NB)]
    finish([base[b] + ys[b] * sg for b in range(NB)])


@jax.jit
def pallas_interleave_layers__compressed_kv_cla__moe_arch_mod__decode_kernel(
    A_x, A_c_kv, A_w_q, A_w_uk, A_w_uv, A_w_o, B_x, B_w_r, B_w_gate, B_w_up, B_w_down,
):
    hbm = pl.BlockSpec(memory_space=pltpu.HBM)
    vm = pltpu.VMEM
    return pl.pallas_call(
        _kernel,
        out_shape=jax.ShapeDtypeStruct((1, 1, M), BF16),
        in_specs=[hbm] * 10,
        scratch_shapes=[
            vm((1, 1, M), BF16), vm((M,), BF16),
            vm((M * H + PAD, D), BF16), vm((DC * H + PAD, D), BF16), vm((NCB, SK, 128), BF16),
            vm((DC * H + PAD, D), BF16), vm((H * D, M), BF16),
            vm((FF, M), BF16), vm((FF, M), BF16), vm((FF, M), BF16),
            vm((NB, H * 64, 128), U32), vm((16, 512, 128), U32), vm((NKB, DC // 2, 128), U32),
            vm((H, DC // 2, 128), U32), vm((NFB, M // 2, 128), U32), vm((NFB, M // 2, 128), U32),
            vm((HQ * NB, 128, 128), F32), vm((HQ * NCB, 128, 128), F32),
            vm((HV * NCB, 128, 128), F32), vm((HV * D, M), F32),
            vm((NB, (H - HV) * 64, 128), U32),
            vm((NVF * 128, M), F32), vm((NVF * 128, M), F32),
            vm((HQ * 16, 8, 128), F32), vm((NY * 128, 128), F32), vm((N_PIN, 8, 128), F32),
            pltpu.SemaphoreType.DMA((N_SEM,)),
        ],
        compiler_params=pltpu.CompilerParams(
            vmem_limit_bytes=110 * 1024 * 1024, disable_semaphore_checks=True),
        name="cla_moe_decode",
    )(A_x, A_w_q.reshape(M * H, D), A_w_uk.reshape(DC * H, D), A_c_kv.reshape(SK, DC),
      A_w_uv.reshape(DC * H, D), A_w_o.reshape(H * D, M), B_w_r, B_w_gate.T, B_w_up.T, B_w_down)
```
